```python
import jax
import jax.numpy as jnp

def _softmax(x, axis=-1):
    return jax.nn.softmax(x, axis=axis)

def _gelu(x):
    return jax.nn.gelu(x, approximate=True)

def _silu(x):
    return jax.nn.silu(x)

def _sigmoid(x):
    return jax.nn.sigmoid(x)

def _layernorm(x, axis=-1, eps=1e-05):
    m = jnp.mean(x, axis=axis, keepdims=True)
    v = jnp.var(x, axis=axis, keepdims=True)
    return (x - m) / jnp.sqrt(v + eps)

def _scatter_add(tgt, idx, src, axis=0):
    return tgt.at[idx].add(src)

def _segment_sum(src, seg, n):
    return jax.ops.segment_sum(src, seg, n)

class _Rng:

    def __init__(self, key):
        self._k = key

    def _next(self):
        self._k, sub = jax.random.split(self._k)
        return sub

    def normal(self, shape):
        return jax.random.normal(self._next(), shape, dtype=jnp.bfloat16)

    def randint(self, lo, hi, shape):
        return jax.random.randint(self._next(), shape, lo, hi, dtype=jnp.int32)

    def uniform(self, shape, lo=0.0, hi=1.0):
        return jax.random.uniform(self._next(), shape, jnp.bfloat16, lo, hi)

    def permutation(self, n):
        return jax.random.permutation(self._next(), n)
kernel_name = 'parallel_sum__memory_aug_infini_attn__moe_arch_mod__prompt'

def setup_inputs():
    _rng = _Rng(jax.random.key(int.from_bytes(__import__("os").urandom(4), "little")))
    _w = lambda a: (lambda t: t.astype(jnp.bfloat16) if jnp.issubdtype(t.dtype, jnp.floating) else t)(jnp.asarray(a))

    def _A_setup():
        B, S, D, H = (1, 2048, 576, 32)
        N = 4
        L = max(1, S // N)
        sc = D ** (-0.5)
        return {'x': _w((lambda *s: _rng.normal(s) * 0.05)(B, N * L, D)), 'wq': _w((lambda *s: _rng.normal(s) * 0.05)(D, D) * sc), 'wk': _w((lambda *s: _rng.normal(s) * 0.05)(D, D) * sc), 'wv': _w((lambda *s: _rng.normal(s) * 0.05)(D, D) * sc), 'wo': _w((lambda *s: _rng.normal(s) * 0.05)(D, D) * sc), 'beta': _w((lambda *s: _rng.normal(s) * 0.05)(H))}
    _A_in = _A_setup()

    def _B_setup():
        B, S, D, F, C = (1, 2048, 576, 4608, 2)
        return {'x': _w((lambda *s: _rng.normal(s) * 0.05)(B, S, D)), 'w_r': _w((lambda *s: _rng.normal(s) * 0.05)(D)), 'w_gate': _w((lambda *s: _rng.normal(s) * 0.05)(D, F)), 'w_up': _w((lambda *s: _rng.normal(s) * 0.05)(D, F)), 'w_down': _w((lambda *s: _rng.normal(s) * 0.05)(F, D))}
    _B_in = _B_setup()
    return {'A_x': _A_in['x'], 'A_wq': _A_in['wq'], 'A_wk': _A_in['wk'], 'A_wv': _A_in['wv'], 'A_wo': _A_in['wo'], 'A_beta': _A_in['beta'], 'B_x': _B_in['x'], 'B_w_r': _B_in['w_r'], 'B_w_gate': _B_in['w_gate'], 'B_w_up': _B_in['w_up'], 'B_w_down': _B_in['w_down']}

def reference(A_x, A_wq, A_wk, A_wv, A_wo, A_beta, B_x, B_w_r, B_w_gate, B_w_up, B_w_down):

    def _A_ref(x, wq, wk, wv, wo, beta):
        B, S, D = x.shape
        H = 32
        Dh = D // H
        N = 4
        L = S // N
        q = (lambda x, *d: x.transpose(*d))((x @ wq).reshape(B, S, H, Dh), 0, 2, 1, 3).reshape(B, H, N, L, Dh)
        k = (lambda x, *d: x.transpose(*d))((x @ wk).reshape(B, S, H, Dh), 0, 2, 1, 3).reshape(B, H, N, L, Dh)
        v = (lambda x, *d: x.transpose(*d))((x @ wv).reshape(B, S, H, Dh), 0, 2, 1, 3).reshape(B, H, N, L, Dh)
        phi = lambda t: jnp.where(t > 0, t + 1.0, jnp.exp(t))
        scale = Dh ** (-0.5)
        ar = jnp.arange(L)
        mask = (lambda x, dt: x.astype(dt))(ar[:, None] < ar[None, :], x.dtype) * -1000000000.0
        g = _sigmoid(beta).reshape(1, H, 1, 1)
        M = jnp.einsum('bhd,bhe->bhde', q[:, :, 0, 0, :] * 0.0, q[:, :, 0, 0, :] * 0.0)
        z = q[:, :, 0, 0, :] * 0.0
        outs = []
        for s in range(N):
            qs, ks, vs = (q[:, :, s].copy(), k[:, :, s].copy(), v[:, :, s].copy())
            logits = jnp.einsum('bhqd,bhkd->bhqk', qs, ks) * scale + mask
            p = _softmax(logits, axis=-1)
            a_dot = jnp.einsum('bhqk,bhkd->bhqd', p, vs)
            pq = phi(qs)
            num = jnp.einsum('bhld,bhde->bhle', pq, M)
            den = jnp.einsum('bhld,bhd->bhl', pq, z)[..., None] + 1e-06
            a_mem = num / den
            o = g * a_mem + (1.0 - g) * a_dot
            outs.append(o)
            pk = phi(ks)
            M = M + jnp.einsum('bhld,bhle->bhde', pk, vs)
            z = z + jnp.einsum('bhld->bhd', pk)
        o = (lambda x, *d: x.transpose(*d))(jnp.stack(outs, 2).reshape(B, H, S, Dh), 0, 2, 1, 3).reshape(B, S, D)
        return o @ wo

    def _B_ref(x, w_r, w_gate, w_up, w_down):
        B, S, D = x.shape
        C = 2
        r = x @ w_r
        idx = jnp.argsort(-r, axis=-1)[:, :C]
        idx_e = jnp.repeat(idx.reshape(B, C, 1), D, axis=2)
        x_sel = jnp.take_along_axis(x, idx_e, axis=1)
        g = _silu(x_sel @ w_gate)
        u = x_sel @ w_up
        y = g * u @ w_down
        r_sel = _sigmoid(jnp.take_along_axis(r, idx, axis=1))
        y = y * r_sel.reshape(B, C, 1)
        b_off = (jnp.arange(B) * S).reshape(B, 1)
        flat_idx = (idx + b_off).reshape(B * C)
        zero = (x * 0.0).reshape(B * S, D)
        upd = _scatter_add(zero, flat_idx, y.reshape(B * C, D), axis=0)
        return x + upd.reshape(B, S, D)
    x = A_x
    xn = _layernorm(x, axis=-1)
    return x + _A_ref(xn, A_wq, A_wk, A_wv, A_wo, A_beta) + _B_ref(xn, B_w_r, B_w_gate, B_w_up, B_w_down)
```

```python
import math

import jax
import jax.numpy as jnp
from jax import lax
import jax.experimental.pallas as pl
import jax.experimental.pallas.tpu as pltpu

S = 2048
D = 576
H = 32
DH = 18
NSEG = 4
L = S // NSEG
F = 4608
NG = 8
HS = 24
QT = L // 128

F32 = jnp.float32
BF16 = jnp.bfloat16
QSCALE = (DH ** -0.5) * math.log2(math.e)
SAFE_LOGIT_BOUND = 32.0

NT = (((1,), (1,)), ((), ()))
TN = (((0,), (0,)), ((), ()))

SEM_X, SEM_WQ, SEM_WK, SEM_WV, SEM_WO, SEM_WG, SEM_WU, SEM_WD, SEM_OUT = 0, 4, 5, 6, 7, 8, 9, 10, 11
N_SEMS = 15


def _bf(x):
    return x.astype(BF16).astype(F32)


def _phi(t):
    return jnp.where(t > 0, t + 1.0, jnp.exp(t))


def _window(tiles, g):
    c, b = divmod(72 * g, 128)
    if b + 72 <= 128:
        return tiles[c]
    lane = lax.broadcasted_iota(jnp.int32, tiles[c].shape, 1)
    return jnp.where(lane >= b, tiles[c], tiles[c + 1])


def _head_lane_mask(shape, g, hh):
    lane = lax.broadcasted_iota(jnp.int32, shape, len(shape) - 1)
    rel = (lane - 72 * g) & 127
    return (rel >= DH * hh) & (rel < DH * hh + DH)


def _kernel(x_hbm, wq_hbm, wk_hbm, wv_hbm, wo_hbm, beta_ref, wr_ref, wg_hbm, wu_hbm, wd_hbm,
            out_hbm,
            xs, xn, wq, wk, wv, wo, wtail, wvt, qwin, kwin, pqwin, pkwin, vt32, vts, mext, ot,
            outs, rbuf, bound, wg, wu, wd, sems):

    def x_copy(s):
        rows = pl.ds(pl.multiple_of(s * L, L), L)
        return pltpu.make_async_copy(x_hbm.at[rows, :], xs.at[rows, :], sems.at[SEM_X + s])

    def out_copy(s):
        rows = pl.ds(pl.multiple_of(s * L, L), L)
        return pltpu.make_async_copy(outs.at[rows, :], out_hbm.at[rows, :], sems.at[SEM_OUT + s])

    cp_wq = pltpu.make_async_copy(wq_hbm, wq, sems.at[SEM_WQ])
    cp_wk = pltpu.make_async_copy(wk_hbm, wk, sems.at[SEM_WK])
    cp_wv = pltpu.make_async_copy(wv_hbm, wv, sems.at[SEM_WV])
    cp_wo = pltpu.make_async_copy(wo_hbm, wo, sems.at[SEM_WO])
    cp_wg = pltpu.make_async_copy(wg_hbm, wg, sems.at[SEM_WG])
    cp_wu = pltpu.make_async_copy(wu_hbm, wu, sems.at[SEM_WU])
    cp_wd = pltpu.make_async_copy(wd_hbm, wd, sems.at[SEM_WD])

    x_copy(0).start()
    cp_wv.start()
    cp_wq.start()
    cp_wk.start()
    for s in range(1, NSEG):
        x_copy(s).start()

    cp_wv.wait()
    wvt[0:D, :] = wv[...].astype(F32).T.astype(BF16)
    row16 = lax.broadcasted_iota(jnp.int32, (16, D), 0)
    wvt[D:D + 16, :] = jnp.where(row16 == 0, wr_ref[...].astype(F32), 0.0).astype(BF16)
    cp_wq.wait()
    cp_wk.wait()
    wtail[...] = jnp.concatenate(
        [wq[:, 512:D].astype(F32), wk[:, 512:D].astype(F32)], axis=1).astype(BF16)
    cp_wo.start()
    cp_wg.start()
    cp_wu.start()
    cp_wd.start()
    mext[...] = jnp.zeros(mext.shape, F32)

    def phase_a(s, carry):
        x_copy(s).wait()
        rows = pl.ds(pl.multiple_of(s * L, L), L)
        x32 = xs[rows, :].astype(F32)
        mean = jnp.sum(x32, axis=-1, keepdims=True) / D
        cen = x32 - mean
        var = jnp.sum(cen * cen, axis=-1, keepdims=True) / D
        den = _bf(jnp.sqrt(_bf(_bf(var) + _bf(jnp.float32(1e-5)))))
        xnb = (_bf(x32 - _bf(mean)) * (1.0 / den)).astype(BF16)
        xn[rows, :] = xnb

        qa = jnp.dot(xnb, wq[:, 0:512], preferred_element_type=F32)
        ka = jnp.dot(xnb, wk[:, 0:512], preferred_element_type=F32)
        tl = jnp.dot(xnb, wtail[...], preferred_element_type=F32)
        vt = lax.dot_general(wvt[...], xnb, NT, preferred_element_type=F32)

        qt = [qa[:, 128 * c:128 * (c + 1)] for c in range(4)] + [tl]
        kt = [ka[:, 128 * c:128 * (c + 1)] for c in range(4)] + [pltpu.roll(tl, 64, 1)]
        qs = [t * QSCALE for t in qt]
        pq = [_phi(t) for t in qt]
        pk = [_phi(t) for t in kt]
        qmax = jnp.zeros((8, 128), F32)
        kmax = jnp.zeros((8, 128), F32)
        for c in range(5):
            qmax = jnp.maximum(qmax, jnp.max(jnp.abs(qs[c]).reshape(L // 8, 8, 128), axis=0))
            kmax = jnp.maximum(kmax, jnp.max(jnp.abs(kt[c]).reshape(L // 8, 8, 128), axis=0))
        bound[s] = DH * jnp.max(qmax) * jnp.max(kmax)
        for g in range(NG):
            qwin[s, g] = _window(qs, g).astype(BF16)
            kwin[s, g] = _window(kt, g).astype(BF16)
            pqwin[s, g] = _window(pq, g).astype(BF16)
            pkwin[s, g] = _window(pk, g).astype(BF16)

        for j in range(QT):
            vt32[j] = vt[:, 128 * j:128 * (j + 1)]
            rbuf[pl.ds(s * QT + j, 1), :] = _bf(vt[D:D + 1, 128 * j:128 * (j + 1)])
        hrow = lax.broadcasted_iota(jnp.int32, (HS, 128), 0)
        for h in range(H):
            g, hh = divmod(h, 4)
            for j in range(QT):
                v = vt32[j, DH * h:DH * h + HS, :]
                v = jnp.where(hrow < DH, v, jnp.where(hrow == DH, 1.0, 0.0))
                vts[s, g, HS * hh:HS * (hh + 1), 128 * j:128 * (j + 1)] = v
        return carry

    lax.fori_loop(0, NSEG, phase_a, 0)

    r = rbuf[...]
    tok = (lax.broadcasted_iota(jnp.int32, r.shape, 0) * 128
           + lax.broadcasted_iota(jnp.int32, r.shape, 1))
    r1 = jnp.max(r)
    i1 = jnp.min(jnp.where(r == r1, tok, S))
    rm = jnp.where(tok == i1, -jnp.inf, r)
    r2 = jnp.max(rm)
    i2 = jnp.min(jnp.where((rm == r2) & (tok != i1), tok, S))
    i1 = jnp.minimum(i1, S - 1)
    i2 = jnp.minimum(i2, S - 1)

    def pick_row(ref, idx):
        base = pl.multiple_of((idx // 16) * 16, 16)
        blk = ref[pl.ds(base, 16), :].astype(F32)
        rid = lax.broadcasted_iota(jnp.int32, blk.shape, 0)
        return jnp.sum(jnp.where(rid == idx - base, blk, 0.0), axis=0, keepdims=True)

    row8 = lax.broadcasted_iota(jnp.int32, (8, D), 0)
    xsel = jnp.where(row8 == 0, pick_row(xn, i1), jnp.where(row8 == 1, pick_row(xn, i2), 0.0))
    cp_wg.wait()
    cp_wu.wait()
    gate = _bf(jnp.dot(xsel, wg[...], preferred_element_type=F32))
    up = _bf(jnp.dot(xsel, wu[...], preferred_element_type=F32))
    hid = _bf(_bf(gate * jax.nn.sigmoid(gate)) * up)
    cp_wd.wait()
    y = _bf(jnp.dot(hid, wd[...], preferred_element_type=F32))
    rsel = jnp.where(row8 == 0, r1, r2)
    y = _bf(y * _bf(jax.nn.sigmoid(rsel)))
    cp_wo.wait()

    krow = lax.broadcasted_iota(jnp.int32, (128, 128), 0)
    kcol = lax.broadcasted_iota(jnp.int32, (128, 128), 1)
    causal = krow <= kcol

    def gate_of(h):
        b = jnp.full((8, 128), beta_ref[h], F32)
        gt = _bf(jax.nn.sigmoid(b))
        return gt[0:1], _bf(1.0 - gt)[0:1]

    def stage_fns(s, g, ret, use_max):
        def qk(i):
            q = qwin[s, g, 128 * i:128 * (i + 1), :]
            qm = jnp.concatenate(
                [jnp.where(_head_lane_mask(q.shape, g, hh), q, jnp.zeros_like(q)) for hh in range(4)],
                axis=0)
            nk = 128 * (i + 1)
            st = lax.dot_general(kwin[s, g, 0:nk, :], qm, NT, preferred_element_type=F32)
            ps = []
            for hh in range(4):
                sc = st[:, 128 * hh:128 * (hh + 1)]
                diag = jnp.where(causal, sc[nk - 128:], -1e30)
                sc = jnp.concatenate([sc[:nk - 128], diag], axis=0) if i > 0 else diag
                if use_max:
                    sc = sc - jnp.max(sc, axis=0, keepdims=True)
                ps.append(jnp.exp2(sc).astype(BF16))
            return ps

        def pv(i, ps):
            nk = 128 * (i + 1)
            for hh in range(4):
                h = 4 * g + hh
                v = vts[s, g, HS * hh:HS * (hh + 1), 0:nk]
                o = jnp.dot(v, ps[hh], preferred_element_type=F32)
                mem = ret[HS * hh:HS * (hh + 1), 128 * i:128 * (i + 1)]
                gt, gc = gate_of(h)
                w_mem = gt / (mem[DH:DH + 1] + 1e-6)
                w_dot = gc / o[DH:DH + 1]
                ot[i, pl.ds(DH * h, HS), :] = mem * w_mem + o * w_dot
        return qk, pv

    def memory(s, g):
        ret = lax.dot_general(mext[g], pqwin[s, g], NT, preferred_element_type=F32)
        upd = jnp.dot(vts[s, g], pkwin[s, g], preferred_element_type=F32)
        keep = jnp.concatenate(
            [_head_lane_mask((HS, 128), g, hh).astype(F32) for hh in range(4)], axis=0) > 0.5
        mext[g] = mext[g] + jnp.where(keep, upd, 0.0)
        return ret

    def attention_fast(s):
        prev = None
        for g in range(NG):
            qk, pv = stage_fns(s, g, memory(s, g), False)
            for i in range(QT):
                p = qk(i)
                if prev is not None:
                    prev[0](prev[1], prev[2])
                prev = (pv, i, p)
        prev[0](prev[1], prev[2])

    def attention_safe(s):
        def body(g, c):
            qk, pv = stage_fns(s, g, memory(s, g), True)
            for i in range(QT):
                pv(i, qk(i))
            return c
        lax.fori_loop(0, NG, body, 0)

    def phase_b(s, carry):
        rows = pl.ds(pl.multiple_of(s * L, L), L)
        lax.cond(bound[s] <= SAFE_LOGIT_BOUND, attention_fast, attention_safe, s)
        otb = jnp.concatenate([ot[i, 0:D, :].astype(BF16) for i in range(QT)], axis=1)
        att = lax.dot_general(otb, wo[...], TN, preferred_element_type=F32)
        res = xs[rows, :].astype(F32) + _bf(att) + xn[rows, :].astype(F32)
        outs[rows, :] = res.astype(BF16)
        for k, idx in enumerate((i1, i2)):
            @pl.when((idx >= s * L) & (idx < (s + 1) * L))
            def _():
                base = pl.multiple_of((idx // 16) * 16, 16)
                blk = outs[pl.ds(base, 16), :].astype(F32)
                rid = lax.broadcasted_iota(jnp.int32, blk.shape, 0)
                outs[pl.ds(base, 16), :] = (
                    blk + jnp.where(rid == idx - base, y[k:k + 1], 0.0)).astype(BF16)
        out_copy(s).start()
        return carry

    lax.fori_loop(0, NSEG, phase_b, 0)
    for s in range(NSEG):
        out_copy(s).wait()


@jax.jit
def pallas_parallel_sum__memory_aug_infini_attn__moe_arch_mod__prompt_kernel(
    A_x: jax.Array,
    A_wq: jax.Array,
    A_wk: jax.Array,
    A_wv: jax.Array,
    A_wo: jax.Array,
    A_beta: jax.Array,
    B_x: jax.Array,
    B_w_r: jax.Array,
    B_w_gate: jax.Array,
    B_w_up: jax.Array,
    B_w_down: jax.Array,
):
    del B_x
    x = A_x.reshape(S, D)
    beta = A_beta.astype(F32)
    wr = B_w_r.reshape(1, D)
    hbm = pl.BlockSpec(memory_space=pl.ANY)
    out = pl.pallas_call(
        _kernel,
        out_shape=jax.ShapeDtypeStruct((S, D), BF16),
        in_specs=[hbm, hbm, hbm, hbm, hbm,
                  pl.BlockSpec(memory_space=pltpu.SMEM),
                  pl.BlockSpec(memory_space=pltpu.VMEM),
                  hbm, hbm, hbm],
        out_specs=hbm,
        scratch_shapes=[
            pltpu.VMEM((S, D), BF16),
            pltpu.VMEM((S, D), BF16),
            pltpu.VMEM((D, D), BF16),
            pltpu.VMEM((D, D), BF16),
            pltpu.VMEM((D, D), BF16),
            pltpu.VMEM((D, D), BF16),
            pltpu.VMEM((D, 128), BF16),
            pltpu.VMEM((D + 16, D), BF16),
            pltpu.VMEM((NSEG, NG, L, 128), BF16),
            pltpu.VMEM((NSEG, NG, L, 128), BF16),
            pltpu.VMEM((NSEG, NG, L, 128), BF16),
            pltpu.VMEM((NSEG, NG, L, 128), BF16),
            pltpu.VMEM((QT, D + 16, 128), F32),
            pltpu.VMEM((NSEG, NG, 4 * HS, L), F32),
            pltpu.VMEM((NG, 4 * HS, 128), F32),
            pltpu.VMEM((QT, D + 24, 128), F32),
            pltpu.VMEM((S, D), BF16),
            pltpu.VMEM((NSEG * QT, 128), F32),
            pltpu.SMEM((NSEG,), F32),
            pltpu.VMEM((D, F), BF16),
            pltpu.VMEM((D, F), BF16),
            pltpu.VMEM((F, D), BF16),
            pltpu.SemaphoreType.DMA((N_SEMS,)),
        ],
        compiler_params=pltpu.CompilerParams(vmem_limit_bytes=110 * 1024 * 1024),
    )(x, A_wq, A_wk, A_wv, A_wo, beta, wr, B_w_gate, B_w_up, B_w_down)
    return out.reshape(1, S, D)
```

```python
import math

import jax
import jax.numpy as jnp
from jax import lax
import jax.experimental.pallas as pl
import jax.experimental.pallas.tpu as pltpu

S = 2048
D = 576
H = 32
DH = 18
NSEG = 4
L = S // NSEG
F = 4608
NG = 8
GD = 4 * DH
HS = 24
QT = L // 128
WROWS = 3 * D + 16

F32 = jnp.float32
BF16 = jnp.bfloat16
QSCALE = (DH ** -0.5) * math.log2(math.e)
SAFE_LOGIT_BOUND = 32.0

NT = (((1,), (1,)), ((), ()))

SEM_X, SEM_WQ, SEM_WK, SEM_WV, SEM_WO, SEM_WG, SEM_WU, SEM_WD, SEM_OUT = 0, 4, 5, 6, 7, 8, 9, 10, 11
N_SEMS = 15


def _bf(x):
    return x.astype(BF16).astype(F32)


def _phi(t):
    return jnp.where(t > 0, t + 1.0, jnp.exp(t))


def _absmax(t):
    return jnp.max(jnp.abs(t).reshape(t.shape[0] // 8, 8, t.shape[1]), axis=0)


def _kernel(x_hbm, wq_hbm, wk_hbm, wv_hbm, wo_hbm, beta_ref, wr_ref, wg_hbm, wu_hbm, wd_hbm,
            out_hbm,
            xs, xn, wq, wk, wv, wo, wt, wot, qts, kwin, pqt, pkwin, vts, mext, ot,
            outs, rbuf, bound, wg, wu, wd, sems):

    def x_copy(s):
        cols = pl.ds(pl.multiple_of(s * L, L), L)
        return pltpu.make_async_copy(x_hbm.at[:, cols], xs.at[:, cols], sems.at[SEM_X + s])

    def out_copy(s):
        cols = pl.ds(pl.multiple_of(s * L, L), L)
        return pltpu.make_async_copy(outs.at[:, cols], out_hbm.at[:, cols], sems.at[SEM_OUT + s])

    cp_wq = pltpu.make_async_copy(wq_hbm, wq, sems.at[SEM_WQ])
    cp_wk = pltpu.make_async_copy(wk_hbm, wk, sems.at[SEM_WK])
    cp_wv = pltpu.make_async_copy(wv_hbm, wv, sems.at[SEM_WV])
    cp_wo = pltpu.make_async_copy(wo_hbm, wo, sems.at[SEM_WO])
    cp_wg = pltpu.make_async_copy(wg_hbm, wg, sems.at[SEM_WG])
    cp_wu = pltpu.make_async_copy(wu_hbm, wu, sems.at[SEM_WU])
    cp_wd = pltpu.make_async_copy(wd_hbm, wd, sems.at[SEM_WD])

    cp_wq.start()
    cp_wk.start()
    cp_wv.start()
    for s in range(NSEG):
        x_copy(s).start()

    cp_wq.wait()
    wt[0:D, :] = wq[...].astype(F32).T.astype(BF16)
    cp_wk.wait()
    wt[D:2 * D, :] = wk[...].astype(F32).T.astype(BF16)
    cp_wv.wait()
    wt[2 * D:3 * D, :] = wv[...].astype(F32).T.astype(BF16)
    row16 = lax.broadcasted_iota(jnp.int32, (16, D), 0)
    wt[3 * D:WROWS, :] = jnp.where(row16 == 0, wr_ref[...].astype(F32), 0.0).astype(BF16)
    cp_wo.start()
    cp_wg.start()
    cp_wu.start()
    cp_wd.start()
    mext[...] = jnp.zeros(mext.shape, F32)

    def phase_a(s, carry):
        x_copy(s).wait()
        cols = pl.ds(pl.multiple_of(s * L, L), L)
        x32 = xs[:, cols].astype(F32)
        mean = jnp.sum(x32, axis=0, keepdims=True) / D
        cen = x32 - mean
        var = jnp.sum(cen * cen, axis=0, keepdims=True) / D
        den = _bf(jnp.sqrt(_bf(_bf(var) + _bf(jnp.float32(1e-5)))))
        xnb = (_bf(x32 - _bf(mean)) * (1.0 / den)).astype(BF16)
        xn[:, cols] = xnb

        big = jnp.dot(wt[...], xnb, preferred_element_type=F32)
        qt_ = big[0:D]
        kt_ = big[D:2 * D]
        qsc = qt_ * QSCALE
        qts[s] = qsc
        bound[s] = DH * jnp.max(_absmax(qsc)) * jnp.max(_absmax(kt_))
        for g in range(NG):
            pqt[s, g] = _phi(big[GD * g:GD * g + 128]).astype(BF16)
            kw = big[D + GD * g:D + GD * g + 128].T
            kwin[s, g] = kw.astype(BF16)
            pkwin[s, g] = _phi(kw).astype(BF16)
        for j in range(QT):
            rbuf[pl.ds(s * QT + j, 1), :] = _bf(big[3 * D:3 * D + 1, 128 * j:128 * (j + 1)])
        hrow = lax.broadcasted_iota(jnp.int32, (HS, L), 0)
        for h in range(H):
            g, hh = divmod(h, 4)
            v = big[2 * D + DH * h:2 * D + DH * h + HS]
            vts[s, g, HS * hh:HS * (hh + 1), :] = jnp.where(
                hrow < DH, v, jnp.where(hrow == DH, 1.0, 0.0))
        return carry

    lax.fori_loop(0, NSEG, phase_a, 0)

    cp_wo.wait()
    wot[...] = wo[...].astype(F32).T.astype(BF16)

    r = rbuf[...]
    tok = (lax.broadcasted_iota(jnp.int32, r.shape, 0) * 128
           + lax.broadcasted_iota(jnp.int32, r.shape, 1))
    r1 = jnp.max(r)
    i1 = jnp.min(jnp.where(r == r1, tok, S))
    rm = jnp.where(tok == i1, -jnp.inf, r)
    r2 = jnp.max(rm)
    i2 = jnp.min(jnp.where((rm == r2) & (tok != i1), tok, S))
    i1 = jnp.minimum(i1, S - 1)
    i2 = jnp.minimum(i2, S - 1)

    def tile_of(idx):
        return pl.ds(pl.multiple_of((idx // 128) * 128, 128), 128)

    row8 = lax.broadcasted_iota(jnp.int32, (8, 128), 0)
    lane8 = lax.broadcasted_iota(jnp.int32, (8, 128), 1)
    hot1 = jnp.where((row8 == 0) & (lane8 == i1 % 128), 1.0, 0.0)
    hot2 = jnp.where((row8 == 1) & (lane8 == i2 % 128), 1.0, 0.0)
    xsel = (lax.dot_general(hot1, xn[:, tile_of(i1)], NT, preferred_element_type=F32)
            + lax.dot_general(hot2, xn[:, tile_of(i2)], NT, preferred_element_type=F32))
    cp_wg.wait()
    cp_wu.wait()
    gate = _bf(jnp.dot(xsel, wg[...], preferred_element_type=F32))
    up = _bf(jnp.dot(xsel, wu[...], preferred_element_type=F32))
    hid = _bf(_bf(gate * jax.nn.sigmoid(gate)) * up)
    cp_wd.wait()
    y = _bf(lax.dot_general(hid, wd[...], NT, preferred_element_type=F32))
    rowd = lax.broadcasted_iota(jnp.int32, (8, D), 0)
    y = _bf(y * _bf(jax.nn.sigmoid(jnp.where(rowd == 0, r1, r2))))
    yt = jnp.concatenate([y, jnp.zeros((120, D), F32)], axis=0).T

    krow = lax.broadcasted_iota(jnp.int32, (128, 128), 0)
    kcol = lax.broadcasted_iota(jnp.int32, (128, 128), 1)
    causal = krow <= kcol

    def gate_of(h):
        b = jnp.full((8, 128), beta_ref[h], F32)
        gt = _bf(jax.nn.sigmoid(b))
        return gt[0:1], _bf(1.0 - gt)[0:1]

    def stage_fns(s, g, g_rows, ret, use_max):
        def qk(i):
            q = qts[s, g_rows, 128 * i:128 * (i + 1)]
            tiles = []
            for hh in range(4):
                lo = (DH * hh) // 8 * 8
                hi = -(-(DH * hh + DH) // 8) * 8
                row = lo + lax.broadcasted_iota(jnp.int32, (hi - lo, 128), 0)
                part = jnp.where((row >= DH * hh) & (row < DH * hh + DH), q[lo:hi], 0.0)
                pieces = ([jnp.zeros((lo, 128), F32)] if lo else []) + [part, jnp.zeros((128 - hi, 128), F32)]
                tiles.append(jnp.concatenate(pieces, axis=0).astype(BF16))
            qm = jnp.concatenate(tiles, axis=1)
            nk = 128 * (i + 1)
            st = jnp.dot(kwin[s, g, 0:nk, :], qm, preferred_element_type=F32)
            ps = []
            for hh in range(4):
                sc = st[:, 128 * hh:128 * (hh + 1)]
                diag = jnp.where(causal, sc[nk - 128:], -1e30)
                sc = jnp.concatenate([sc[:nk - 128], diag], axis=0) if i > 0 else diag
                if use_max:
                    sc = sc - jnp.max(sc, axis=0, keepdims=True)
                ps.append(jnp.exp2(sc).astype(BF16))
            return ps

        def pv(i, ps):
            nk = 128 * (i + 1)
            for hh in range(4):
                h = 4 * g + hh
                v = vts[s, g, HS * hh:HS * (hh + 1), 0:nk]
                o = jnp.dot(v, ps[hh], preferred_element_type=F32)
                mem = ret[HS * hh:HS * (hh + 1), 128 * i:128 * (i + 1)]
                gt, gc = gate_of(h)
                w_mem = gt / (mem[DH:DH + 1] + 1e-6)
                w_dot = gc / o[DH:DH + 1]
                ot[i, pl.ds(DH * h, HS), :] = mem * w_mem + o * w_dot
        return qk, pv

    def memory(s, g):
        ret = jnp.dot(mext[g], pqt[s, g], preferred_element_type=F32)
        upd = jnp.dot(vts[s, g], pkwin[s, g], preferred_element_type=F32)
        row = lax.broadcasted_iota(jnp.int32, (4 * HS, 128), 0)
        lane = lax.broadcasted_iota(jnp.int32, (4 * HS, 128), 1)
        lo = (row // HS) * DH
        mext[g] = mext[g] + jnp.where((lane >= lo) & (lane < lo + DH), upd, 0.0)
        return ret

    def attention_fast(s):
        prev = None
        for g in range(NG):
            qk, pv = stage_fns(s, g, slice(GD * g, GD * (g + 1)), memory(s, g), False)
            for i in range(QT):
                p = qk(i)
                if prev is not None:
                    prev[0](prev[1], prev[2])
                prev = (pv, i, p)
        prev[0](prev[1], prev[2])

    def attention_safe(s):
        def body(g, c):
            g_rows = pl.ds(pl.multiple_of(GD * g, 8), GD)
            qk, pv = stage_fns(s, g, g_rows, memory(s, g), True)
            for i in range(QT):
                pv(i, qk(i))
            return c
        lax.fori_loop(0, NG, body, 0)

    def phase_b(s, carry):
        cols = pl.ds(pl.multiple_of(s * L, L), L)
        lax.cond(bound[s] <= SAFE_LOGIT_BOUND, attention_fast, attention_safe, s)
        otb = jnp.concatenate([ot[i, 0:D, :].astype(BF16) for i in range(QT)], axis=1)
        att = jnp.dot(wot[...], otb, preferred_element_type=F32)
        res = xs[:, cols].astype(F32) + _bf(att) + xn[:, cols].astype(F32)
        outs[:, cols] = res.astype(BF16)
        lane = lax.broadcasted_iota(jnp.int32, (D, 128), 1)
        for k, idx in enumerate((i1, i2)):
            @pl.when((idx >= s * L) & (idx < (s + 1) * L))
            def _():
                blk = outs[:, tile_of(idx)].astype(F32)
                col = jnp.sum(jnp.where(lane == k, yt, 0.0), axis=1, keepdims=True)
                outs[:, tile_of(idx)] = (blk + jnp.where(lane == idx % 128, col, 0.0)).astype(BF16)
        out_copy(s).start()
        return carry

    lax.fori_loop(0, NSEG, phase_b, 0)
    for s in range(NSEG):
        out_copy(s).wait()


@jax.jit
def pallas_parallel_sum__memory_aug_infini_attn__moe_arch_mod__prompt_kernel(
    A_x: jax.Array,
    A_wq: jax.Array,
    A_wk: jax.Array,
    A_wv: jax.Array,
    A_wo: jax.Array,
    A_beta: jax.Array,
    B_x: jax.Array,
    B_w_r: jax.Array,
    B_w_gate: jax.Array,
    B_w_up: jax.Array,
    B_w_down: jax.Array,
):
    del B_x
    xt = A_x.reshape(S, D).T
    beta = A_beta.astype(F32)
    wr = B_w_r.reshape(1, D)
    wdt = B_w_down.T
    hbm = pl.BlockSpec(memory_space=pltpu.HBM)
    out = pl.pallas_call(
        _kernel,
        out_shape=jax.ShapeDtypeStruct((D, S), BF16),
        in_specs=[hbm, hbm, hbm, hbm, hbm,
                  pl.BlockSpec(memory_space=pltpu.SMEM),
                  pl.BlockSpec(memory_space=pltpu.VMEM),
                  hbm, hbm, hbm],
        out_specs=hbm,
        scratch_shapes=[
            pltpu.VMEM((D, S), BF16),
            pltpu.VMEM((D, S), BF16),
            pltpu.VMEM((D, D), BF16),
            pltpu.VMEM((D, D), BF16),
            pltpu.VMEM((D, D), BF16),
            pltpu.VMEM((D, D), BF16),
            pltpu.VMEM((WROWS, D), BF16),
            pltpu.VMEM((D, D), BF16),
            pltpu.VMEM((NSEG, D, L), F32),
            pltpu.VMEM((NSEG, NG, L, 128), BF16),
            pltpu.VMEM((NSEG, NG, 128, L), BF16),
            pltpu.VMEM((NSEG, NG, L, 128), BF16),
            pltpu.VMEM((NSEG, NG, 4 * HS, L), F32),
            pltpu.VMEM((NG, 4 * HS, 128), F32),
            pltpu.VMEM((QT, D + 24, 128), F32),
            pltpu.VMEM((D, S), BF16),
            pltpu.VMEM((NSEG * QT, 128), F32),
            pltpu.SMEM((NSEG,), F32),
            pltpu.VMEM((D, F), BF16),
            pltpu.VMEM((D, F), BF16),
            pltpu.VMEM((D, F), BF16),
            pltpu.SemaphoreType.DMA((N_SEMS,)),
        ],
        compiler_params=pltpu.CompilerParams(vmem_limit_bytes=110 * 1024 * 1024),
    )(xt, A_wq, A_wk, A_wv, A_wo, beta, wr, B_w_gate, B_w_up, wdt)
    return out.T.reshape(1, S, D)
```

```python
import math

import jax
import jax.numpy as jnp
from jax import lax
import jax.experimental.pallas as pl
import jax.experimental.pallas.tpu as pltpu

S = 2048
D = 576
H = 32
DH = 18
NSEG = 4
L = S // NSEG
F = 4608
NG = 8
GD = 4 * DH
HS = 24
QT = L // 128
WROWS = 3 * D + 16
FU = F // 128 // NSEG
FC = F // NSEG
KP = 80

F32 = jnp.float32
BF16 = jnp.bfloat16
QSCALE = (DH ** -0.5) * math.log2(math.e)
SAFE_LOGIT_BOUND = 32.0

NT = (((1,), (1,)), ((), ()))

(SEM_X, SEM_WQ, SEM_WK, SEM_WV, SEM_WO, SEM_BETA, SEM_WR,
 SEM_OUT, SEM_FIX, SEM_LAST, SEM_FFN) = 0, 4, 5, 6, 7, 8, 9, 10, 13, 15, 19
N_SEMS = SEM_FFN + 3 * NSEG


def _bf(x):
    return x.astype(BF16).astype(F32)


def _phi(t):
    return jnp.where(t > 0, t + 1.0, jnp.exp(t))


def _absmax(t):
    return jnp.max(jnp.abs(t).reshape(t.shape[0] // 8, 8, t.shape[1]), axis=0)


def _rows_padded(a, start, rows):
    stop = min(start + rows, a.shape[0])
    part = a[start:stop]
    if stop - start < rows:
        part = jnp.concatenate([part, jnp.zeros((rows - (stop - start), a.shape[1]), a.dtype)], axis=0)
    return part


def _kernel(x_hbm, wq_hbm, wk_hbm, wv_hbm, wo_hbm, beta_hbm, wr_hbm, wg_hbm, wu_hbm, wd_hbm,
            out_hbm,
            xs, xn, wq, wk, wv, wo, beta, wr, wt, wot, gtab, qts, kwin, pqt, pkwin, vts, mext, ot,
            outs, rbuf, bound, yacc, xsel_ref, wg, wu, wd, sems):

    def seg_cols(s):
        if isinstance(s, int):
            return slice(s * L, (s + 1) * L)
        return pl.ds(pl.multiple_of(s * L, L), L)

    def x_copy(s):
        return pltpu.make_async_copy(x_hbm.at[:, seg_cols(s)], xs.at[:, seg_cols(s)], sems.at[SEM_X + s])

    def out_copy(s):
        return pltpu.make_async_copy(outs.at[:, seg_cols(s)], out_hbm.at[:, seg_cols(s)],
                                     sems.at[SEM_OUT + s])

    cp_wq = pltpu.make_async_copy(wq_hbm, wq, sems.at[SEM_WQ])
    cp_wk = pltpu.make_async_copy(wk_hbm, wk, sems.at[SEM_WK])
    cp_wv = pltpu.make_async_copy(wv_hbm, wv, sems.at[SEM_WV])
    cp_wo = pltpu.make_async_copy(wo_hbm, wo, sems.at[SEM_WO])

    def ffn_copies(s):
        if isinstance(s, int):
            cols = slice(s * FC, (s + 1) * FC)
        else:
            cols = pl.ds(pl.multiple_of(s * FC, 128), FC)
        return [pltpu.make_async_copy(src.at[:, cols], dst.at[:, cols], sems.at[SEM_FFN + 3 * s + k])
                for k, (src, dst) in enumerate(((wg_hbm, wg), (wu_hbm, wu), (wd_hbm, wd)))]

    cp_beta = pltpu.make_async_copy(beta_hbm, beta, sems.at[SEM_BETA])
    cp_wr = pltpu.make_async_copy(wr_hbm, wr, sems.at[SEM_WR])

    def transposed(w_ref):
        return w_ref[...].astype(F32).T.astype(BF16)

    def layernorm(s):
        x32 = xs[:, seg_cols(s)].astype(F32)
        mean = jnp.sum(x32, axis=0, keepdims=True) / D
        cen = x32 - mean
        var = jnp.sum(cen * cen, axis=0, keepdims=True) / D
        den = _bf(jnp.sqrt(_bf(_bf(var) + _bf(jnp.float32(1e-5)))))
        xn[:, seg_cols(s)] = (_bf(x32 - _bf(mean)) * (1.0 / den)).astype(BF16)

    def proj_q(s, g0, g1):
        q = jnp.dot(wt[GD * g0:GD * g1, :], xn[:, seg_cols(s)], preferred_element_type=F32)
        qsc = q * QSCALE
        qts[s, GD * g0:GD * g1, :] = qsc
        pq = _phi(q)
        pad = jnp.zeros((KP - GD, L), F32)
        for g in range(g0, g1):
            win = jnp.concatenate([pq[GD * (g - g0):GD * (g - g0 + 1)], pad], axis=0)
            pqt[s, g] = win.astype(BF16)
        return jnp.max(_absmax(qsc))

    def proj_k(s):
        k = jnp.dot(wt[D:2 * D, :], xn[:, seg_cols(s)], preferred_element_type=F32)
        for g in range(NG):
            kw = _rows_padded(k, GD * g, 128).T
            kwin[s, g] = kw.astype(BF16)
            pkwin[s, g] = _phi(kw).astype(BF16)
        return jnp.max(_absmax(k))

    def proj_v(s):
        v = jnp.dot(wt[2 * D:WROWS, :], xn[:, seg_cols(s)], preferred_element_type=F32)
        for j in range(QT):
            rbuf[s * QT + j:s * QT + j + 1, :] = _bf(v[D:D + 1, 128 * j:128 * (j + 1)])
        hrow = lax.broadcasted_iota(jnp.int32, (HS, L), 0)
        fill = jnp.where(hrow == DH, 1.0, 0.0)
        for h in range(H):
            g, hh = divmod(h, 4)
            vts[s, g, HS * hh:HS * (hh + 1), :] = jnp.where(
                hrow < DH, v[DH * h:DH * h + HS], fill)

    def tile_of(idx):
        return pl.ds(pl.multiple_of((idx // 128) * 128, 128), 128)

    def router():
        r = rbuf[...]
        tok = (lax.broadcasted_iota(jnp.int32, r.shape, 0) * 128
               + lax.broadcasted_iota(jnp.int32, r.shape, 1))
        r1 = jnp.max(r)
        i1 = jnp.min(jnp.where(r == r1, tok, S))
        rm = jnp.where(tok == i1, -jnp.inf, r)
        r2 = jnp.max(rm)
        i2 = jnp.min(jnp.where((rm == r2) & (tok != i1), tok, S))
        i1 = jnp.minimum(i1, S - 1)
        i2 = jnp.minimum(i2, S - 1)
        row8 = lax.broadcasted_iota(jnp.int32, (8, 128), 0)
        lane8 = lax.broadcasted_iota(jnp.int32, (8, 128), 1)
        hot1 = jnp.where((row8 == 0) & (lane8 == i1 % 128), 1.0, 0.0)
        hot2 = jnp.where((row8 == 1) & (lane8 == i2 % 128), 1.0, 0.0)
        return r1, r2, i1, i2, hot1, hot2

    x_copy(0).start()
    cp_wq.start()
    cp_wr.start()
    cp_beta.start()
    mext[...] = jnp.zeros(mext.shape, F32)
    yacc[...] = jnp.zeros(yacc.shape, F32)
    x_copy(0).wait()
    cp_wv.start()
    cp_wk.start()
    layernorm(0)
    cp_wq.wait()
    for s in range(1, NSEG):
        x_copy(s).start()
    cp_wo.start()
    wt[0:D, :] = transposed(wq)
    qm = proj_q(0, 0, NG // 2)
    cp_wv.wait()
    cp_wk.wait()
    cp_wr.wait()
    wt[2 * D:3 * D, :] = transposed(wv)
    row16 = lax.broadcasted_iota(jnp.int32, (16, D), 0)
    wt[3 * D:WROWS, :] = jnp.where(
        row16 == 0, wr[...].astype(F32).reshape(1, D), 0.0).astype(BF16)
    qm = jnp.maximum(qm, proj_q(0, NG // 2, NG))
    wt[D:2 * D, :] = transposed(wk)
    proj_v(0)
    for s in range(1, NSEG):
        x_copy(s).wait()
    cp_wo.wait()
    for s in range(NSEG):
        for cp in ffn_copies(s):
            cp.start()
    cp_beta.wait()
    bound[0] = DH * qm * proj_k(0)
    layernorm(1)
    for s in range(1, NSEG):
        if s == NSEG - 1:
            proj_v(s)
            r1, r2, i1, i2, hot1, hot2 = router()
            km = proj_k(s)
            bound[s] = DH * km * proj_q(s, 0, NG)
            xsel_ref[...] = (
                lax.dot_general(hot1, xn[:, tile_of(i1)], NT, preferred_element_type=F32)
                + lax.dot_general(hot2, xn[:, tile_of(i2)], NT, preferred_element_type=F32))
            continue
        qm = proj_q(s, 0, NG)
        layernorm(s + 1)
        if s == 1:
            wot[...] = transposed(wo)
            b = beta[...].astype(F32).reshape(1, H)
            bt = jnp.broadcast_to(
                jnp.concatenate([b, jnp.zeros((1, 128 - H), F32)], axis=1), (128, 128)).T
            gt_all = _bf(jax.nn.sigmoid(bt[0:H]))
            gtab[0] = gt_all
            gtab[1] = _bf(1.0 - gt_all)
        bound[s] = DH * qm * proj_k(s)
        proj_v(s)

    krow = lax.broadcasted_iota(jnp.int32, (128, 128), 0)
    kcol = lax.broadcasted_iota(jnp.int32, (128, 128), 1)
    causal = krow <= kcol

    def ffn_up(s, u):
        cols = pl.ds(pl.multiple_of((s * FU + u) * 128, 128), 128)
        w2 = jnp.concatenate([wg[:, cols], wu[:, cols]], axis=1)
        gu = jnp.dot(xsel_ref[...], w2, preferred_element_type=F32)
        gate = _bf(gu[:, 0:128])
        return _bf(_bf(gate * jax.nn.sigmoid(gate)) * _bf(gu[:, 128:256]))

    def ffn_down(s, u, hid):
        cols = pl.ds(pl.multiple_of((s * FU + u) * 128, 128), 128)
        yacc[...] += lax.dot_general(hid, wd[:, cols], NT, preferred_element_type=F32)

    def stage_fns(s, g, g_rows, ret, use_max):
        def qk(i):
            q = qts[s, g_rows, 128 * i:128 * (i + 1)]
            tiles = []
            for hh in range(4):
                lo = (DH * hh) // 8 * 8
                hi = -(-(DH * hh + DH) // 8) * 8
                row = lo + lax.broadcasted_iota(jnp.int32, (hi - lo, 128), 0)
                part = jnp.where((row >= DH * hh) & (row < DH * hh + DH), q[lo:hi], 0.0)
                pieces = ([jnp.zeros((lo, 128), F32)] if lo else []) + [part, jnp.zeros((128 - hi, 128), F32)]
                tiles.append(jnp.concatenate(pieces, axis=0).astype(BF16))
            qm = jnp.concatenate(tiles, axis=1)
            nk = 128 * (i + 1)
            st = jnp.dot(kwin[s, g, 0:nk, :], qm, preferred_element_type=F32)
            ps = []
            for hh in range(4):
                sc = st[:, 128 * hh:128 * (hh + 1)]
                diag = jnp.where(causal, sc[nk - 128:], -1e30)
                sc = jnp.concatenate([sc[:nk - 128], diag], axis=0) if i > 0 else diag
                if use_max:
                    sc = sc - jnp.max(sc, axis=0, keepdims=True)
                ps.append(jnp.exp2(sc).astype(BF16))
            return ps

        def pv(i, ps):
            nk = 128 * (i + 1)
            for hh in range(4):
                h = 4 * g + hh
                v = vts[s, g, HS * hh:HS * (hh + 1), 0:nk]
                o = jnp.dot(v, ps[hh], preferred_element_type=F32)
                mem = ret[HS * hh:HS * (hh + 1), 128 * i:128 * (i + 1)]
                w_mem = gtab[0, pl.ds(h, 1), :] / (mem[DH:DH + 1] + 1e-6)
                w_dot = gtab[1, pl.ds(h, 1), :] / o[DH:DH + 1]
                ot[i, pl.ds(DH * h, HS), :] = mem * w_mem + o * w_dot
        return qk, pv

    def memory(s, g):
        ret = jnp.dot(mext[g][:, 0:KP], pqt[s, g], preferred_element_type=F32)
        upd = jnp.dot(vts[s, g], pkwin[s, g], preferred_element_type=F32)
        row = lax.broadcasted_iota(jnp.int32, (4 * HS, 128), 0)
        lane = lax.broadcasted_iota(jnp.int32, (4 * HS, 128), 1)
        lo = (row // HS) * DH
        mext[g] = mext[g] + jnp.where((lane >= lo) & (lane < lo + DH), upd, 0.0)
        return ret

    def wo_part(lo, hi):
        otb = jnp.concatenate([ot[i, lo:hi, :].astype(BF16) for i in range(QT)], axis=1)
        return jnp.dot(wot[:, lo:hi], otb, preferred_element_type=F32)

    def finish(s, att):
        cols = seg_cols(s)
        res = xs[:, cols].astype(F32) + _bf(att) + xn[:, cols].astype(F32)
        outs[:, cols] = res.astype(BF16)

    def segment_fast(s):
        prev = None
        hid = {}
        for g in range(NG):
            qk, pv = stage_fns(s, g, slice(GD * g, GD * (g + 1)), memory(s, g), False)
            for i in range(QT):
                p = qk(i)
                if prev is not None:
                    prev[0](prev[1], prev[2])
                prev = (pv, i, p)
                if i == 1:
                    hid[g] = ffn_up(s, g)
                if i == 3:
                    ffn_down(s, g, hid[g])
                if (g, i) == (3, 0):
                    hid[8] = ffn_up(s, 8)
                if (g, i) == (4, 0):
                    ffn_down(s, 8, hid[8])
        att = wo_part(0, 384)
        prev[0](prev[1], prev[2])
        finish(s, att + wo_part(384, D))

    def segment_safe(s):
        def body(g, c):
            g_rows = pl.ds(pl.multiple_of(GD * g, 8), GD)
            qk, pv = stage_fns(s, g, g_rows, memory(s, g), True)
            for i in range(QT):
                pv(i, qk(i))
            return c
        lax.fori_loop(0, NG, body, 0)

        def ffn_body(u, c):
            ffn_down(s, u, ffn_up(s, u))
            return c
        lax.fori_loop(0, FU, ffn_body, 0)
        finish(s, wo_part(0, D))

    def phase_b(s, carry):
        for cp in ffn_copies(s):
            cp.wait()
        lax.cond(bound[s] <= SAFE_LOGIT_BOUND, segment_fast, segment_safe, s)

        @pl.when(s < NSEG - 1)
        def _():
            out_copy(s).start()
        return carry

    lax.fori_loop(0, NSEG, phase_b, 0)

    def tile_copy(t, sem):
        return pltpu.make_async_copy(outs.at[:, t], out_hbm.at[:, t], sems.at[sem])

    last = (NSEG - 1) * L
    t1, t2 = i1 // 128, i2 // 128
    last_tiles = [slice(last + 128 * j, last + 128 * (j + 1)) for j in range(QT)]
    touched = [(t1 == (NSEG - 1) * QT + j) | (t2 == (NSEG - 1) * QT + j) for j in range(QT)]
    for j in range(QT):
        @pl.when(jnp.logical_not(touched[j]))
        def _():
            tile_copy(last_tiles[j], SEM_LAST + j).start()

    rowd = lax.broadcasted_iota(jnp.int32, (8, D), 0)
    y = _bf(_bf(yacc[...]) * _bf(jax.nn.sigmoid(jnp.where(rowd == 0, r1, r2))))
    for s in range(NSEG - 1):
        out_copy(s).wait()
    TN = (((0,), (0,)), ((), ()))
    for idx, hot in ((i1, hot1), (i2, hot2)):
        add = lax.dot_general(y, hot, TN, preferred_element_type=F32)
        outs[:, tile_of(idx)] = (outs[:, tile_of(idx)].astype(F32) + add).astype(BF16)

    fix1 = i1 < last
    fix2 = (i2 < last) & (t2 != t1)
    for j in range(QT):
        @pl.when(touched[j])
        def _():
            tile_copy(last_tiles[j], SEM_LAST + j).start()

    @pl.when(fix1)
    def _():
        tile_copy(tile_of(i1), SEM_FIX).start()

    @pl.when(fix2)
    def _():
        tile_copy(tile_of(i2), SEM_FIX + 1).start()

    for j in range(QT):
        tile_copy(last_tiles[j], SEM_LAST + j).wait()

    @pl.when(fix1)
    def _():
        tile_copy(tile_of(i1), SEM_FIX).wait()

    @pl.when(fix2)
    def _():
        tile_copy(tile_of(i2), SEM_FIX + 1).wait()


@jax.jit
def pallas_parallel_sum__memory_aug_infini_attn__moe_arch_mod__prompt_kernel(
    A_x: jax.Array,
    A_wq: jax.Array,
    A_wk: jax.Array,
    A_wv: jax.Array,
    A_wo: jax.Array,
    A_beta: jax.Array,
    B_x: jax.Array,
    B_w_r: jax.Array,
    B_w_gate: jax.Array,
    B_w_up: jax.Array,
    B_w_down: jax.Array,
):
    del B_x
    xt = A_x.reshape(S, D).T
    wdt = B_w_down.T
    hbm = pl.BlockSpec(memory_space=pltpu.HBM)
    out = pl.pallas_call(
        _kernel,
        out_shape=jax.ShapeDtypeStruct((D, S), BF16),
        in_specs=[hbm] * 10,
        out_specs=hbm,
        scratch_shapes=[
            pltpu.VMEM((D, S), BF16),
            pltpu.VMEM((D, S), BF16),
            pltpu.VMEM((D, D), BF16),
            pltpu.VMEM((D, D), BF16),
            pltpu.VMEM((D, D), BF16),
            pltpu.VMEM((D, D), BF16),
            pltpu.VMEM((H,), BF16),
            pltpu.VMEM((D,), BF16),
            pltpu.VMEM((WROWS, D), BF16),
            pltpu.VMEM((D, D), BF16),
            pltpu.VMEM((2, H, 128), F32),
            pltpu.VMEM((NSEG, D, L), F32),
            pltpu.VMEM((NSEG, NG, L, 128), BF16),
            pltpu.VMEM((NSEG, NG, KP, L), BF16),
            pltpu.VMEM((NSEG, NG, L, 128), BF16),
            pltpu.VMEM((NSEG, NG, 4 * HS, L), F32),
            pltpu.VMEM((NG, 4 * HS, 128), F32),
            pltpu.VMEM((QT, D + 24, 128), F32),
            pltpu.VMEM((D, S), BF16),
            pltpu.VMEM((NSEG * QT, 128), F32),
            pltpu.SMEM((NSEG,), F32),
            pltpu.VMEM((8, D), F32),
            pltpu.VMEM((8, D), F32),
            pltpu.VMEM((D, F), BF16),
            pltpu.VMEM((D, F), BF16),
            pltpu.VMEM((D, F), BF16),
            pltpu.SemaphoreType.DMA((N_SEMS,)),
        ],
        compiler_params=pltpu.CompilerParams(vmem_limit_bytes=110 * 1024 * 1024),
    )(xt, A_wq, A_wk, A_wv, A_wo, A_beta, B_w_r, B_w_gate, B_w_up, wdt)
    return out.T.reshape(1, S, D)
```

```python
import math

import jax
import jax.numpy as jnp
from jax import lax
import jax.experimental.pallas as pl
import jax.experimental.pallas.tpu as pltpu

S = 2048
D = 576
H = 32
DH = 18
NSEG = 4
L = S // NSEG
F = 4608
NG = 8
GD = 4 * DH
HS = 24
QT = L // 128
WROWS = 3 * D + 16
FU = F // 128 // NSEG
FC = F // NSEG
KP = 80

F32 = jnp.float32
BF16 = jnp.bfloat16
QSCALE = (DH ** -0.5) * math.log2(math.e)
SAFE_LOGIT_BOUND = 32.0

NT = (((1,), (1,)), ((), ()))

(SEM_X, SEM_WQ, SEM_WK, SEM_WV, SEM_WO, SEM_BETA, SEM_WR,
 SEM_OUT, SEM_FIX, SEM_LAST, SEM_FFN) = 0, 4, 5, 6, 7, 8, 9, 10, 13, 15, 19
N_SEMS = SEM_FFN + 3 * NSEG


def _bf(x):
    return x.astype(BF16).astype(F32)


def _phi(t):
    return jnp.where(t > 0, t + 1.0, jnp.exp(t))


def _absmax(t):
    return jnp.max(jnp.abs(t).reshape(t.shape[0] // 8, 8, t.shape[1]), axis=0)


def _rows_padded(a, start, rows):
    stop = min(start + rows, a.shape[0])
    part = a[start:stop]
    if stop - start < rows:
        part = jnp.concatenate([part, jnp.zeros((rows - (stop - start), a.shape[1]), a.dtype)], axis=0)
    return part


def _kernel(x_hbm, wq_hbm, wk_hbm, wv_hbm, wo_hbm, beta_hbm, wr_hbm, wg_hbm, wu_hbm, wd_hbm,
            out_hbm,
            xs, xn, wq, wk, wv, wo, beta, wr, wt, wot, gtab, qts, kwin, pqt, pkwin, vts, mext, ot,
            outs, rbuf, bound, yacc, xsel_ref, wg, wu, wd, sems):

    def seg_cols(s):
        if isinstance(s, int):
            return slice(s * L, (s + 1) * L)
        return pl.ds(pl.multiple_of(s * L, L), L)

    def x_copy(s):
        return pltpu.make_async_copy(x_hbm.at[:, seg_cols(s)], xs.at[:, seg_cols(s)], sems.at[SEM_X + s])

    def out_copy(s):
        return pltpu.make_async_copy(outs.at[:, seg_cols(s)], out_hbm.at[:, seg_cols(s)],
                                     sems.at[SEM_OUT + s])

    cp_wq = pltpu.make_async_copy(wq_hbm, wq, sems.at[SEM_WQ])
    cp_wk = pltpu.make_async_copy(wk_hbm, wk, sems.at[SEM_WK])
    cp_wv = pltpu.make_async_copy(wv_hbm, wv, sems.at[SEM_WV])
    cp_wo = pltpu.make_async_copy(wo_hbm, wo, sems.at[SEM_WO])

    def ffn_copies(s):
        if isinstance(s, int):
            cols = slice(s * FC, (s + 1) * FC)
        else:
            cols = pl.ds(pl.multiple_of(s * FC, 128), FC)
        return [pltpu.make_async_copy(src.at[:, cols], dst.at[:, cols], sems.at[SEM_FFN + 3 * s + k])
                for k, (src, dst) in enumerate(((wg_hbm, wg), (wu_hbm, wu), (wd_hbm, wd)))]

    cp_beta = pltpu.make_async_copy(beta_hbm, beta, sems.at[SEM_BETA])
    cp_wr = pltpu.make_async_copy(wr_hbm, wr, sems.at[SEM_WR])

    def transposed(w_ref):
        return w_ref[...].astype(F32).T.astype(BF16)

    def layernorm(s):
        x32 = xs[:, seg_cols(s)].astype(F32)
        mean = jnp.sum(x32, axis=0, keepdims=True) / D
        cen = x32 - mean
        var = jnp.sum(cen * cen, axis=0, keepdims=True) / D
        den = _bf(jnp.sqrt(_bf(_bf(var) + _bf(jnp.float32(1e-5)))))
        xn[:, seg_cols(s)] = (_bf(x32 - _bf(mean)) * (1.0 / den)).astype(BF16)

    def proj_q(s, g0, g1):
        q = jnp.dot(wt[GD * g0:GD * g1, :], xn[:, seg_cols(s)], preferred_element_type=F32)
        qsc = q * QSCALE
        qts[s, GD * g0:GD * g1, :] = qsc
        pq = _phi(q)
        pad = jnp.zeros((KP - GD, L), F32)
        for g in range(g0, g1):
            win = jnp.concatenate([pq[GD * (g - g0):GD * (g - g0 + 1)], pad], axis=0)
            pqt[s, g] = win.astype(BF16)
        return jnp.max(_absmax(qsc))

    def proj_k(s):
        k = jnp.dot(wt[D:2 * D, :], xn[:, seg_cols(s)], preferred_element_type=F32)
        for g in range(NG):
            kw = _rows_padded(k, GD * g, 128).T
            kwin[s, g] = kw.astype(BF16)
            pkwin[s, g] = _phi(kw).astype(BF16)
        return jnp.max(_absmax(k))

    def proj_v(s):
        v = jnp.dot(wt[2 * D:WROWS, :], xn[:, seg_cols(s)], preferred_element_type=F32)
        for j in range(QT):
            rbuf[s * QT + j:s * QT + j + 1, :] = _bf(v[D:D + 1, 128 * j:128 * (j + 1)])
        hrow = lax.broadcasted_iota(jnp.int32, (HS, L), 0)
        fill = jnp.where(hrow == DH, 1.0, 0.0)
        for h in range(H):
            g, hh = divmod(h, 4)
            vts[s, g, HS * hh:HS * (hh + 1), :] = jnp.where(
                hrow < DH, v[DH * h:DH * h + HS], fill)

    def tile_of(idx):
        return pl.ds(pl.multiple_of((idx // 128) * 128, 128), 128)

    def router():
        r = rbuf[...]
        tok = (lax.broadcasted_iota(jnp.int32, r.shape, 0) * 128
               + lax.broadcasted_iota(jnp.int32, r.shape, 1))
        r1 = jnp.max(r)
        i1 = jnp.min(jnp.where(r == r1, tok, S))
        rm = jnp.where(tok == i1, -jnp.inf, r)
        r2 = jnp.max(rm)
        i2 = jnp.min(jnp.where((rm == r2) & (tok != i1), tok, S))
        i1 = jnp.minimum(i1, S - 1)
        i2 = jnp.minimum(i2, S - 1)
        row8 = lax.broadcasted_iota(jnp.int32, (8, 128), 0)
        lane8 = lax.broadcasted_iota(jnp.int32, (8, 128), 1)
        hot1 = jnp.where((row8 == 0) & (lane8 == i1 % 128), 1.0, 0.0)
        hot2 = jnp.where((row8 == 1) & (lane8 == i2 % 128), 1.0, 0.0)
        return r1, r2, i1, i2, hot1, hot2

    x_copy(0).start()
    cp_wq.start()
    cp_wr.start()
    cp_beta.start()
    mext[...] = jnp.zeros(mext.shape, F32)
    yacc[...] = jnp.zeros(yacc.shape, F32)
    x_copy(0).wait()
    cp_wv.start()
    cp_wk.start()
    layernorm(0)
    cp_wq.wait()
    for s in range(1, NSEG):
        x_copy(s).start()
    cp_wo.start()
    wt[0:D, :] = transposed(wq)
    qm = proj_q(0, 0, NG // 2)
    cp_wv.wait()
    cp_wk.wait()
    cp_wr.wait()
    wt[2 * D:3 * D, :] = transposed(wv)
    row16 = lax.broadcasted_iota(jnp.int32, (16, D), 0)
    wt[3 * D:WROWS, :] = jnp.where(
        row16 == 0, wr[...].astype(F32).reshape(1, D), 0.0).astype(BF16)
    qm = jnp.maximum(qm, proj_q(0, NG // 2, NG))
    wt[D:2 * D, :] = transposed(wk)
    proj_v(0)
    for s in range(1, NSEG):
        x_copy(s).wait()
    cp_wo.wait()
    for s in range(NSEG):
        for cp in ffn_copies(s):
            cp.start()
    cp_beta.wait()
    bound[0] = DH * qm * proj_k(0)
    layernorm(1)
    for s in range(1, NSEG):
        if s == NSEG - 1:
            proj_v(s)
            r1, r2, i1, i2, hot1, hot2 = router()
            km = proj_k(s)
            bound[s] = DH * km * proj_q(s, 0, NG)
            xsel_ref[...] = (
                lax.dot_general(hot1, xn[:, tile_of(i1)], NT, preferred_element_type=F32)
                + lax.dot_general(hot2, xn[:, tile_of(i2)], NT, preferred_element_type=F32))
            continue
        qm = proj_q(s, 0, NG)
        layernorm(s + 1)
        if s == 1:
            wot[...] = transposed(wo)
            b = beta[...].astype(F32).reshape(1, H)
            bt = jnp.broadcast_to(
                jnp.concatenate([b, jnp.zeros((1, 128 - H), F32)], axis=1), (128, 128)).T
            gt_all = _bf(jax.nn.sigmoid(bt[0:H]))
            gtab[0] = gt_all
            gtab[1] = _bf(1.0 - gt_all)
        bound[s] = DH * qm * proj_k(s)
        proj_v(s)

    krow = lax.broadcasted_iota(jnp.int32, (128, 128), 0)
    kcol = lax.broadcasted_iota(jnp.int32, (128, 128), 1)
    causal = krow <= kcol

    def ffn_cols(s, u):
        return pl.ds(pl.multiple_of((s * FU + u) * 128, 128), 128)

    def ffn_up_part(s, u, lo, hi):
        w2 = jnp.concatenate([wg[lo:hi, ffn_cols(s, u)], wu[lo:hi, ffn_cols(s, u)]], axis=1)
        return jnp.dot(xsel_ref[:, lo:hi], w2, preferred_element_type=F32)

    def ffn_act(gu):
        gate = _bf(gu[:, 0:128])
        return _bf(_bf(gate * jax.nn.sigmoid(gate)) * _bf(gu[:, 128:256]))

    def ffn_down_part(s, u, hid, lo, hi):
        yacc[:, lo:hi] += lax.dot_general(hid, wd[lo:hi, ffn_cols(s, u)], NT,
                                          preferred_element_type=F32)

    def ffn_items(s):
        st = {}

        def up(u, lo, hi):
            def run():
                part = ffn_up_part(s, u, lo, hi)
                st[u] = part if lo == 0 else st[u] + part
                if hi == D:
                    st[u] = ffn_act(st[u])
            return run

        def down(u, lo, hi):
            return lambda: ffn_down_part(s, u, st[u], lo, hi)

        items = []
        for u in range(FU + 1):
            if u < FU:
                items += [up(u, 0, 256), up(u, 256, 512), up(u, 512, D)]
            if u > 0:
                items += [down(u - 1, 0, 512), down(u - 1, 512, D)]
        return items

    def weight_tile(parts):
        blocks = []
        for b in range(KP // 8):
            row = 8 * b + lax.broadcasted_iota(jnp.int32, (8, 128), 0)
            lane = lax.broadcasted_iota(jnp.int32, (8, 128), 1)
            blk = jnp.zeros((8, 128), F32)
            for hh, vals, lo, hi in parts:
                r0, r1 = DH * hh, DH * hh + DH
                if r1 <= 8 * b or r0 >= 8 * b + 8:
                    continue
                keep = None
                for cond in ([row >= r0] if r0 > 8 * b else []) + ([row < r1] if r1 < 8 * b + 8 else []) \
                        + ([lane >= lo] if lo > 0 else []) + ([lane < hi] if hi < 128 else []):
                    keep = cond if keep is None else keep & cond
                v = vals[8 * b:8 * b + 8]
                blk = v if keep is None else jnp.where(keep, v, blk)
            blocks.append(blk)
        return jnp.concatenate(blocks, axis=0).astype(BF16)

    def stage_fns(s, g, g_rows, ret):
        def qk_safe(i):
            q = qts[s, g_rows, 128 * i:128 * (i + 1)]
            qm = jnp.concatenate([weight_tile([(hh, q, 0, 128)]) for hh in range(4)], axis=1)
            nk = 128 * (i + 1)
            st = jnp.dot(kwin[s, g, 0:nk, 0:KP], qm, preferred_element_type=F32)
            ps = []
            for hh in range(4):
                sc = st[:, 128 * hh:128 * (hh + 1)]
                diag = jnp.where(causal, sc[nk - 128:], -1e30)
                sc = jnp.concatenate([sc[:nk - 128], diag], axis=0) if i > 0 else diag
                sc = sc - jnp.max(sc, axis=0, keepdims=True)
                ps.append(jnp.exp2(sc).astype(BF16))
            return ps

        qk = qk_safe

        def pv(i, ps):
            nk = 128 * (i + 1)
            for hh in range(4):
                v = vts[s, g, HS * hh:HS * (hh + 1), 0:nk]
                combine(s, g, ret, i, hh, jnp.dot(v, ps[hh], preferred_element_type=F32))
        return qk, pv

    def combine(s, g, ret, i, hh, o):
        h = 4 * g + hh
        mem = ret[HS * hh:HS * (hh + 1), 128 * i:128 * (i + 1)]
        w_mem = gtab[0, pl.ds(h, 1), :] / (mem[DH:DH + 1] + 1e-6)
        w_dot = gtab[1, pl.ds(h, 1), :] / o[DH:DH + 1]
        ot[i, pl.ds(DH * h, HS), :] = mem * w_mem + o * w_dot

    def qk_items(s, g, i):
        q = qts[s, GD * g:GD * (g + 1), 128 * i:128 * (i + 1)]
        base = 128 * i
        blocks = {}
        st = {}

        def scores(lo, hi, w):
            return jnp.exp2(jnp.dot(kwin[s, g, lo:hi, 0:KP], w, preferred_element_type=F32))

        tile = lambda e, t: e[:, 128 * t:128 * (t + 1)]
        roll = lambda e, t: pltpu.roll(e, t, 1)
        qm = jnp.concatenate([weight_tile([(hh, q, 0, 128)]) for hh in range(4)], axis=1)

        def full(j):
            def run():
                last = j == i - 1
                e = scores(128 * j, 128 * (j + 1) + (32 if last else 0), qm)
                blocks[j] = [tile(e, hh)[0:128].astype(BF16) for hh in range(4)]
                if last:
                    st[0] = e[128:160]
            return run

        def d0():
            st[0] = scores(0, 32, qm)

        def d1():
            st['q'] = [roll(q, t) for t in (32, 64, 96)]
            q32, q64, q96 = st['q']
            st[1] = scores(base + 32, base + 64, jnp.concatenate([
                weight_tile([(0, q, 32, 128), (3, q96, 0, 32)]),
                weight_tile([(1, q, 32, 128), (3, q64, 0, 32)]),
                weight_tile([(2, q, 32, 128), (3, q32, 0, 32)])], axis=1))

        def d2():
            q32, q64, q96 = st['q']
            st[2] = scores(base + 64, base + 96, jnp.concatenate([
                weight_tile([(0, q, 64, 128), (2, q64, 0, 64)]),
                weight_tile([(1, q, 64, 128), (3, q64, 0, 64)])], axis=1))

        def d3():
            q32, q64, q96 = st['q']
            e3 = scores(base + 96, base + 128,
                        weight_tile([(0, q, 96, 128), (1, q96, 64, 96), (2, q64, 32, 64), (3, q32, 0, 32)]))
            e0, e1, e2 = st[0], st[1], st[2]
            lane = lax.broadcasted_iota(jnp.int32, (32, 128), 1)
            blk1 = [tile(e1, 0), tile(e1, 1), tile(e1, 2),
                    jnp.where(lane < 64, roll(tile(e1, 0), 32),
                              jnp.where(lane < 96, roll(tile(e1, 1), 64), roll(tile(e1, 2), 96)))]
            blk2 = [tile(e2, 0), tile(e2, 1), roll(tile(e2, 0), 64), roll(tile(e2, 1), 64)]
            blk3 = [e3, roll(e3, 32), roll(e3, 64), roll(e3, 96)]
            blocks[i] = [
                jnp.where(causal, jnp.concatenate([tile(e0, hh), blk1[hh], blk2[hh], blk3[hh]], axis=0),
                          0.0).astype(BF16) for hh in range(4)]

        items = [full(j) for j in range(i)] + ([d0] if i == 0 else []) + [d1, d2, d3]
        return items, blocks

    def pv_items(s, g, i, rets, blocks):
        acc = {}

        def block(j):
            def run():
                for hh in range(4):
                    v = vts[s, g, HS * hh:HS * (hh + 1), 128 * j:128 * (j + 1)]
                    o = jnp.dot(v, blocks[j][hh], preferred_element_type=F32)
                    acc[hh] = o if j == 0 else acc[hh] + o
                    if j == i:
                        combine(s, g, rets[g], i, hh, acc[hh])
            return run
        return [block(j) for j in range(i + 1)]

    def mem_read(s, g):
        return jnp.dot(mext[g][:, 0:KP], pqt[s, g], preferred_element_type=F32)

    def mem_update(s, g):
        upd = jnp.dot(vts[s, g], pkwin[s, g], preferred_element_type=F32)
        row = lax.broadcasted_iota(jnp.int32, (4 * HS, 128), 0)
        lane = lax.broadcasted_iota(jnp.int32, (4 * HS, 128), 1)
        lo = (row // HS) * DH
        mext[g] = mext[g] + jnp.where((lane >= lo) & (lane < lo + DH), upd, 0.0)

    def wo_part(lo, hi):
        otb = jnp.concatenate([ot[i, lo:hi, :].astype(BF16) for i in range(QT)], axis=1)
        return jnp.dot(wot[:, lo:hi], otb, preferred_element_type=F32)

    def finish(s, att):
        cols = seg_cols(s)
        res = xs[:, cols].astype(F32) + _bf(att) + xn[:, cols].astype(F32)
        outs[:, cols] = res.astype(BF16)

    def segment_fast(s):
        pending = []
        ffn = ffn_items(s)
        rets = {}

        def read(g):
            rets[g] = mem_read(s, g)

        for g in range(NG):
            for i in range(QT):
                items, blocks = qk_items(s, g, i)
                for n in range(len(items)):
                    items[n]()
                    if n < i and ffn:
                        ffn.pop(0)()
                    if n < len(pending) - 1:
                        pending[n]()
                    if (i, n) == (0, 1):
                        read(g)
                    if (i, n) == (0, 3):
                        mem_update(s, g)
                if pending:
                    pending[-1]()
                pending = pv_items(s, g, i, rets, blocks)
        assert not ffn
        att = wo_part(0, 384)
        for f in pending:
            f()
        finish(s, att + wo_part(384, D))

    def segment_safe(s):
        def body(g, c):
            g_rows = pl.ds(pl.multiple_of(GD * g, 8), GD)
            qk, pv = stage_fns(s, g, g_rows, mem_read(s, g))
            mem_update(s, g)
            for i in range(QT):
                pv(i, qk(i))
            return c
        lax.fori_loop(0, NG, body, 0)

        def ffn_body(u, c):
            hid = ffn_act(ffn_up_part(s, u, 0, D))
            ffn_down_part(s, u, hid, 0, D)
            return c
        lax.fori_loop(0, FU, ffn_body, 0)
        finish(s, wo_part(0, D))

    def phase_b(s, carry):
        for cp in ffn_copies(s):
            cp.wait()
        lax.cond(bound[s] <= SAFE_LOGIT_BOUND, segment_fast, segment_safe, s)

        @pl.when(s < NSEG - 1)
        def _():
            out_copy(s).start()
        return carry

    lax.fori_loop(0, NSEG, phase_b, 0)

    def tile_copy(t, sem):
        return pltpu.make_async_copy(outs.at[:, t], out_hbm.at[:, t], sems.at[sem])

    last = (NSEG - 1) * L
    t1, t2 = i1 // 128, i2 // 128
    last_tiles = [slice(last + 128 * j, last + 128 * (j + 1)) for j in range(QT)]
    touched = [(t1 == (NSEG - 1) * QT + j) | (t2 == (NSEG - 1) * QT + j) for j in range(QT)]
    for j in range(QT):
        @pl.when(jnp.logical_not(touched[j]))
        def _():
            tile_copy(last_tiles[j], SEM_LAST + j).start()

    rowd = lax.broadcasted_iota(jnp.int32, (8, D), 0)
    y = _bf(_bf(yacc[...]) * _bf(jax.nn.sigmoid(jnp.where(rowd == 0, r1, r2))))
    for s in range(NSEG - 1):
        out_copy(s).wait()
    TN = (((0,), (0,)), ((), ()))
    for idx, hot in ((i1, hot1), (i2, hot2)):
        add = lax.dot_general(y, hot, TN, preferred_element_type=F32)
        outs[:, tile_of(idx)] = (outs[:, tile_of(idx)].astype(F32) + add).astype(BF16)

    fix1 = i1 < last
    fix2 = (i2 < last) & (t2 != t1)
    for j in range(QT):
        @pl.when(touched[j])
        def _():
            tile_copy(last_tiles[j], SEM_LAST + j).start()

    @pl.when(fix1)
    def _():
        tile_copy(tile_of(i1), SEM_FIX).start()

    @pl.when(fix2)
    def _():
        tile_copy(tile_of(i2), SEM_FIX + 1).start()

    for j in range(QT):
        tile_copy(last_tiles[j], SEM_LAST + j).wait()

    @pl.when(fix1)
    def _():
        tile_copy(tile_of(i1), SEM_FIX).wait()

    @pl.when(fix2)
    def _():
        tile_copy(tile_of(i2), SEM_FIX + 1).wait()


@jax.jit
def pallas_parallel_sum__memory_aug_infini_attn__moe_arch_mod__prompt_kernel(
    A_x: jax.Array,
    A_wq: jax.Array,
    A_wk: jax.Array,
    A_wv: jax.Array,
    A_wo: jax.Array,
    A_beta: jax.Array,
    B_x: jax.Array,
    B_w_r: jax.Array,
    B_w_gate: jax.Array,
    B_w_up: jax.Array,
    B_w_down: jax.Array,
):
    del B_x
    xt = A_x.reshape(S, D).T
    wdt = B_w_down.T
    hbm = pl.BlockSpec(memory_space=pltpu.HBM)
    out = pl.pallas_call(
        _kernel,
        out_shape=jax.ShapeDtypeStruct((D, S), BF16),
        in_specs=[hbm] * 10,
        out_specs=hbm,
        scratch_shapes=[
            pltpu.VMEM((D, S), BF16),
            pltpu.VMEM((D, S), BF16),
            pltpu.VMEM((D, D), BF16),
            pltpu.VMEM((D, D), BF16),
            pltpu.VMEM((D, D), BF16),
            pltpu.VMEM((D, D), BF16),
            pltpu.VMEM((H,), BF16),
            pltpu.VMEM((D,), BF16),
            pltpu.VMEM((WROWS, D), BF16),
            pltpu.VMEM((D, D), BF16),
            pltpu.VMEM((2, H, 128), F32),
            pltpu.VMEM((NSEG, D, L), F32),
            pltpu.VMEM((NSEG, NG, L, 128), BF16),
            pltpu.VMEM((NSEG, NG, KP, L), BF16),
            pltpu.VMEM((NSEG, NG, L, 128), BF16),
            pltpu.VMEM((NSEG, NG, 4 * HS, L), F32),
            pltpu.VMEM((NG, 4 * HS, 128), F32),
            pltpu.VMEM((QT, D + 24, 128), F32),
            pltpu.VMEM((D, S), BF16),
            pltpu.VMEM((NSEG * QT, 128), F32),
            pltpu.SMEM((NSEG,), F32),
            pltpu.VMEM((8, D), F32),
            pltpu.VMEM((8, D), F32),
            pltpu.VMEM((D, F), BF16),
            pltpu.VMEM((D, F), BF16),
            pltpu.VMEM((D, F), BF16),
            pltpu.SemaphoreType.DMA((N_SEMS,)),
        ],
        compiler_params=pltpu.CompilerParams(vmem_limit_bytes=110 * 1024 * 1024),
    )(xt, A_wq, A_wk, A_wv, A_wo, A_beta, B_w_r, B_w_gate, B_w_up, wdt)
    return out.T.reshape(1, S, D)
```

```python
import math

import jax
import jax.numpy as jnp
from jax import lax
import jax.experimental.pallas as pl
import jax.experimental.pallas.tpu as pltpu

S = 2048
D = 576
H = 32
DH = 18
NSEG = 4
L = S // NSEG
F = 4608
NG = 8
GD = 4 * DH
HS = 24
QT = L // 128
WROWS = 3 * D + 16
FU = F // 128 // NSEG
FC = F // NSEG
KP = 80

F32 = jnp.float32
BF16 = jnp.bfloat16
QSCALE = (DH ** -0.5) * math.log2(math.e)
SAFE_LOGIT_BOUND = 60.0
SAFE_VALUE_BOUND = 2.0 ** 40
XN_SQ_BOUND = 2.0 * D * 1.1

NT = (((1,), (1,)), ((), ()))

(SEM_X, SEM_WQ, SEM_WK, SEM_WV, SEM_WO, SEM_BETA, SEM_WR,
 SEM_OUT, SEM_FIX, SEM_LAST, SEM_FFN) = 0, 4, 5, 6, 7, 8, 9, 10, 13, 15, 19
N_SEMS = SEM_FFN + 3 * NSEG


def _bf(x):
    return x.astype(BF16).astype(F32)


def _phi(t):
    return jnp.where(t > 0, t + 1.0, jnp.exp(t))


def _max_col_sq(w32):
    return jnp.max(jnp.sum(w32 * w32, axis=0, keepdims=True))


def _rows_padded(a, start, rows):
    stop = min(start + rows, a.shape[0])
    part = a[start:stop]
    if stop - start < rows:
        part = jnp.concatenate([part, jnp.zeros((rows - (stop - start), a.shape[1]), a.dtype)], axis=0)
    return part


def _kernel(x_hbm, wq_hbm, wk_hbm, wv_hbm, wo_hbm, beta_hbm, wr_hbm, wg_hbm, wu_hbm, wd_hbm,
            out_hbm,
            xs, xn, wq, wk, wv, wo, beta, wr, wt, wot, gtab, qts, kwin, pqt, pkwin, vts, mext, ot,
            outs, rbuf, yacc, xsel_ref, wg, wu, wd, sems):

    def seg_cols(s):
        if isinstance(s, int):
            return slice(s * L, (s + 1) * L)
        return pl.ds(pl.multiple_of(s * L, L), L)

    def x_copy(s):
        return pltpu.make_async_copy(x_hbm.at[:, seg_cols(s)], xs.at[:, seg_cols(s)], sems.at[SEM_X + s])

    def out_copy(s):
        return pltpu.make_async_copy(outs.at[:, seg_cols(s)], out_hbm.at[:, seg_cols(s)],
                                     sems.at[SEM_OUT + s])

    cp_wq = pltpu.make_async_copy(wq_hbm, wq, sems.at[SEM_WQ])
    cp_wk = pltpu.make_async_copy(wk_hbm, wk, sems.at[SEM_WK])
    cp_wv = pltpu.make_async_copy(wv_hbm, wv, sems.at[SEM_WV])
    cp_wo = pltpu.make_async_copy(wo_hbm, wo, sems.at[SEM_WO])

    def ffn_copies(s):
        if isinstance(s, int):
            cols = slice(s * FC, (s + 1) * FC)
        else:
            cols = pl.ds(pl.multiple_of(s * FC, 128), FC)
        return [pltpu.make_async_copy(src.at[:, cols], dst.at[:, cols], sems.at[SEM_FFN + 3 * s + k])
                for k, (src, dst) in enumerate(((wg_hbm, wg), (wu_hbm, wu), (wd_hbm, wd)))]

    cp_beta = pltpu.make_async_copy(beta_hbm, beta, sems.at[SEM_BETA])
    cp_wr = pltpu.make_async_copy(wr_hbm, wr, sems.at[SEM_WR])

    def transposed(w_ref):
        w32 = w_ref[...].astype(F32)
        return w32.T.astype(BF16), _max_col_sq(w32)

    def layernorm(s):
        x32 = xs[:, seg_cols(s)].astype(F32)
        mean = jnp.sum(x32, axis=0, keepdims=True) / D
        mean_b = _bf(mean)
        cen = x32 - mean_b
        shift = mean - mean_b
        var = jnp.sum(cen * cen, axis=0, keepdims=True) / D - shift * shift
        den = _bf(jnp.sqrt(_bf(_bf(var) + _bf(jnp.float32(1e-5)))))
        xn[:, seg_cols(s)] = (_bf(cen) * (1.0 / den)).astype(BF16)

    def proj_q(s, g0, g1):
        q = jnp.dot(wt[GD * g0:GD * g1, :], xn[:, seg_cols(s)], preferred_element_type=F32)
        qts[s, GD * g0:GD * g1, :] = q * QSCALE
        pq = _phi(q)
        pad = jnp.zeros((KP - GD, L), F32)
        for g in range(g0, g1):
            win = jnp.concatenate([pq[GD * (g - g0):GD * (g - g0 + 1)], pad], axis=0)
            pqt[s, g] = win.astype(BF16)

    def proj_k(s):
        k = jnp.dot(wt[D:2 * D, :], xn[:, seg_cols(s)], preferred_element_type=F32)
        for g in range(NG):
            kw = _rows_padded(k, GD * g, 128).T
            kwin[s, g] = kw.astype(BF16)
            pkwin[s, g] = _phi(kw).astype(BF16)

    def proj_v(s):
        v = jnp.dot(wt[2 * D:WROWS, :], xn[:, seg_cols(s)], preferred_element_type=F32)
        for j in range(QT):
            rbuf[s * QT + j:s * QT + j + 1, :] = _bf(v[D:D + 1, 128 * j:128 * (j + 1)])
        hrow = lax.broadcasted_iota(jnp.int32, (HS, L), 0)
        fill = jnp.where(hrow == DH, 1.0, 0.0)
        for h in range(H):
            g, hh = divmod(h, 4)
            vts[s, g, HS * hh:HS * (hh + 1), :] = jnp.where(
                hrow < DH, v[DH * h:DH * h + HS], fill)

    def tile_of(idx):
        return pl.ds(pl.multiple_of((idx // 128) * 128, 128), 128)

    def router():
        r = rbuf[...]
        tok = (lax.broadcasted_iota(jnp.int32, r.shape, 0) * 128
               + lax.broadcasted_iota(jnp.int32, r.shape, 1))
        r1 = jnp.max(r)
        i1 = jnp.min(jnp.where(r == r1, tok, S))
        rm = jnp.where(tok == i1, -jnp.inf, r)
        r2 = jnp.max(rm)
        i2 = jnp.min(jnp.where((rm == r2) & (tok != i1), tok, S))
        i1 = jnp.minimum(i1, S - 1)
        i2 = jnp.minimum(i2, S - 1)
        row8 = lax.broadcasted_iota(jnp.int32, (8, 128), 0)
        lane8 = lax.broadcasted_iota(jnp.int32, (8, 128), 1)
        hot1 = jnp.where((row8 == 0) & (lane8 == i1 % 128), 1.0, 0.0)
        hot2 = jnp.where((row8 == 1) & (lane8 == i2 % 128), 1.0, 0.0)
        return r1, r2, i1, i2, hot1, hot2

    x_copy(0).start()
    cp_wq.start()
    cp_wr.start()
    cp_beta.start()
    mext[...] = jnp.zeros(mext.shape, F32)
    yacc[...] = jnp.zeros(yacc.shape, F32)
    x_copy(0).wait()
    cp_wv.start()
    cp_wk.start()
    layernorm(0)
    cp_wq.wait()
    for s in range(1, NSEG):
        x_copy(s).start()
    cp_wo.start()
    wt[0:D, :], nq = transposed(wq)
    proj_q(0, 0, NG // 2)
    cp_wv.wait()
    cp_wk.wait()
    cp_wr.wait()
    wt[2 * D:3 * D, :], nv = transposed(wv)
    row16 = lax.broadcasted_iota(jnp.int32, (16, D), 0)
    wt[3 * D:WROWS, :] = jnp.where(
        row16 == 0, wr[...].astype(F32).reshape(1, D), 0.0).astype(BF16)
    proj_q(0, NG // 2, NG)
    wt[D:2 * D, :], nk = transposed(wk)
    proj_v(0)
    for s in range(1, NSEG):
        x_copy(s).wait()
    cp_wo.wait()
    for s in range(NSEG):
        for cp in ffn_copies(s):
            cp.start()
    cp_beta.wait()
    layernorm(1)
    proj_k(0)
    for s in range(1, NSEG):
        if s == NSEG - 1:
            proj_v(s)
            r1, r2, i1, i2, hot1, hot2 = router()
            proj_k(s)
            proj_q(s, 0, NG)
            xsel_ref[...] = (
                lax.dot_general(hot1, xn[:, tile_of(i1)], NT, preferred_element_type=F32)
                + lax.dot_general(hot2, xn[:, tile_of(i2)], NT, preferred_element_type=F32))
            continue
        layernorm(s + 1)
        proj_q(s, 0, NG)
        if s == 1:
            wot[...] = wo[...].astype(F32).T.astype(BF16)
            b = beta[...].astype(F32).reshape(1, H)
            bt = jnp.broadcast_to(
                jnp.concatenate([b, jnp.zeros((1, 128 - H), F32)], axis=1), (128, 128)).T
            gt_all = _bf(jax.nn.sigmoid(bt[0:H]))
            gtab[0] = gt_all
            gtab[1] = _bf(1.0 - gt_all)
            logit_bound = (DH * QSCALE * XN_SQ_BOUND) * jnp.sqrt(nq) * jnp.sqrt(nk)
            no_shift_needed = ((logit_bound <= SAFE_LOGIT_BOUND)
                               & (XN_SQ_BOUND * nv <= SAFE_VALUE_BOUND * SAFE_VALUE_BOUND))
        proj_k(s)
        proj_v(s)

    krow = lax.broadcasted_iota(jnp.int32, (128, 128), 0)
    kcol = lax.broadcasted_iota(jnp.int32, (128, 128), 1)
    causal = krow <= kcol

    def ffn_cols(s, u):
        return pl.ds(pl.multiple_of((s * FU + u) * 128, 128), 128)

    def ffn_up_part(s, u, lo, hi):
        w2 = jnp.concatenate([wg[lo:hi, ffn_cols(s, u)], wu[lo:hi, ffn_cols(s, u)]], axis=1)
        return jnp.dot(xsel_ref[:, lo:hi], w2, preferred_element_type=F32)

    def ffn_act(gu):
        gate = _bf(gu[:, 0:128])
        return _bf(_bf(gate * jax.nn.sigmoid(gate)) * _bf(gu[:, 128:256]))

    def ffn_down_part(s, u, hid, lo, hi):
        yacc[:, lo:hi] += lax.dot_general(hid, wd[lo:hi, ffn_cols(s, u)], NT,
                                          preferred_element_type=F32)

    def ffn_items(s):
        st = {}

        def up(u, lo, hi):
            def run():
                part = ffn_up_part(s, u, lo, hi)
                st[u] = part if lo == 0 else st[u] + part
                if hi == D:
                    st[u] = ffn_act(st[u])
            return run

        def down(u, lo, hi):
            return lambda: ffn_down_part(s, u, st[u], lo, hi)

        items = []
        for u in range(FU + 1):
            if u < FU:
                items += [up(u, 0, 256), up(u, 256, 512), up(u, 512, D)]
            if u > 0:
                items += [down(u - 1, 0, 512), down(u - 1, 512, D)]
        return items

    def weight_tile(parts):
        blocks = []
        for b in range(KP // 8):
            row = 8 * b + lax.broadcasted_iota(jnp.int32, (8, 128), 0)
            lane = lax.broadcasted_iota(jnp.int32, (8, 128), 1)
            blk = jnp.zeros((8, 128), F32)
            for hh, vals, lo, hi in parts:
                r0, r1 = DH * hh, DH * hh + DH
                if r1 <= 8 * b or r0 >= 8 * b + 8:
                    continue
                keep = None
                for cond in ([row >= r0] if r0 > 8 * b else []) + ([row < r1] if r1 < 8 * b + 8 else []) \
                        + ([lane >= lo] if lo > 0 else []) + ([lane < hi] if hi < 128 else []):
                    keep = cond if keep is None else keep & cond
                v = vals[8 * b:8 * b + 8]
                blk = v if keep is None else jnp.where(keep, v, blk)
            blocks.append(blk)
        return jnp.concatenate(blocks, axis=0).astype(BF16)

    def stage_fns(s, g, g_rows, ret):
        def qk_safe(i):
            q = qts[s, g_rows, 128 * i:128 * (i + 1)]
            qm = jnp.concatenate([weight_tile([(hh, q, 0, 128)]) for hh in range(4)], axis=1)
            nk = 128 * (i + 1)
            st = jnp.dot(kwin[s, g, 0:nk, 0:KP], qm, preferred_element_type=F32)
            ps = []
            for hh in range(4):
                sc = st[:, 128 * hh:128 * (hh + 1)]
                diag = jnp.where(causal, sc[nk - 128:], -1e30)
                sc = jnp.concatenate([sc[:nk - 128], diag], axis=0) if i > 0 else diag
                sc = sc - jnp.max(sc, axis=0, keepdims=True)
                ps.append(jnp.exp2(sc).astype(BF16))
            return ps

        qk = qk_safe

        def pv(i, ps):
            nk = 128 * (i + 1)
            for hh in range(4):
                v = vts[s, g, HS * hh:HS * (hh + 1), 0:nk]
                combine(s, g, ret, i, hh, jnp.dot(v, ps[hh], preferred_element_type=F32))
        return qk, pv

    def combine(s, g, ret, i, hh, o):
        h = 4 * g + hh
        mem = ret[HS * hh:HS * (hh + 1), 128 * i:128 * (i + 1)]
        w_mem = gtab[0, pl.ds(h, 1), :] / (mem[DH:DH + 1] + 1e-6)
        w_dot = gtab[1, pl.ds(h, 1), :] / o[DH:DH + 1]
        ot[i, pl.ds(DH * h, HS), :] = mem * w_mem + o * w_dot

    def qk_items(s, g, i):
        q = qts[s, GD * g:GD * (g + 1), 128 * i:128 * (i + 1)]
        base = 128 * i
        blocks = {}
        st = {}

        def scores(lo, hi, w):
            return jnp.exp2(jnp.dot(kwin[s, g, lo:hi, 0:KP], w, preferred_element_type=F32))

        tile = lambda e, t: e[:, 128 * t:128 * (t + 1)]
        roll = lambda e, t: pltpu.roll(e, t, 1)
        qm = jnp.concatenate([weight_tile([(hh, q, 0, 128)]) for hh in range(4)], axis=1)

        def full(j):
            def run():
                last = j == i - 1
                e = scores(128 * j, 128 * (j + 1) + (32 if last else 0), qm)
                blocks[j] = [tile(e, hh)[0:128].astype(BF16) for hh in range(4)]
                if last:
                    st[0] = e[128:160]
            return run

        def d0():
            st[0] = scores(0, 32, qm)

        def d1():
            st['q'] = [roll(q, t) for t in (32, 64, 96)]
            q32, q64, q96 = st['q']
            st[1] = scores(base + 32, base + 64, jnp.concatenate([
                weight_tile([(0, q, 32, 128), (3, q96, 0, 32)]),
                weight_tile([(1, q, 32, 128), (3, q64, 0, 32)]),
                weight_tile([(2, q, 32, 128), (3, q32, 0, 32)])], axis=1))

        def d2():
            q32, q64, q96 = st['q']
            st[2] = scores(base + 64, base + 96, jnp.concatenate([
                weight_tile([(0, q, 64, 128), (2, q64, 0, 64)]),
                weight_tile([(1, q, 64, 128), (3, q64, 0, 64)])], axis=1))

        def d3():
            q32, q64, q96 = st['q']
            e3 = scores(base + 96, base + 128,
                        weight_tile([(0, q, 96, 128), (1, q96, 64, 96), (2, q64, 32, 64), (3, q32, 0, 32)]))
            e0, e1, e2 = st[0], st[1], st[2]
            lane = lax.broadcasted_iota(jnp.int32, (32, 128), 1)
            blk1 = [tile(e1, 0), tile(e1, 1), tile(e1, 2),
                    jnp.where(lane < 64, roll(tile(e1, 0), 32),
                              jnp.where(lane < 96, roll(tile(e1, 1), 64), roll(tile(e1, 2), 96)))]
            blk2 = [tile(e2, 0), tile(e2, 1), roll(tile(e2, 0), 64), roll(tile(e2, 1), 64)]
            blk3 = [e3, roll(e3, 32), roll(e3, 64), roll(e3, 96)]
            blocks[i] = [
                jnp.where(causal, jnp.concatenate([tile(e0, hh), blk1[hh], blk2[hh], blk3[hh]], axis=0),
                          0.0).astype(BF16) for hh in range(4)]

        items = [full(j) for j in range(i)] + ([d0] if i == 0 else []) + [d1, d2, d3]
        return items, blocks

    def pv_items(s, g, i, rets, blocks):
        acc = {}

        def block(j):
            def run():
                for hh in range(4):
                    v = vts[s, g, HS * hh:HS * (hh + 1), 128 * j:128 * (j + 1)]
                    o = jnp.dot(v, blocks[j][hh], preferred_element_type=F32)
                    acc[hh] = o if j == 0 else acc[hh] + o
                    if j == i:
                        combine(s, g, rets[g], i, hh, acc[hh])
            return run
        return [block(j) for j in range(i + 1)]

    def mem_read(s, g):
        return jnp.dot(mext[g][:, 0:KP], pqt[s, g], preferred_element_type=F32)

    def mem_update(s, g):
        upd = jnp.dot(vts[s, g], pkwin[s, g], preferred_element_type=F32)
        row = lax.broadcasted_iota(jnp.int32, (4 * HS, 128), 0)
        lane = lax.broadcasted_iota(jnp.int32, (4 * HS, 128), 1)
        lo = (row // HS) * DH
        mext[g] = mext[g] + jnp.where((lane >= lo) & (lane < lo + DH), upd, 0.0)

    def wo_part(lo, hi):
        otb = jnp.concatenate([ot[i, lo:hi, :].astype(BF16) for i in range(QT)], axis=1)
        return jnp.dot(wot[:, lo:hi], otb, preferred_element_type=F32)

    def finish(s, att):
        cols = seg_cols(s)
        res = xs[:, cols].astype(F32) + _bf(att) + xn[:, cols].astype(F32)
        outs[:, cols] = res.astype(BF16)

    def segment_fast(s):
        pending = []
        ffn = ffn_items(s)
        rets = {}

        def read(g):
            rets[g] = mem_read(s, g)

        for g in range(NG):
            for i in range(QT):
                items, blocks = qk_items(s, g, i)
                for n in range(len(items)):
                    items[n]()
                    if n < len(pending) - 1:
                        pending[n]()
                    if n < i and ffn:
                        ffn.pop(0)()
                    if (i, n) == (0, 1):
                        read(g)
                    if (i, n) == (0, 3):
                        mem_update(s, g)
                if pending:
                    pending[-1]()
                pending = pv_items(s, g, i, rets, blocks)
        assert not ffn
        att = wo_part(0, 384)
        for f in pending:
            f()
        finish(s, att + wo_part(384, D))

    def segment_safe(s):
        def body(g, c):
            g_rows = pl.ds(pl.multiple_of(GD * g, 8), GD)
            qk, pv = stage_fns(s, g, g_rows, mem_read(s, g))
            mem_update(s, g)
            for i in range(QT):
                pv(i, qk(i))
            return c
        lax.fori_loop(0, NG, body, 0)

        def ffn_body(u, c):
            hid = ffn_act(ffn_up_part(s, u, 0, D))
            ffn_down_part(s, u, hid, 0, D)
            return c
        lax.fori_loop(0, FU, ffn_body, 0)
        finish(s, wo_part(0, D))

    def phase_b(s, carry):
        for cp in ffn_copies(s):
            cp.wait()
        lax.cond(no_shift_needed, segment_fast, segment_safe, s)

        @pl.when(s < NSEG - 1)
        def _():
            out_copy(s).start()
        return carry

    lax.fori_loop(0, NSEG, phase_b, 0)

    def tile_copy(t, sem):
        return pltpu.make_async_copy(outs.at[:, t], out_hbm.at[:, t], sems.at[sem])

    last = (NSEG - 1) * L
    t1, t2 = i1 // 128, i2 // 128
    last_tiles = [slice(last + 128 * j, last + 128 * (j + 1)) for j in range(QT)]
    touched = [(t1 == (NSEG - 1) * QT + j) | (t2 == (NSEG - 1) * QT + j) for j in range(QT)]
    for j in range(QT):
        @pl.when(jnp.logical_not(touched[j]))
        def _():
            tile_copy(last_tiles[j], SEM_LAST + j).start()

    rowd = lax.broadcasted_iota(jnp.int32, (8, D), 0)
    y = _bf(_bf(yacc[...]) * _bf(jax.nn.sigmoid(jnp.where(rowd == 0, r1, r2))))
    for s in range(NSEG - 1):
        out_copy(s).wait()
    TN = (((0,), (0,)), ((), ()))
    for idx, hot in ((i1, hot1), (i2, hot2)):
        add = lax.dot_general(y, hot, TN, preferred_element_type=F32)
        outs[:, tile_of(idx)] = (outs[:, tile_of(idx)].astype(F32) + add).astype(BF16)

    fix1 = i1 < last
    fix2 = (i2 < last) & (t2 != t1)
    for j in range(QT):
        @pl.when(touched[j])
        def _():
            tile_copy(last_tiles[j], SEM_LAST + j).start()

    @pl.when(fix1)
    def _():
        tile_copy(tile_of(i1), SEM_FIX).start()

    @pl.when(fix2)
    def _():
        tile_copy(tile_of(i2), SEM_FIX + 1).start()

    for j in range(QT):
        tile_copy(last_tiles[j], SEM_LAST + j).wait()

    @pl.when(fix1)
    def _():
        tile_copy(tile_of(i1), SEM_FIX).wait()

    @pl.when(fix2)
    def _():
        tile_copy(tile_of(i2), SEM_FIX + 1).wait()


@jax.jit
def pallas_parallel_sum__memory_aug_infini_attn__moe_arch_mod__prompt_kernel(
    A_x: jax.Array,
    A_wq: jax.Array,
    A_wk: jax.Array,
    A_wv: jax.Array,
    A_wo: jax.Array,
    A_beta: jax.Array,
    B_x: jax.Array,
    B_w_r: jax.Array,
    B_w_gate: jax.Array,
    B_w_up: jax.Array,
    B_w_down: jax.Array,
):
    del B_x
    xt = A_x.reshape(S, D).T
    wdt = B_w_down.T
    hbm = pl.BlockSpec(memory_space=pltpu.HBM)
    out = pl.pallas_call(
        _kernel,
        out_shape=jax.ShapeDtypeStruct((D, S), BF16),
        in_specs=[hbm] * 10,
        out_specs=hbm,
        scratch_shapes=[
            pltpu.VMEM((D, S), BF16),
            pltpu.VMEM((D, S), BF16),
            pltpu.VMEM((D, D), BF16),
            pltpu.VMEM((D, D), BF16),
            pltpu.VMEM((D, D), BF16),
            pltpu.VMEM((D, D), BF16),
            pltpu.VMEM((H,), BF16),
            pltpu.VMEM((D,), BF16),
            pltpu.VMEM((WROWS, D), BF16),
            pltpu.VMEM((D, D), BF16),
            pltpu.VMEM((2, H, 128), F32),
            pltpu.VMEM((NSEG, D, L), F32),
            pltpu.VMEM((NSEG, NG, L, 128), BF16),
            pltpu.VMEM((NSEG, NG, KP, L), BF16),
            pltpu.VMEM((NSEG, NG, L, 128), BF16),
            pltpu.VMEM((NSEG, NG, 4 * HS, L), F32),
            pltpu.VMEM((NG, 4 * HS, 128), F32),
            pltpu.VMEM((QT, D + 24, 128), F32),
            pltpu.VMEM((D, S), BF16),
            pltpu.VMEM((NSEG * QT, 128), F32),
            pltpu.VMEM((8, D), F32),
            pltpu.VMEM((8, D), F32),
            pltpu.VMEM((D, F), BF16),
            pltpu.VMEM((D, F), BF16),
            pltpu.VMEM((D, F), BF16),
            pltpu.SemaphoreType.DMA((N_SEMS,)),
        ],
        compiler_params=pltpu.CompilerParams(vmem_limit_bytes=110 * 1024 * 1024),
    )(xt, A_wq, A_wk, A_wv, A_wo, A_beta, B_w_r, B_w_gate, B_w_up, wdt)
    return out.T.reshape(1, S, D)
```

```python
import math

import jax
import jax.numpy as jnp
from jax import lax
import jax.experimental.pallas as pl
import jax.experimental.pallas.tpu as pltpu

S = 2048
D = 576
H = 32
DH = 18
NSEG = 4
L = S // NSEG
F = 4608
NG = 8
GD = 4 * DH
HS = 24
QT = L // 128
WROWS = 3 * D + 16
FU = F // 128
FC = F // NSEG
DX = D + 16
KP = 80

F32 = jnp.float32
BF16 = jnp.bfloat16
QSCALE = (DH ** -0.5) * math.log2(math.e)
SAFE_LOGIT_BOUND = 60.0
SAFE_VALUE_BOUND = 2.0 ** 40
XN_SQ_BOUND = 2.0 * D * 1.1

NT = (((1,), (1,)), ((), ()))

(SEM_X, SEM_WQ, SEM_WK, SEM_WV, SEM_WO, SEM_BETA, SEM_WR,
 SEM_OUT, SEM_PIN, SEM_FFN) = 0, 4, 5, 6, 7, 8, 9, 10, 14, 15
N_SEMS = SEM_FFN + 3 * NSEG


def _bf(x):
    return x.astype(BF16).astype(F32)


def _phi(t):
    return jnp.where(t > 0, t + 1.0, jnp.exp(t))


def _max_col_sq(w32):
    return jnp.max(jnp.sum(w32 * w32, axis=0, keepdims=True))


def _rows_padded(a, start, rows):
    stop = min(start + rows, a.shape[0])
    part = a[start:stop]
    if stop - start < rows:
        part = jnp.concatenate([part, jnp.zeros((rows - (stop - start), a.shape[1]), a.dtype)], axis=0)
    return part


def _kernel(x_hbm, wq_hbm, wk_hbm, wv_hbm, wo_hbm, beta_hbm, wr_hbm, wg_hbm, wu_hbm, wd_hbm,
            out_hbm,
            xs, xn, wq, wk, wv, wo, beta, pin, wr, wt, wot, gtab, qts, kwin, pqt, pkwin, vts, mext, ot,
            outs, rbuf, yacc, xsel_ref, wg, wu, wd, sems):

    def seg_cols(s):
        if isinstance(s, int):
            return slice(s * L, (s + 1) * L)
        return pl.ds(pl.multiple_of(s * L, L), L)

    def x_copy(s):
        return pltpu.make_async_copy(x_hbm.at[:, seg_cols(s)], xs.at[:, seg_cols(s)], sems.at[SEM_X + s])

    def out_copy(s):
        return pltpu.make_async_copy(outs.at[:, seg_cols(s)], out_hbm.at[:, seg_cols(s)],
                                     sems.at[SEM_OUT + s])

    cp_wq = pltpu.make_async_copy(wq_hbm, wq, sems.at[SEM_WQ])
    cp_wk = pltpu.make_async_copy(wk_hbm, wk, sems.at[SEM_WK])
    cp_wv = pltpu.make_async_copy(wv_hbm, wv, sems.at[SEM_WV])
    cp_wo = pltpu.make_async_copy(wo_hbm, wo, sems.at[SEM_WO])

    def ffn_copies(s):
        if isinstance(s, int):
            cols = slice(s * FC, (s + 1) * FC)
        else:
            cols = pl.ds(pl.multiple_of(s * FC, 128), FC)
        return [pltpu.make_async_copy(src.at[:, cols], dst.at[:, cols], sems.at[SEM_FFN + 3 * s + k])
                for k, (src, dst) in enumerate(((wg_hbm, wg), (wu_hbm, wu), (wd_hbm, wd)))]

    cp_beta = pltpu.make_async_copy(beta_hbm, beta, sems.at[SEM_BETA])
    cp_wr = pltpu.make_async_copy(wr_hbm, wr, sems.at[SEM_WR])
    pin_copy = pltpu.make_async_copy(beta_hbm, pin, sems.at[SEM_PIN])

    def transposed(w_ref):
        w32 = w_ref[...].astype(F32)
        return w32.T.astype(BF16), _max_col_sq(w32)

    def layernorm(s):
        x32 = xs[:, seg_cols(s)].astype(F32)
        mean = jnp.sum(x32, axis=0, keepdims=True) / D
        mean_b = _bf(mean)
        cen = x32 - mean_b
        shift = mean - mean_b
        var = jnp.sum(cen * cen, axis=0, keepdims=True) / D - shift * shift
        den = _bf(jnp.sqrt(_bf(_bf(var) + _bf(jnp.float32(1e-5)))))
        xn[:, seg_cols(s)] = (_bf(cen) * (1.0 / den)).astype(BF16)

    def proj_q(s, g0, g1):
        q = jnp.dot(wt[GD * g0:GD * g1, :], xn[:, seg_cols(s)], preferred_element_type=F32)
        qts[s, GD * g0:GD * g1, :] = q * QSCALE
        pq = _phi(q)
        pad = jnp.zeros((KP - GD, L), F32)
        for g in range(g0, g1):
            win = jnp.concatenate([pq[GD * (g - g0):GD * (g - g0 + 1)], pad], axis=0)
            pqt[s, g] = win.astype(BF16)

    def proj_k(s):
        k = jnp.dot(wt[D:2 * D, :], xn[:, seg_cols(s)], preferred_element_type=F32)
        for g in range(NG):
            kw = _rows_padded(k, GD * g, 128).T
            kwin[s, g] = kw.astype(BF16)
            pkwin[s, g] = _phi(kw).astype(BF16)

    def proj_v(s):
        v = jnp.dot(wt[2 * D:WROWS, :], xn[:, seg_cols(s)], preferred_element_type=F32)
        for j in range(QT):
            rbuf[s * QT + j:s * QT + j + 1, :] = _bf(v[D:D + 1, 128 * j:128 * (j + 1)])
        hrow = lax.broadcasted_iota(jnp.int32, (HS, L), 0)
        fill = jnp.where(hrow == DH, 1.0, 0.0)
        for h in range(H):
            g, hh = divmod(h, 4)
            vts[s, g, HS * hh:HS * (hh + 1), :] = jnp.where(
                hrow < DH, v[DH * h:DH * h + HS], fill)

    def tile_of(idx):
        return pl.ds(pl.multiple_of((idx // 128) * 128, 128), 128)

    def router():
        r = rbuf[...]
        tok = (lax.broadcasted_iota(jnp.int32, r.shape, 0) * 128
               + lax.broadcasted_iota(jnp.int32, r.shape, 1))
        r1 = jnp.max(r)
        i1 = jnp.min(jnp.where(r == r1, tok, S))
        rm = jnp.where(tok == i1, -jnp.inf, r)
        r2 = jnp.max(rm)
        i2 = jnp.min(jnp.where((rm == r2) & (tok != i1), tok, S))
        i1 = jnp.minimum(i1, S - 1)
        i2 = jnp.minimum(i2, S - 1)
        row8 = lax.broadcasted_iota(jnp.int32, (8, 128), 0)
        lane8 = lax.broadcasted_iota(jnp.int32, (8, 128), 1)
        hot1 = jnp.where((row8 == 0) & (lane8 == i1 % 128), 1.0, 0.0)
        hot2 = jnp.where((row8 == 1) & (lane8 == i2 % 128), 1.0, 0.0)
        return r1, r2, i1, i2, hot1, hot2

    x_copy(0).start()
    cp_wq.start()
    cp_wr.start()
    cp_beta.start()
    pin_copy.start()
    mext[...] = jnp.zeros(mext.shape, F32)
    yacc[...] = jnp.zeros(yacc.shape, F32)
    x_copy(0).wait()
    cp_wv.start()
    cp_wk.start()
    layernorm(0)
    cp_wq.wait()
    for s in range(1, NSEG):
        x_copy(s).start()
    cp_wo.start()
    for s in range(NSEG):
        for cp in ffn_copies(s):
            cp.start()
    cp_wr.wait()
    wt[0:D, :], nq = transposed(wq)
    proj_q(0, 0, NG // 2)
    cp_wv.wait()
    cp_wk.wait()
    wt[2 * D:3 * D, :], nv = transposed(wv)
    row16 = lax.broadcasted_iota(jnp.int32, (16, D), 0)
    wt[3 * D:WROWS, :] = jnp.where(
        row16 == 0, wr[...].astype(F32).reshape(1, D), 0.0).astype(BF16)
    proj_q(0, NG // 2, NG)
    wt[D:2 * D, :], nk = transposed(wk)
    proj_v(0)
    for s in range(1, NSEG):
        x_copy(s).wait()
    cp_wo.wait()
    cp_beta.wait()
    layernorm(1)
    proj_k(0)
    for s in range(1, NSEG):
        if s == NSEG - 1:
            proj_v(s)
            r1, r2, i1, i2, hot1, hot2 = router()
            proj_k(s)
            proj_q(s, 0, NG)
            xsel_ref[...] = (
                lax.dot_general(hot1, xn[:, tile_of(i1)], NT, preferred_element_type=F32)
                + lax.dot_general(hot2, xn[:, tile_of(i2)], NT, preferred_element_type=F32))
            continue
        layernorm(s + 1)
        proj_q(s, 0, NG)
        if s == 1:
            wot[:, 0:D] = wo[...].astype(F32).T.astype(BF16)
            b = beta[...].astype(F32).reshape(1, H)
            bt = jnp.broadcast_to(
                jnp.concatenate([b, jnp.zeros((1, 128 - H), F32)], axis=1), (128, 128)).T
            gt_all = _bf(jax.nn.sigmoid(bt[0:H]))
            gtab[0] = gt_all
            gtab[1] = _bf(1.0 - gt_all)
            logit_bound = (DH * QSCALE * XN_SQ_BOUND) * jnp.sqrt(nq) * jnp.sqrt(nk)
            no_shift_needed = ((logit_bound <= SAFE_LOGIT_BOUND)
                               & (XN_SQ_BOUND * nv <= SAFE_VALUE_BOUND * SAFE_VALUE_BOUND))
        proj_k(s)
        proj_v(s)

    krow = lax.broadcasted_iota(jnp.int32, (128, 128), 0)
    kcol = lax.broadcasted_iota(jnp.int32, (128, 128), 1)
    causal = krow <= kcol

    def ffn_cols(u, n=1):
        if isinstance(u, int):
            return slice(u * 128, (u + n) * 128)
        return pl.ds(pl.multiple_of(u * 128, 128), n * 128)

    def ffn_up_part(u, n, lo, hi):
        w2 = jnp.concatenate([wg[lo:hi, ffn_cols(u, n)], wu[lo:hi, ffn_cols(u, n)]], axis=1)
        return jnp.dot(xsel_ref[:, lo:hi], w2, preferred_element_type=F32)

    def ffn_act(gu):
        n = gu.shape[1] // 2
        gate = _bf(gu[:, 0:n])
        return _bf(_bf(gate * jax.nn.sigmoid(gate)) * _bf(gu[:, n:]))

    def ffn_down_part(u, n, hid, lo, hi):
        yacc[:, lo:hi] += lax.dot_general(hid, wd[lo:hi, ffn_cols(u, n)], NT,
                                          preferred_element_type=F32)

    def ffn_items():
        st = {}

        def up(u, lo, hi):
            def run():
                part = ffn_up_part(u, 2, lo, hi)
                st[u] = part if lo == 0 else st[u] + part
                if hi == D:
                    st[u] = ffn_act(st[u])
            return run

        def down(u):
            return lambda: ffn_down_part(u, 1, st[u - u % 2][:, 128 * (u % 2):128 * (u % 2 + 1)], 0, 512)

        def down_tail(u):
            return lambda: ffn_down_part(
                u, 4, jnp.concatenate([st[u], st[u + 2]], axis=1), 512, D)

        bounds = [0, 128, 256, 384, 512, D]
        ups = lambda u: [up(u, bounds[k], bounds[k + 1]) for k in range(5)]
        downs = lambda u: [down(u + k) for k in range(4)] + [down_tail(u)]
        items = []
        for u in range(0, FU + 4, 4):
            if u < FU:
                items += [(f, u + 2) for f in ups(u)] + [(f, u + 4) for f in ups(u + 2)]
            if u > 0:
                items += [(f, u) for f in downs(u - 4)]
        return items + [(ffn_finish, FU)]

    def ffn_finish():
        rowd = lax.broadcasted_iota(jnp.int32, (8, D), 0)
        y = _bf(_bf(yacc[...]) * _bf(jax.nn.sigmoid(jnp.where(rowd == 0, r1, r2))))
        y = jnp.where(rowd < 2, y, 0.0)
        yt = jnp.concatenate([y, jnp.zeros((120, D), F32)], axis=0).T
        wot[:, D:DX] = yt[:, 0:DX - D].astype(BF16)

    def scatter_rows(s):
        row = lax.broadcasted_iota(jnp.int32, (DX - D, L), 0)
        tok = s * L + lax.broadcasted_iota(jnp.int32, (DX - D, L), 1)
        hit = ((row == 0) & (tok == i1)) | ((row == 1) & (tok == i2))
        return jnp.where(hit, 1.0, 0.0)

    def weight_tile(parts):
        blocks = []
        for b in range(KP // 8):
            row = 8 * b + lax.broadcasted_iota(jnp.int32, (8, 128), 0)
            lane = lax.broadcasted_iota(jnp.int32, (8, 128), 1)
            blk = jnp.zeros((8, 128), F32)
            for hh, vals, lo, hi in parts:
                r0, r1 = DH * hh, DH * hh + DH
                if r1 <= 8 * b or r0 >= 8 * b + 8:
                    continue
                keep = None
                for cond in ([row >= r0] if r0 > 8 * b else []) + ([row < r1] if r1 < 8 * b + 8 else []) \
                        + ([lane >= lo] if lo > 0 else []) + ([lane < hi] if hi < 128 else []):
                    keep = cond if keep is None else keep & cond
                v = vals[8 * b:8 * b + 8]
                blk = v if keep is None else jnp.where(keep, v, blk)
            blocks.append(blk)
        return jnp.concatenate(blocks, axis=0).astype(BF16)

    def stage_fns(s, g, g_rows, ret):
        def qk_safe(i):
            q = qts[s, g_rows, 128 * i:128 * (i + 1)]
            qm = jnp.concatenate([weight_tile([(hh, q, 0, 128)]) for hh in range(4)], axis=1)
            nk = 128 * (i + 1)
            st = jnp.dot(kwin[s, g, 0:nk, 0:KP], qm, preferred_element_type=F32)
            ps = []
            for hh in range(4):
                sc = st[:, 128 * hh:128 * (hh + 1)]
                diag = jnp.where(causal, sc[nk - 128:], -1e30)
                sc = jnp.concatenate([sc[:nk - 128], diag], axis=0) if i > 0 else diag
                sc = sc - jnp.max(sc, axis=0, keepdims=True)
                ps.append(jnp.exp2(sc).astype(BF16))
            return ps

        qk = qk_safe

        def pv(i, ps):
            nk = 128 * (i + 1)
            for hh in range(4):
                v = vts[s, g, HS * hh:HS * (hh + 1), 0:nk]
                combine(s, g, ret, i, hh, jnp.dot(v, ps[hh], preferred_element_type=F32))
        return qk, pv

    def combine(s, g, ret, i, hh, o):
        h = 4 * g + hh
        res = o * (gtab[1, pl.ds(h, 1), :] / o[DH:DH + 1])
        if ret is not None:
            mem = ret[HS * hh:HS * (hh + 1), 128 * i:128 * (i + 1)]
            res = res + mem * (gtab[0, pl.ds(h, 1), :] / (mem[DH:DH + 1] + 1e-6))
        ot[s, i, pl.ds(DH * h, HS), :] = res

    def qk_items(s, g, i):
        q = qts[s, GD * g:GD * (g + 1), 128 * i:128 * (i + 1)]
        base = 128 * i
        blocks = {}
        st = {}

        def scores(lo, hi, w):
            return jnp.exp2(jnp.dot(kwin[s, g, lo:hi, 0:KP], w, preferred_element_type=F32))

        tile = lambda e, t: e[:, 128 * t:128 * (t + 1)]
        roll = lambda e, t: pltpu.roll(e, t, 1)
        qm = jnp.concatenate([weight_tile([(hh, q, 0, 128)]) for hh in range(4)], axis=1)

        def full(j):
            def run():
                last = j == i - 1
                e = scores(128 * j, 128 * (j + 1) + (32 if last else 0), qm)
                blocks[j] = [tile(e, hh)[0:128].astype(BF16) for hh in range(4)]
                if last:
                    st[0] = e[128:160]
            return run

        def d0():
            st[0] = scores(0, 32, qm)

        def d1():
            st['q'] = [roll(q, t) for t in (32, 64, 96)]
            q32, q64, q96 = st['q']
            st[1] = scores(base + 32, base + 64, jnp.concatenate([
                weight_tile([(0, q, 32, 128), (3, q96, 0, 32)]),
                weight_tile([(1, q, 32, 128), (3, q64, 0, 32)]),
                weight_tile([(2, q, 32, 128), (3, q32, 0, 32)])], axis=1))

        def d2():
            q32, q64, q96 = st['q']
            st[2] = scores(base + 64, base + 96, jnp.concatenate([
                weight_tile([(0, q, 64, 128), (2, q64, 0, 64)]),
                weight_tile([(1, q, 64, 128), (3, q64, 0, 64)])], axis=1))

        def d3():
            q32, q64, q96 = st['q']
            e3 = scores(base + 96, base + 128,
                        weight_tile([(0, q, 96, 128), (1, q96, 64, 96), (2, q64, 32, 64), (3, q32, 0, 32)]))
            e0, e1, e2 = st[0], st[1], st[2]
            lane = lax.broadcasted_iota(jnp.int32, (32, 128), 1)
            blk1 = [tile(e1, 0), tile(e1, 1), tile(e1, 2),
                    jnp.where(lane < 64, roll(tile(e1, 0), 32),
                              jnp.where(lane < 96, roll(tile(e1, 1), 64), roll(tile(e1, 2), 96)))]
            blk2 = [tile(e2, 0), tile(e2, 1), roll(tile(e2, 0), 64), roll(tile(e2, 1), 64)]
            blk3 = [e3, roll(e3, 32), roll(e3, 64), roll(e3, 96)]
            blocks[i] = [
                jnp.where(causal, jnp.concatenate([tile(e0, hh), blk1[hh], blk2[hh], blk3[hh]], axis=0),
                          0.0).astype(BF16) for hh in range(4)]

        items = [full(j) for j in range(i)] + ([d0] if i == 0 else []) + [d1, d2, d3]
        return items, blocks

    def pv_items(s, g, i, rets, blocks):
        acc = {}

        def block(j):
            def run():
                for hh in range(4):
                    v = vts[s, g, HS * hh:HS * (hh + 1), 128 * j:128 * (j + 1)]
                    o = jnp.dot(v, blocks[j][hh], preferred_element_type=F32)
                    acc[hh] = o if j == 0 else acc[hh] + o
                    if j == i:
                        combine(s, g, rets[g], i, hh, acc[hh])
            return run
        return [block(j) for j in range(i + 1)]

    def mem_read(s, g):
        return jnp.dot(mext[g][:, 0:KP], pqt[s, g], preferred_element_type=F32)

    def mem_update(s, g):
        upd = jnp.dot(vts[s, g], pkwin[s, g], preferred_element_type=F32)
        row = lax.broadcasted_iota(jnp.int32, (4 * HS, 128), 0)
        lane = lax.broadcasted_iota(jnp.int32, (4 * HS, 128), 1)
        lo = (row // HS) * DH
        mext[g] = mext[g] + jnp.where((lane >= lo) & (lane < lo + DH), upd, 0.0)

    def wo_part(s, lo, hi):
        rows = min(hi, D)
        otb = jnp.concatenate([ot[s, i, lo:rows, :] for i in range(QT)], axis=1)
        if hi > D:
            otb = jnp.concatenate([otb, scatter_rows(s)], axis=0)
        return jnp.dot(wot[:, lo:hi], otb.astype(BF16), preferred_element_type=F32)

    def finish(s, att):
        cols = seg_cols(s)
        res = xs[:, cols].astype(F32) + att + xn[:, cols].astype(F32)
        outs[:, cols] = res.astype(BF16)

    def attention_fast(s, ffn, ffn_tiles_ready):
        pending = []
        rets = {}

        def extra():
            if ffn:
                f, needs = ffn.pop(0)
                assert needs <= ffn_tiles_ready
                f()

        for g in range(NG):
            rets[g] = None
            for i in range(QT):
                items, blocks = qk_items(s, g, i)
                for n in range(len(items)):
                    items[n]()
                    if n < len(pending) - 1:
                        pending[n]()
                    if n < i:
                        extra()
                    if (i, n) == (0, 1) and s > 0:
                        rets[g] = mem_read(s, g)
                        extra()
                    if (i, n) == (0, 3) and s < NSEG - 1:
                        mem_update(s, g)
                        extra()
                if pending:
                    pending[-1]()
                pending = pv_items(s, g, i, rets, blocks)
        return pending

    def wait_ffn_weights(lo, hi):
        for c in range(lo, hi):
            for cp in ffn_copies(c):
                cp.wait()

    KS = 384

    def main_fast():
        ffn = ffn_items()
        for s in range(NSEG - 1):
            for f in attention_fast(s, ffn, FU // 2 if s == 0 else FU):
                f()
            if s == 0:
                wait_ffn_weights(2, NSEG)
        assert not ffn
        for s in range(NSEG - 1):
            finish(s, wo_part(s, 0, DX))
        for s in range(NSEG - 1):
            out_copy(s).start()
        pin_copy.wait()
        pending = attention_fast(NSEG - 1, [], FU)
        att = wo_part(NSEG - 1, 0, KS)
        for f in pending:
            f()
        finish(NSEG - 1, att + wo_part(NSEG - 1, KS, DX))

    def main_safe():
        wait_ffn_weights(2, NSEG)

        def segment(s, carry):
            def body(g, c):
                g_rows = pl.ds(pl.multiple_of(GD * g, 8), GD)
                qk, pv = stage_fns(s, g, g_rows, mem_read(s, g))
                mem_update(s, g)
                for i in range(QT):
                    pv(i, qk(i))
                return c
            return lax.fori_loop(0, NG, body, carry)
        lax.fori_loop(0, NSEG, segment, 0)

        def ffn_body(u, c):
            ffn_down_part(u, 1, ffn_act(ffn_up_part(u, 1, 0, D)), 0, D)
            return c
        lax.fori_loop(0, FU, ffn_body, 0)
        ffn_finish()

        def project(s, c):
            finish(s, wo_part(s, 0, DX))
            return c
        lax.fori_loop(0, NSEG, project, 0)
        for s in range(NSEG - 1):
            out_copy(s).start()
        pin_copy.wait()

    wait_ffn_weights(0, 2)
    lax.cond(no_shift_needed, main_fast, main_safe)
    out_copy(NSEG - 1).start()
    for s in range(NSEG):
        out_copy(s).wait()


@jax.jit
def pallas_parallel_sum__memory_aug_infini_attn__moe_arch_mod__prompt_kernel(
    A_x: jax.Array,
    A_wq: jax.Array,
    A_wk: jax.Array,
    A_wv: jax.Array,
    A_wo: jax.Array,
    A_beta: jax.Array,
    B_x: jax.Array,
    B_w_r: jax.Array,
    B_w_gate: jax.Array,
    B_w_up: jax.Array,
    B_w_down: jax.Array,
):
    del B_x
    xt = A_x.reshape(S, D).T
    wdt = B_w_down.T
    hbm = pl.BlockSpec(memory_space=pltpu.HBM)
    out = pl.pallas_call(
        _kernel,
        out_shape=jax.ShapeDtypeStruct((D, S), BF16),
        in_specs=[hbm] * 10,
        out_specs=hbm,
        scratch_shapes=[
            pltpu.VMEM((D, S), BF16),
            pltpu.VMEM((D, S), BF16),
            pltpu.VMEM((D, D), BF16),
            pltpu.VMEM((D, D), BF16),
            pltpu.VMEM((D, D), BF16),
            pltpu.VMEM((D, D), BF16),
            pltpu.VMEM((H,), BF16),
            pltpu.VMEM((H,), BF16),
            pltpu.VMEM((D,), BF16),
            pltpu.VMEM((WROWS, D), BF16),
            pltpu.VMEM((D, DX), BF16),
            pltpu.VMEM((2, H, 128), F32),
            pltpu.VMEM((NSEG, D, L), F32),
            pltpu.VMEM((NSEG, NG, L, 128), BF16),
            pltpu.VMEM((NSEG, NG, KP, L), BF16),
            pltpu.VMEM((NSEG, NG, L, 128), BF16),
            pltpu.VMEM((NSEG, NG, 4 * HS, L), F32),
            pltpu.VMEM((NG, 4 * HS, 128), F32),
            pltpu.VMEM((NSEG, QT, D + 24, 128), F32),
            pltpu.VMEM((D, S), BF16),
            pltpu.VMEM((NSEG * QT, 128), F32),
            pltpu.VMEM((8, D), F32),
            pltpu.VMEM((8, D), F32),
            pltpu.VMEM((D, F), BF16),
            pltpu.VMEM((D, F), BF16),
            pltpu.VMEM((D, F), BF16),
            pltpu.SemaphoreType.DMA((N_SEMS,)),
        ],
        compiler_params=pltpu.CompilerParams(vmem_limit_bytes=110 * 1024 * 1024),
    )(xt, A_wq, A_wk, A_wv, A_wo, A_beta, B_w_r, B_w_gate, B_w_up, wdt)
    return out.T.reshape(1, S, D)
```

```python
import math

import jax
import jax.numpy as jnp
from jax import lax
import jax.experimental.pallas as pl
import jax.experimental.pallas.tpu as pltpu

S = 2048
D = 576
H = 32
DH = 18
NSEG = 4
L = S // NSEG
F = 4608
NG = 8
GD = 4 * DH
HS = 24
QT = L // 128
WROWS = 3 * D + 16
FU = F // 128
FC = F // NSEG
DX = D + 16
KP = 80

F32 = jnp.float32
BF16 = jnp.bfloat16
QSCALE = (DH ** -0.5) * math.log2(math.e)
SAFE_LOGIT_BOUND = 60.0
SAFE_VALUE_BOUND = 2.0 ** 40
XN_SQ_BOUND = 2.0 * D * 1.1

NT = (((1,), (1,)), ((), ()))

(SEM_X, SEM_WQ, SEM_WK, SEM_WV, SEM_WO, SEM_BETA, SEM_WR,
 SEM_OUT, SEM_PIN, SEM_FFN) = 0, 4, 5, 6, 7, 8, 9, 10, 14, 15
N_SEMS = SEM_FFN + 3 * NSEG


def _bf(x):
    return x.astype(BF16).astype(F32)


def _phi(t):
    return jnp.where(t > 0, t + 1.0, jnp.exp(t))


def _max_col_sq(w32):
    return jnp.max(jnp.sum(w32 * w32, axis=0, keepdims=True))


def _rows_padded(a, start, rows):
    stop = min(start + rows, a.shape[0])
    part = a[start:stop]
    if stop - start < rows:
        part = jnp.concatenate([part, jnp.zeros((rows - (stop - start), a.shape[1]), a.dtype)], axis=0)
    return part


def _kernel(x_hbm, wq_hbm, wk_hbm, wv_hbm, wo_hbm, beta_hbm, wr_hbm, wg_hbm, wu_hbm, wd_hbm,
            out_hbm,
            xs, xn, wq, wk, wv, wo, beta, pin, wr, wt, wot, gtab, qts, kwin, pqt, pkwin, vts, mext, ot,
            outs, rbuf, yacc, xsel_ref, wg, wu, wd, sems):

    def seg_cols(s):
        if isinstance(s, int):
            return slice(s * L, (s + 1) * L)
        return pl.ds(pl.multiple_of(s * L, L), L)

    def x_copy(s):
        return pltpu.make_async_copy(x_hbm.at[:, seg_cols(s)], xs.at[:, seg_cols(s)], sems.at[SEM_X + s])

    def out_copy(s):
        return pltpu.make_async_copy(outs.at[:, seg_cols(s)], out_hbm.at[:, seg_cols(s)],
                                     sems.at[SEM_OUT + s])

    cp_wq = pltpu.make_async_copy(wq_hbm, wq, sems.at[SEM_WQ])
    cp_wk = pltpu.make_async_copy(wk_hbm, wk, sems.at[SEM_WK])
    cp_wv = pltpu.make_async_copy(wv_hbm, wv, sems.at[SEM_WV])
    cp_wo = pltpu.make_async_copy(wo_hbm, wo, sems.at[SEM_WO])

    def ffn_copies(s):
        if isinstance(s, int):
            cols = slice(s * FC, (s + 1) * FC)
        else:
            cols = pl.ds(pl.multiple_of(s * FC, 128), FC)
        return [pltpu.make_async_copy(src.at[:, cols], dst.at[:, cols], sems.at[SEM_FFN + 3 * s + k])
                for k, (src, dst) in enumerate(((wg_hbm, wg), (wu_hbm, wu), (wd_hbm, wd)))]

    cp_beta = pltpu.make_async_copy(beta_hbm, beta, sems.at[SEM_BETA])
    cp_wr = pltpu.make_async_copy(wr_hbm, wr, sems.at[SEM_WR])
    pin_copy = pltpu.make_async_copy(beta_hbm, pin, sems.at[SEM_PIN])

    def transposed(w_ref):
        w32 = w_ref[...].astype(F32)
        return w32.T.astype(BF16), _max_col_sq(w32)

    def layernorm(s):
        x32 = xs[:, seg_cols(s)].astype(F32)
        mean = jnp.sum(x32, axis=0, keepdims=True) / D
        mean_b = _bf(mean)
        cen = x32 - mean_b
        shift = mean - mean_b
        var = jnp.sum(cen * cen, axis=0, keepdims=True) / D - shift * shift
        den = _bf(jnp.sqrt(_bf(_bf(var) + _bf(jnp.float32(1e-5)))))
        xn[:, seg_cols(s)] = (_bf(cen) * (1.0 / den)).astype(BF16)

    def proj_q(s, g0, g1):
        q = jnp.dot(wt[GD * g0:GD * g1, :], xn[:, seg_cols(s)], preferred_element_type=F32)
        qts[s, GD * g0:GD * g1, :] = q * QSCALE
        pq = _phi(q)
        pad = jnp.zeros((KP - GD, L), F32)
        for g in range(g0, g1):
            win = jnp.concatenate([pq[GD * (g - g0):GD * (g - g0 + 1)], pad], axis=0)
            pqt[s, g] = win.astype(BF16)

    def proj_k(s):
        k = jnp.dot(wt[D:2 * D, :], xn[:, seg_cols(s)], preferred_element_type=F32)
        for g in range(NG):
            kw = _rows_padded(k, GD * g, 128).T
            kwin[s, g] = kw.astype(BF16)
            pkwin[s, g] = _phi(kw).astype(BF16)

    def proj_v(s):
        v = jnp.dot(wt[2 * D:WROWS, :], xn[:, seg_cols(s)], preferred_element_type=F32)
        for j in range(QT):
            rbuf[s * QT + j:s * QT + j + 1, :] = _bf(v[D:D + 1, 128 * j:128 * (j + 1)])
        hrow = lax.broadcasted_iota(jnp.int32, (HS, L), 0)
        fill = jnp.where(hrow == DH, 1.0, 0.0)
        for h in range(H):
            g, hh = divmod(h, 4)
            vts[s, g, HS * hh:HS * (hh + 1), :] = jnp.where(
                hrow < DH, v[DH * h:DH * h + HS], fill)

    def tile_of(idx):
        return pl.ds(pl.multiple_of((idx // 128) * 128, 128), 128)

    def router():
        r = rbuf[...]
        tok = (lax.broadcasted_iota(jnp.int32, r.shape, 0) * 128
               + lax.broadcasted_iota(jnp.int32, r.shape, 1))
        r1 = jnp.max(r)
        i1 = jnp.min(jnp.where(r == r1, tok, S))
        rm = jnp.where(tok == i1, -jnp.inf, r)
        r2 = jnp.max(rm)
        i2 = jnp.min(jnp.where((rm == r2) & (tok != i1), tok, S))
        i1 = jnp.minimum(i1, S - 1)
        i2 = jnp.minimum(i2, S - 1)
        row8 = lax.broadcasted_iota(jnp.int32, (8, 128), 0)
        lane8 = lax.broadcasted_iota(jnp.int32, (8, 128), 1)
        hot1 = jnp.where((row8 == 0) & (lane8 == i1 % 128), 1.0, 0.0)
        hot2 = jnp.where((row8 == 1) & (lane8 == i2 % 128), 1.0, 0.0)
        return r1, r2, i1, i2, hot1, hot2

    x_copy(0).start()
    cp_wr.start()
    cp_beta.start()
    pin_copy.start()
    cp_wq.start()
    mext[...] = jnp.zeros(mext.shape, F32)
    yacc[...] = jnp.zeros(yacc.shape, F32)
    x_copy(0).wait()
    x_copy(1).start()
    cp_wv.start()
    cp_wk.start()
    cp_wr.wait()
    layernorm(0)
    cp_wq.wait()
    wt[0:D, :], nq = transposed(wq)
    proj_q(0, 0, NG // 2)
    x_copy(1).wait()
    proj_q(0, NG // 2, NG)
    layernorm(1)
    cp_wv.wait()
    wt[2 * D:3 * D, :], nv = transposed(wv)
    row16 = lax.broadcasted_iota(jnp.int32, (16, D), 0)
    wt[3 * D:WROWS, :] = jnp.where(
        row16 == 0, wr[...].astype(F32).reshape(1, D), 0.0).astype(BF16)
    cp_wk.wait()
    x_copy(2).start()
    x_copy(3).start()
    cp_wo.start()
    for s in range(NSEG):
        for cp in ffn_copies(s):
            cp.start()
    cp_beta.wait()
    proj_q(1, 0, NG)
    wt[D:2 * D, :], nk = transposed(wk)
    x_copy(2).wait()
    x_copy(3).wait()
    proj_v(0)
    proj_k(0)
    layernorm(2)
    layernorm(3)
    cp_wo.wait()
    for s in range(1, NSEG):
        proj_v(s)
    r1, r2, i1, i2, hot1, hot2 = router()
    wot[:, 0:D] = wo[...].astype(F32).T.astype(BF16)
    b = beta[...].astype(F32).reshape(1, H)
    bt = jnp.broadcast_to(
        jnp.concatenate([b, jnp.zeros((1, 128 - H), F32)], axis=1), (128, 128)).T
    gt_all = _bf(jax.nn.sigmoid(bt[0:H]))
    gtab[0] = gt_all
    gtab[1] = _bf(1.0 - gt_all)
    logit_bound = (DH * QSCALE * XN_SQ_BOUND) * jnp.sqrt(nq) * jnp.sqrt(nk)
    no_shift_needed = ((logit_bound <= SAFE_LOGIT_BOUND)
                       & (XN_SQ_BOUND * nv <= SAFE_VALUE_BOUND * SAFE_VALUE_BOUND))
    for s in range(1, NSEG):
        proj_k(s)
    for s in range(2, NSEG):
        proj_q(s, 0, NG)
    xsel_ref[...] = (
        lax.dot_general(hot1, xn[:, tile_of(i1)], NT, preferred_element_type=F32)
        + lax.dot_general(hot2, xn[:, tile_of(i2)], NT, preferred_element_type=F32))

    krow = lax.broadcasted_iota(jnp.int32, (128, 128), 0)
    kcol = lax.broadcasted_iota(jnp.int32, (128, 128), 1)
    causal = krow <= kcol

    def ffn_cols(u, n=1):
        if isinstance(u, int):
            return slice(u * 128, (u + n) * 128)
        return pl.ds(pl.multiple_of(u * 128, 128), n * 128)

    def ffn_up_part(u, n, lo, hi):
        w2 = jnp.concatenate([wg[lo:hi, ffn_cols(u, n)], wu[lo:hi, ffn_cols(u, n)]], axis=1)
        return jnp.dot(xsel_ref[:, lo:hi], w2, preferred_element_type=F32)

    def ffn_act(gu):
        n = gu.shape[1] // 2
        gate = _bf(gu[:, 0:n])
        return _bf(_bf(gate * jax.nn.sigmoid(gate)) * _bf(gu[:, n:]))

    def ffn_down_part(u, n, hid, lo, hi):
        yacc[:, lo:hi] += lax.dot_general(hid, wd[lo:hi, ffn_cols(u, n)], NT,
                                          preferred_element_type=F32)

    def ffn_items():
        st = {}

        def up(u, lo, hi):
            def run():
                part = ffn_up_part(u, 2, lo, hi)
                st[u] = part if lo == 0 else st[u] + part
                if hi == D:
                    st[u] = ffn_act(st[u])
            return run

        def down(u):
            return lambda: ffn_down_part(u, 1, st[u - u % 2][:, 128 * (u % 2):128 * (u % 2 + 1)], 0, 512)

        def down_tail(u):
            return lambda: ffn_down_part(
                u, 4, jnp.concatenate([st[u], st[u + 2]], axis=1), 512, D)

        bounds = [0, 128, 256, 384, 512, D]
        ups = lambda u: [up(u, bounds[k], bounds[k + 1]) for k in range(5)]
        downs = lambda u: [down(u + k) for k in range(4)] + [down_tail(u)]
        items = []
        for u in range(0, FU + 4, 4):
            if u < FU:
                items += [(f, u + 2) for f in ups(u)] + [(f, u + 4) for f in ups(u + 2)]
            if u > 0:
                items += [(f, u) for f in downs(u - 4)]
        return items + [(ffn_finish, FU)]

    def ffn_finish():
        rowd = lax.broadcasted_iota(jnp.int32, (8, D), 0)
        y = _bf(_bf(yacc[...]) * _bf(jax.nn.sigmoid(jnp.where(rowd == 0, r1, r2))))
        y = jnp.where(rowd < 2, y, 0.0)
        yt = jnp.concatenate([y, jnp.zeros((120, D), F32)], axis=0).T
        wot[:, D:DX] = yt[:, 0:DX - D].astype(BF16)

    def scatter_rows(s):
        row = lax.broadcasted_iota(jnp.int32, (DX - D, L), 0)
        tok = s * L + lax.broadcasted_iota(jnp.int32, (DX - D, L), 1)
        hit = ((row == 0) & (tok == i1)) | ((row == 1) & (tok == i2))
        return jnp.where(hit, 1.0, 0.0)

    def weight_tile(parts):
        blocks = []
        for b in range(KP // 8):
            row = 8 * b + lax.broadcasted_iota(jnp.int32, (8, 128), 0)
            lane = lax.broadcasted_iota(jnp.int32, (8, 128), 1)
            blk = jnp.zeros((8, 128), F32)
            for hh, vals, lo, hi in parts:
                r0, r1 = DH * hh, DH * hh + DH
                if r1 <= 8 * b or r0 >= 8 * b + 8:
                    continue
                keep = None
                for cond in ([row >= r0] if r0 > 8 * b else []) + ([row < r1] if r1 < 8 * b + 8 else []) \
                        + ([lane >= lo] if lo > 0 else []) + ([lane < hi] if hi < 128 else []):
                    keep = cond if keep is None else keep & cond
                v = vals[8 * b:8 * b + 8]
                blk = v if keep is None else jnp.where(keep, v, blk)
            blocks.append(blk)
        return jnp.concatenate(blocks, axis=0).astype(BF16)

    def stage_fns(s, g, g_rows, ret):
        def qk_safe(i):
            q = qts[s, g_rows, 128 * i:128 * (i + 1)]
            qm = jnp.concatenate([weight_tile([(hh, q, 0, 128)]) for hh in range(4)], axis=1)
            nk = 128 * (i + 1)
            st = jnp.dot(kwin[s, g, 0:nk, 0:KP], qm, preferred_element_type=F32)
            ps = []
            for hh in range(4):
                sc = st[:, 128 * hh:128 * (hh + 1)]
                diag = jnp.where(causal, sc[nk - 128:], -1e30)
                sc = jnp.concatenate([sc[:nk - 128], diag], axis=0) if i > 0 else diag
                sc = sc - jnp.max(sc, axis=0, keepdims=True)
                ps.append(jnp.exp2(sc).astype(BF16))
            return ps

        qk = qk_safe

        def pv(i, ps):
            nk = 128 * (i + 1)
            for hh in range(4):
                v = vts[s, g, HS * hh:HS * (hh + 1), 0:nk]
                combine(s, g, ret, i, hh, jnp.dot(v, ps[hh], preferred_element_type=F32))
        return qk, pv

    def combine(s, g, ret, i, hh, o):
        h = 4 * g + hh
        res = o * (gtab[1, pl.ds(h, 1), :] / o[DH:DH + 1])
        if ret is not None:
            mem = ret[DH * hh:DH * hh + HS, 128 * i:128 * (i + 1)]
            den = ret[GD + hh:GD + hh + 1, 128 * i:128 * (i + 1)]
            res = res + mem * (gtab[0, pl.ds(h, 1), :] / (den + 1e-6))
        ot[s, i, pl.ds(DH * h, HS), :] = res

    def qk_items(s, g, i):
        q = qts[s, GD * g:GD * (g + 1), 128 * i:128 * (i + 1)]
        base = 128 * i
        blocks = {}
        st = {}

        def scores(lo, hi, w):
            return jnp.exp2(jnp.dot(kwin[s, g, lo:hi, 0:KP], w, preferred_element_type=F32))

        tile = lambda e, t: e[:, 128 * t:128 * (t + 1)]
        roll = lambda e, t: pltpu.roll(e, t, 1)
        qm = jnp.concatenate([weight_tile([(hh, q, 0, 128)]) for hh in range(4)], axis=1)

        def full(j):
            def run():
                last = j == i - 1
                e = scores(128 * j, 128 * (j + 1) + (32 if last else 0), qm)
                blocks[j] = [tile(e, hh)[0:128].astype(BF16) for hh in range(4)]
                if last:
                    st[0] = e[128:160]
            return run

        def d0():
            st[0] = scores(0, 32, qm)

        def d1():
            st['q'] = [roll(q, t) for t in (32, 64, 96)]
            q32, q64, q96 = st['q']
            st[1] = scores(base + 32, base + 64, jnp.concatenate([
                weight_tile([(0, q, 32, 128), (3, q96, 0, 32)]),
                weight_tile([(1, q, 32, 128), (3, q64, 0, 32)]),
                weight_tile([(2, q, 32, 128), (3, q32, 0, 32)])], axis=1))

        def d2():
            q32, q64, q96 = st['q']
            st[2] = scores(base + 64, base + 96, jnp.concatenate([
                weight_tile([(0, q, 64, 128), (2, q64, 0, 64)]),
                weight_tile([(1, q, 64, 128), (3, q64, 0, 64)])], axis=1))

        def d3():
            q32, q64, q96 = st['q']
            e3 = scores(base + 96, base + 128,
                        weight_tile([(0, q, 96, 128), (1, q96, 64, 96), (2, q64, 32, 64), (3, q32, 0, 32)]))
            e0, e1, e2 = st[0], st[1], st[2]
            lane = lax.broadcasted_iota(jnp.int32, (32, 128), 1)
            blk1 = [tile(e1, 0), tile(e1, 1), tile(e1, 2),
                    jnp.where(lane < 64, roll(tile(e1, 0), 32),
                              jnp.where(lane < 96, roll(tile(e1, 1), 64), roll(tile(e1, 2), 96)))]
            blk2 = [tile(e2, 0), tile(e2, 1), roll(tile(e2, 0), 64), roll(tile(e2, 1), 64)]
            blk3 = [e3, roll(e3, 32), roll(e3, 64), roll(e3, 96)]
            blocks[i] = [
                jnp.where(causal, jnp.concatenate([tile(e0, hh), blk1[hh], blk2[hh], blk3[hh]], axis=0),
                          0.0).astype(BF16) for hh in range(4)]

        items = [full(j) for j in range(i)] + ([d0] if i == 0 else []) + [d1, d2, d3]
        return items, blocks

    def pv_items(s, g, i, rets, blocks):
        acc = {}

        def block(j):
            def run():
                for hh in range(4):
                    v = vts[s, g, HS * hh:HS * (hh + 1), 128 * j:128 * (j + 1)]
                    o = jnp.dot(v, blocks[j][hh], preferred_element_type=F32)
                    acc[hh] = o if j == 0 else acc[hh] + o
                    if j == i:
                        combine(s, g, rets[g], i, hh, acc[hh])
            return run
        return [block(j) for j in range(i + 1)]

    def mem_read(s, g):
        return jnp.dot(mext[g][:, 0:KP], pqt[s, g], preferred_element_type=F32)

    def mem_update(s, g):
        tail = lax.broadcasted_iota(jnp.int32, (KP - GD, L), 0)
        lhs = jnp.concatenate([vts[s, g, HS * hh:HS * hh + DH, :] for hh in range(4)]
                              + [jnp.where(tail == 0, 1.0, 0.0)], axis=0)
        upd = jnp.dot(lhs, pkwin[s, g], preferred_element_type=F32)
        upd = jnp.concatenate(
            [upd[0:GD], jnp.broadcast_to(upd[GD:GD + 1], (KP - GD, 128))], axis=0)
        row = lax.broadcasted_iota(jnp.int32, (KP, 128), 0)
        lane = lax.broadcasted_iota(jnp.int32, (KP, 128), 1)
        head = jnp.where(row < GD, row // DH, row - GD)
        mext[g] = mext[g] + jnp.where((lane >= head * DH) & (lane < head * DH + DH) & (head < 4),
                                      upd, 0.0)

    def wo_part(s, lo, hi):
        rows = min(hi, D)
        otb = jnp.concatenate([ot[s, i, lo:rows, :] for i in range(QT)], axis=1)
        if hi > D:
            otb = jnp.concatenate([otb, scatter_rows(s)], axis=0)
        return jnp.dot(wot[:, lo:hi], otb.astype(BF16), preferred_element_type=F32)

    def finish(s, att):
        cols = seg_cols(s)
        res = xs[:, cols].astype(F32) + att + xn[:, cols].astype(F32)
        outs[:, cols] = res.astype(BF16)

    def attention_fast(s, ffn, ffn_tiles_ready):
        pending = []
        rets = {}

        def extra():
            if ffn:
                f, needs = ffn.pop(0)
                assert needs <= ffn_tiles_ready
                f()

        for g in range(NG):
            rets[g] = None
            for i in range(QT):
                items, blocks = qk_items(s, g, i)
                for n in range(len(items)):
                    items[n]()
                    if n < len(pending) - 1:
                        pending[n]()
                    if n < i:
                        extra()
                    if (i, n) == (3, 1) and s == 1:
                        extra()
                    if (i, n) == (0, 1 if s < NSEG - 1 else 3) and s > 0:
                        rets[g] = mem_read(s, g)
                    if (i, n) == (0, 3) and s < NSEG - 1:
                        mem_update(s, g)
                if pending:
                    pending[-1]()
                pending = pv_items(s, g, i, rets, blocks)
        return pending

    def wait_ffn_weights(lo, hi):
        for c in range(lo, hi):
            for cp in ffn_copies(c):
                cp.wait()

    KS = 384

    def main_fast():
        ffn = ffn_items()
        for s in range(NSEG - 1):
            for f in attention_fast(s, ffn, FU // 2 if s == 0 else FU):
                f()
            if s == 0:
                wait_ffn_weights(2, NSEG)
        assert not ffn
        for s in range(NSEG - 1):
            finish(s, wo_part(s, 0, DX))
        for s in range(NSEG - 1):
            out_copy(s).start()
        pin_copy.wait()
        pending = attention_fast(NSEG - 1, [], FU)
        att = wo_part(NSEG - 1, 0, KS)
        for f in pending:
            f()
        finish(NSEG - 1, att + wo_part(NSEG - 1, KS, DX))

    def main_safe():
        wait_ffn_weights(2, NSEG)

        def segment(s, carry):
            def body(g, c):
                g_rows = pl.ds(pl.multiple_of(GD * g, 8), GD)
                qk, pv = stage_fns(s, g, g_rows, mem_read(s, g))
                mem_update(s, g)
                for i in range(QT):
                    pv(i, qk(i))
                return c
            return lax.fori_loop(0, NG, body, carry)
        lax.fori_loop(0, NSEG, segment, 0)

        def ffn_body(u, c):
            ffn_down_part(u, 1, ffn_act(ffn_up_part(u, 1, 0, D)), 0, D)
            return c
        lax.fori_loop(0, FU, ffn_body, 0)
        ffn_finish()

        def project(s, c):
            finish(s, wo_part(s, 0, DX))
            return c
        lax.fori_loop(0, NSEG, project, 0)
        for s in range(NSEG - 1):
            out_copy(s).start()
        pin_copy.wait()

    wait_ffn_weights(0, 2)
    lax.cond(no_shift_needed, main_fast, main_safe)
    out_copy(NSEG - 1).start()
    for s in range(NSEG):
        out_copy(s).wait()


@jax.jit
def pallas_parallel_sum__memory_aug_infini_attn__moe_arch_mod__prompt_kernel(
    A_x: jax.Array,
    A_wq: jax.Array,
    A_wk: jax.Array,
    A_wv: jax.Array,
    A_wo: jax.Array,
    A_beta: jax.Array,
    B_x: jax.Array,
    B_w_r: jax.Array,
    B_w_gate: jax.Array,
    B_w_up: jax.Array,
    B_w_down: jax.Array,
):
    del B_x
    xt = A_x.reshape(S, D).T
    wdt = B_w_down.T
    hbm = pl.BlockSpec(memory_space=pltpu.HBM)
    out = pl.pallas_call(
        _kernel,
        out_shape=jax.ShapeDtypeStruct((D, S), BF16),
        in_specs=[hbm] * 10,
        out_specs=hbm,
        scratch_shapes=[
            pltpu.VMEM((D, S), BF16),
            pltpu.VMEM((D, S), BF16),
            pltpu.VMEM((D, D), BF16),
            pltpu.VMEM((D, D), BF16),
            pltpu.VMEM((D, D), BF16),
            pltpu.VMEM((D, D), BF16),
            pltpu.VMEM((H,), BF16),
            pltpu.VMEM((H,), BF16),
            pltpu.VMEM((D,), BF16),
            pltpu.VMEM((WROWS, D), BF16),
            pltpu.VMEM((D, DX), BF16),
            pltpu.VMEM((2, H, 128), F32),
            pltpu.VMEM((NSEG, D, L), F32),
            pltpu.VMEM((NSEG, NG, L, 128), BF16),
            pltpu.VMEM((NSEG, NG, KP, L), BF16),
            pltpu.VMEM((NSEG, NG, L, 128), BF16),
            pltpu.VMEM((NSEG, NG, 4 * HS, L), F32),
            pltpu.VMEM((NG, KP, 128), F32),
            pltpu.VMEM((NSEG, QT, D + 24, 128), F32),
            pltpu.VMEM((D, S), BF16),
            pltpu.VMEM((NSEG * QT, 128), F32),
            pltpu.VMEM((8, D), F32),
            pltpu.VMEM((8, D), F32),
            pltpu.VMEM((D, F), BF16),
            pltpu.VMEM((D, F), BF16),
            pltpu.VMEM((D, F), BF16),
            pltpu.SemaphoreType.DMA((N_SEMS,)),
        ],
        compiler_params=pltpu.CompilerParams(vmem_limit_bytes=110 * 1024 * 1024),
    )(xt, A_wq, A_wk, A_wv, A_wo, A_beta, B_w_r, B_w_gate, B_w_up, wdt)
    return out.T.reshape(1, S, D)
```

```python
import math

import jax
import jax.numpy as jnp
from jax import lax
import jax.experimental.pallas as pl
import jax.experimental.pallas.tpu as pltpu

S = 2048
D = 576
H = 32
DH = 18
NSEG = 4
L = S // NSEG
F = 4608
NG = 8
GD = 4 * DH
HS = 24
QT = L // 128
WROWS = 3 * D + 16
FU = F // 128
FC = F // NSEG
DX = D + 16
KP = 80

F32 = jnp.float32
BF16 = jnp.bfloat16
QSCALE = (DH ** -0.5) * math.log2(math.e)
SAFE_LOGIT_BOUND = 60.0
SAFE_VALUE_BOUND = 2.0 ** 40
XN_SQ_BOUND = 2.0 * D * 1.1

NT = (((1,), (1,)), ((), ()))

(SEM_X, SEM_WQ, SEM_WK, SEM_WV, SEM_WO, SEM_BETA, SEM_WR,
 SEM_OUT, SEM_FFN) = 0, 4, 5, 6, 7, 8, 9, 10, 14
N_SEMS = SEM_FFN + 3 * NSEG


def _bf(x):
    return x.astype(BF16).astype(F32)


def _phi(t):
    return jnp.where(t > 0, t + 1.0, jnp.exp(t))


def _max_col_sq(w32):
    return jnp.max(jnp.sum(w32 * w32, axis=0, keepdims=True))


def _rows_padded(a, start, rows):
    stop = min(start + rows, a.shape[0])
    part = a[start:stop]
    if stop - start < rows:
        part = jnp.concatenate([part, jnp.zeros((rows - (stop - start), a.shape[1]), a.dtype)], axis=0)
    return part


def _kernel(x_hbm, wq_hbm, wk_hbm, wv_hbm, wo_hbm, beta_hbm, wr_hbm, wg_hbm, wu_hbm, wd_hbm,
            out_hbm,
            xs, xn, wq, wk, wv, wo, beta, wr, wt, wot, gtab, qts, kwin, pqt, pkwin, vts, mext, ot,
            outs, rbuf, yacc, xsel_ref, wg, wu, wd, sems):

    def seg_cols(s):
        if isinstance(s, int):
            return slice(s * L, (s + 1) * L)
        return pl.ds(pl.multiple_of(s * L, L), L)

    def x_copy(s):
        return pltpu.make_async_copy(x_hbm.at[:, seg_cols(s)], xs.at[:, seg_cols(s)], sems.at[SEM_X + s])

    def out_copy(s):
        return pltpu.make_async_copy(outs.at[:, seg_cols(s)], out_hbm.at[:, seg_cols(s)],
                                     sems.at[SEM_OUT + s])

    cp_wq = pltpu.make_async_copy(wq_hbm, wq, sems.at[SEM_WQ])
    cp_wk = pltpu.make_async_copy(wk_hbm, wk, sems.at[SEM_WK])
    cp_wv = pltpu.make_async_copy(wv_hbm, wv, sems.at[SEM_WV])
    cp_wo = pltpu.make_async_copy(wo_hbm, wo, sems.at[SEM_WO])

    def ffn_copies(s):
        if isinstance(s, int):
            cols = slice(s * FC, (s + 1) * FC)
        else:
            cols = pl.ds(pl.multiple_of(s * FC, 128), FC)
        return [pltpu.make_async_copy(src.at[:, cols], dst.at[:, cols], sems.at[SEM_FFN + 3 * s + k])
                for k, (src, dst) in enumerate(((wg_hbm, wg), (wu_hbm, wu), (wd_hbm, wd)))]

    cp_beta = pltpu.make_async_copy(beta_hbm, beta, sems.at[SEM_BETA])
    cp_wr = pltpu.make_async_copy(wr_hbm, wr, sems.at[SEM_WR])

    def transposed(w_ref):
        w32 = w_ref[...].astype(F32)
        return w32.T.astype(BF16), _max_col_sq(w32)

    def layernorm(s):
        x32 = xs[:, seg_cols(s)].astype(F32)
        mean = jnp.sum(x32, axis=0, keepdims=True) / D
        mean_b = _bf(mean)
        cen = x32 - mean_b
        shift = mean - mean_b
        var = jnp.sum(cen * cen, axis=0, keepdims=True) / D - shift * shift
        den = _bf(jnp.sqrt(_bf(_bf(var) + _bf(jnp.float32(1e-5)))))
        xn[:, seg_cols(s)] = (_bf(cen) * (1.0 / den)).astype(BF16)

    def proj_q(s, g0, g1):
        q = jnp.dot(wt[GD * g0:GD * g1, :], xn[:, seg_cols(s)], preferred_element_type=F32)
        qts[s, GD * g0:GD * g1, :] = q * QSCALE
        pq = _phi(q)
        pad = jnp.zeros((KP - GD, L), F32)
        for g in range(g0, g1):
            win = jnp.concatenate([pq[GD * (g - g0):GD * (g - g0 + 1)], pad], axis=0)
            pqt[s, g] = win.astype(BF16)

    def proj_k(s):
        k = jnp.dot(wt[D:2 * D, :], xn[:, seg_cols(s)], preferred_element_type=F32)
        for g in range(NG):
            kw = _rows_padded(k, GD * g, 128).T
            kwin[s, g] = kw.astype(BF16)
            pkwin[s, g] = _phi(kw).astype(BF16)

    def proj_v(s):
        v = jnp.dot(wt[2 * D:WROWS, :], xn[:, seg_cols(s)], preferred_element_type=F32)
        for j in range(QT):
            rbuf[s * QT + j:s * QT + j + 1, :] = _bf(v[D:D + 1, 128 * j:128 * (j + 1)])
        hrow = lax.broadcasted_iota(jnp.int32, (HS, L), 0)
        fill = jnp.where(hrow == DH, 1.0, 0.0)
        for h in range(H):
            g, hh = divmod(h, 4)
            vts[s, g, HS * hh:HS * (hh + 1), :] = jnp.where(
                hrow < DH, v[DH * h:DH * h + HS], fill)

    def tile_of(idx):
        return pl.ds(pl.multiple_of((idx // 128) * 128, 128), 128)

    def router():
        r = rbuf[...]
        tok = (lax.broadcasted_iota(jnp.int32, r.shape, 0) * 128
               + lax.broadcasted_iota(jnp.int32, r.shape, 1))
        r1 = jnp.max(r)
        i1 = jnp.min(jnp.where(r == r1, tok, S))
        rm = jnp.where(tok == i1, -jnp.inf, r)
        r2 = jnp.max(rm)
        i2 = jnp.min(jnp.where((rm == r2) & (tok != i1), tok, S))
        i1 = jnp.minimum(i1, S - 1)
        i2 = jnp.minimum(i2, S - 1)
        row8 = lax.broadcasted_iota(jnp.int32, (8, 128), 0)
        lane8 = lax.broadcasted_iota(jnp.int32, (8, 128), 1)
        hot1 = jnp.where((row8 == 0) & (lane8 == i1 % 128), 1.0, 0.0)
        hot2 = jnp.where((row8 == 1) & (lane8 == i2 % 128), 1.0, 0.0)
        return r1, r2, i1, i2, hot1, hot2

    x_copy(0).start()
    cp_wr.start()
    cp_beta.start()
    cp_wq.start()
    mext[...] = jnp.zeros(mext.shape, F32)
    yacc[...] = jnp.zeros(yacc.shape, F32)
    x_copy(0).wait()
    x_copy(1).start()
    cp_wv.start()
    cp_wk.start()
    cp_wr.wait()
    layernorm(0)
    cp_wq.wait()
    wt[0:D, :], nq = transposed(wq)
    proj_q(0, 0, NG // 2)
    x_copy(1).wait()
    proj_q(0, NG // 2, NG)
    layernorm(1)
    cp_wv.wait()
    wt[2 * D:3 * D, :], nv = transposed(wv)
    row16 = lax.broadcasted_iota(jnp.int32, (16, D), 0)
    wt[3 * D:WROWS, :] = jnp.where(
        row16 == 0, wr[...].astype(F32).reshape(1, D), 0.0).astype(BF16)
    cp_wk.wait()
    x_copy(2).start()
    x_copy(3).start()
    cp_wo.start()
    for s in range(NSEG):
        for cp in ffn_copies(s):
            cp.start()
    cp_beta.wait()
    proj_q(1, 0, NG)
    wt[D:2 * D, :], nk = transposed(wk)
    x_copy(2).wait()
    x_copy(3).wait()
    proj_v(0)
    proj_k(0)
    layernorm(2)
    layernorm(3)
    cp_wo.wait()
    for s in range(1, NSEG):
        proj_v(s)
    r1, r2, i1, i2, hot1, hot2 = router()
    wot[:, 0:D] = wo[...].astype(F32).T.astype(BF16)
    b = beta[...].astype(F32).reshape(1, H)
    bt = jnp.broadcast_to(
        jnp.concatenate([b, jnp.zeros((1, 128 - H), F32)], axis=1), (128, 128)).T
    gt_all = _bf(jax.nn.sigmoid(bt[0:H]))
    gtab[0] = gt_all
    gtab[1] = _bf(1.0 - gt_all)
    logit_bound = (DH * QSCALE * XN_SQ_BOUND) * jnp.sqrt(nq) * jnp.sqrt(nk)
    no_shift_needed = ((logit_bound <= SAFE_LOGIT_BOUND)
                       & (XN_SQ_BOUND * nv <= SAFE_VALUE_BOUND * SAFE_VALUE_BOUND))
    for s in range(1, NSEG):
        proj_k(s)
    for s in range(2, NSEG):
        proj_q(s, 0, NG)
    xsel_ref[...] = (
        lax.dot_general(hot1, xn[:, tile_of(i1)], NT, preferred_element_type=F32)
        + lax.dot_general(hot2, xn[:, tile_of(i2)], NT, preferred_element_type=F32))

    krow = lax.broadcasted_iota(jnp.int32, (128, 128), 0)
    kcol = lax.broadcasted_iota(jnp.int32, (128, 128), 1)
    causal = krow <= kcol

    def ffn_cols(u, n=1):
        if isinstance(u, int):
            return slice(u * 128, (u + n) * 128)
        return pl.ds(pl.multiple_of(u * 128, 128), n * 128)

    def ffn_up_part(u, n, lo, hi):
        w2 = jnp.concatenate([wg[lo:hi, ffn_cols(u, n)], wu[lo:hi, ffn_cols(u, n)]], axis=1)
        return jnp.dot(xsel_ref[:, lo:hi], w2, preferred_element_type=F32)

    def ffn_act(gu):
        n = gu.shape[1] // 2
        gate = _bf(gu[:, 0:n])
        return _bf(_bf(gate * jax.nn.sigmoid(gate)) * _bf(gu[:, n:]))

    def ffn_down_part(u, n, hid, lo, hi):
        yacc[:, lo:hi] += lax.dot_general(hid, wd[lo:hi, ffn_cols(u, n)], NT,
                                          preferred_element_type=F32)

    def ffn_items():
        st = {}

        def up(u, lo, hi):
            def run():
                part = ffn_up_part(u, 2, lo, hi)
                st[u] = part if lo == 0 else st[u] + part
                if hi == D:
                    st[u] = ffn_act(st[u])
            return run

        def down(u):
            return lambda: ffn_down_part(u, 1, st[u - u % 2][:, 128 * (u % 2):128 * (u % 2 + 1)], 0, 512)

        def down_tail(u):
            return lambda: ffn_down_part(
                u, 4, jnp.concatenate([st[u], st[u + 2]], axis=1), 512, D)

        bounds = [0, 128, 256, 384, 512, D]
        ups = lambda u: [up(u, bounds[k], bounds[k + 1]) for k in range(5)]
        downs = lambda u: [down(u + k) for k in range(4)] + [down_tail(u)]
        items = []
        for u in range(0, FU + 4, 4):
            if u < FU:
                items += [(f, u + 2) for f in ups(u)] + [(f, u + 4) for f in ups(u + 2)]
            if u > 0:
                items += [(f, u) for f in downs(u - 4)]
        return items + [(ffn_finish, FU)]

    def ffn_finish():
        rowd = lax.broadcasted_iota(jnp.int32, (8, D), 0)
        y = _bf(_bf(yacc[...]) * _bf(jax.nn.sigmoid(jnp.where(rowd == 0, r1, r2))))
        y = jnp.where(rowd < 2, y, 0.0)
        yt = jnp.concatenate([y, jnp.zeros((120, D), F32)], axis=0).T
        wot[:, D:DX] = yt[:, 0:DX - D].astype(BF16)

    def scatter_rows(s):
        row = lax.broadcasted_iota(jnp.int32, (DX - D, L), 0)
        tok = s * L + lax.broadcasted_iota(jnp.int32, (DX - D, L), 1)
        hit = ((row == 0) & (tok == i1)) | ((row == 1) & (tok == i2))
        return jnp.where(hit, 1.0, 0.0)

    def weight_tile(parts):
        blocks = []
        for b in range(KP // 8):
            row = 8 * b + lax.broadcasted_iota(jnp.int32, (8, 128), 0)
            lane = lax.broadcasted_iota(jnp.int32, (8, 128), 1)
            blk = jnp.zeros((8, 128), F32)
            for hh, vals, lo, hi in parts:
                r0, r1 = DH * hh, DH * hh + DH
                if r1 <= 8 * b or r0 >= 8 * b + 8:
                    continue
                keep = None
                for cond in ([row >= r0] if r0 > 8 * b else []) + ([row < r1] if r1 < 8 * b + 8 else []) \
                        + ([lane >= lo] if lo > 0 else []) + ([lane < hi] if hi < 128 else []):
                    keep = cond if keep is None else keep & cond
                v = vals[8 * b:8 * b + 8]
                blk = v if keep is None else jnp.where(keep, v, blk)
            blocks.append(blk)
        return jnp.concatenate(blocks, axis=0).astype(BF16)

    def stage_fns(s, g, g_rows, ret):
        def qk_safe(i):
            q = qts[s, g_rows, 128 * i:128 * (i + 1)]
            qm = jnp.concatenate([weight_tile([(hh, q, 0, 128)]) for hh in range(4)], axis=1)
            nk = 128 * (i + 1)
            st = jnp.dot(kwin[s, g, 0:nk, 0:KP], qm, preferred_element_type=F32)
            ps = []
            for hh in range(4):
                sc = st[:, 128 * hh:128 * (hh + 1)]
                diag = jnp.where(causal, sc[nk - 128:], -1e30)
                sc = jnp.concatenate([sc[:nk - 128], diag], axis=0) if i > 0 else diag
                sc = sc - jnp.max(sc, axis=0, keepdims=True)
                ps.append(jnp.exp2(sc).astype(BF16))
            return ps

        qk = qk_safe

        def pv(i, ps):
            nk = 128 * (i + 1)
            for hh in range(4):
                v = vts[s, g, HS * hh:HS * (hh + 1), 0:nk]
                combine(s, g, ret, i, hh, jnp.dot(v, ps[hh], preferred_element_type=F32))
        return qk, pv

    def combine(s, g, ret, i, hh, o):
        h = 4 * g + hh
        res = o * (gtab[1, pl.ds(h, 1), :] / o[DH:DH + 1])
        if ret is not None:
            mem = ret[DH * hh:DH * hh + HS, 128 * i:128 * (i + 1)]
            den = ret[GD + hh:GD + hh + 1, 128 * i:128 * (i + 1)]
            res = res + mem * (gtab[0, pl.ds(h, 1), :] / (den + 1e-6))
        ot[s, i, pl.ds(DH * h, HS), :] = res

    def qk_items(s, g, i):
        q = qts[s, GD * g:GD * (g + 1), 128 * i:128 * (i + 1)]
        base = 128 * i
        blocks = {}
        st = {}

        def scores(lo, hi, w):
            return jnp.exp2(jnp.dot(kwin[s, g, lo:hi, 0:KP], w, preferred_element_type=F32))

        tile = lambda e, t: e[:, 128 * t:128 * (t + 1)]
        roll = lambda e, t: pltpu.roll(e, t, 1)
        qm = jnp.concatenate([weight_tile([(hh, q, 0, 128)]) for hh in range(4)], axis=1)

        def full(j):
            def run():
                last = j == i - 1
                e = scores(128 * j, 128 * (j + 1) + (32 if last else 0), qm)
                blocks[j] = [tile(e, hh)[0:128].astype(BF16) for hh in range(4)]
                if last:
                    st[0] = e[128:160]
            return run

        def d0():
            st[0] = scores(0, 32, qm)

        def d1():
            st['q'] = [roll(q, t) for t in (32, 64, 96)]
            q32, q64, q96 = st['q']
            st[1] = scores(base + 32, base + 64, jnp.concatenate([
                weight_tile([(0, q, 32, 128), (3, q96, 0, 32)]),
                weight_tile([(1, q, 32, 128), (3, q64, 0, 32)]),
                weight_tile([(2, q, 32, 128), (3, q32, 0, 32)])], axis=1))

        def d2():
            q32, q64, q96 = st['q']
            st[2] = scores(base + 64, base + 96, jnp.concatenate([
                weight_tile([(0, q, 64, 128), (2, q64, 0, 64)]),
                weight_tile([(1, q, 64, 128), (3, q64, 0, 64)])], axis=1))

        def d3():
            q32, q64, q96 = st['q']
            e3 = scores(base + 96, base + 128,
                        weight_tile([(0, q, 96, 128), (1, q96, 64, 96), (2, q64, 32, 64), (3, q32, 0, 32)]))
            e0, e1, e2 = st[0], st[1], st[2]
            lane = lax.broadcasted_iota(jnp.int32, (32, 128), 1)
            blk1 = [tile(e1, 0), tile(e1, 1), tile(e1, 2),
                    jnp.where(lane < 64, roll(tile(e1, 0), 32),
                              jnp.where(lane < 96, roll(tile(e1, 1), 64), roll(tile(e1, 2), 96)))]
            blk2 = [tile(e2, 0), tile(e2, 1), roll(tile(e2, 0), 64), roll(tile(e2, 1), 64)]
            blk3 = [e3, roll(e3, 32), roll(e3, 64), roll(e3, 96)]
            blocks[i] = [
                jnp.where(causal, jnp.concatenate([tile(e0, hh), blk1[hh], blk2[hh], blk3[hh]], axis=0),
                          0.0).astype(BF16) for hh in range(4)]

        items = [full(j) for j in range(i)] + ([d0] if i == 0 else []) + [d1, d2, d3]
        return items, blocks

    def pv_items(s, g, i, rets, blocks):
        acc = {}

        def block(j):
            def run():
                for hh in range(4):
                    v = vts[s, g, HS * hh:HS * (hh + 1), 128 * j:128 * (j + 1)]
                    o = jnp.dot(v, blocks[j][hh], preferred_element_type=F32)
                    acc[hh] = o if j == 0 else acc[hh] + o
                    if j == i:
                        combine(s, g, rets[g], i, hh, acc[hh])
            return run
        return [block(j) for j in range(i + 1)]

    def mem_read(s, g):
        return jnp.dot(mext[g][:, 0:KP], pqt[s, g], preferred_element_type=F32)

    def mem_update(s, g):
        tail = lax.broadcasted_iota(jnp.int32, (KP - GD, L), 0)
        lhs = jnp.concatenate([vts[s, g, HS * hh:HS * hh + DH, :] for hh in range(4)]
                              + [jnp.where(tail == 0, 1.0, 0.0)], axis=0)
        upd = jnp.dot(lhs, pkwin[s, g], preferred_element_type=F32)
        upd = jnp.concatenate(
            [upd[0:GD], jnp.broadcast_to(upd[GD:GD + 1], (KP - GD, 128))], axis=0)
        row = lax.broadcasted_iota(jnp.int32, (KP, 128), 0)
        lane = lax.broadcasted_iota(jnp.int32, (KP, 128), 1)
        head = jnp.where(row < GD, row // DH, row - GD)
        mext[g] = mext[g] + jnp.where((lane >= head * DH) & (lane < head * DH + DH) & (head < 4),
                                      upd, 0.0)

    def wo_part(s, lo, hi):
        rows = min(hi, D)
        otb = jnp.concatenate([ot[s, i, lo:rows, :] for i in range(QT)], axis=1)
        if hi > D:
            otb = jnp.concatenate([otb, scatter_rows(s)], axis=0)
        return jnp.dot(wot[:, lo:hi], otb.astype(BF16), preferred_element_type=F32)

    def finish(s, att):
        cols = seg_cols(s)
        res = xs[:, cols].astype(F32) + att + xn[:, cols].astype(F32)
        outs[:, cols] = res.astype(BF16)

    def attention_fast(s, ffn, ffn_tiles_ready):
        pending = []
        rets = {}

        def extra():
            if ffn:
                f, needs = ffn.pop(0)
                assert needs <= ffn_tiles_ready
                f()

        for g in range(NG):
            rets[g] = None
            for i in range(QT):
                items, blocks = qk_items(s, g, i)
                for n in range(len(items)):
                    items[n]()
                    if n < len(pending) - 1:
                        pending[n]()
                    if n < i:
                        extra()
                    if (i, n) == (3, 1) and s == 1:
                        extra()
                    if (i, n) == (0, 1 if s < NSEG - 1 else 3) and s > 0:
                        rets[g] = mem_read(s, g)
                    if (i, n) == (0, 3) and s < NSEG - 1:
                        mem_update(s, g)
                if pending:
                    pending[-1]()
                pending = pv_items(s, g, i, rets, blocks)
        return pending

    def wait_ffn_weights(lo, hi):
        for c in range(lo, hi):
            for cp in ffn_copies(c):
                cp.wait()

    KS = 384

    def main_fast():
        ffn = ffn_items()
        for s in range(NSEG - 1):
            for f in attention_fast(s, ffn, FU // 2 if s == 0 else FU):
                f()
            if s == 0:
                wait_ffn_weights(2, NSEG)
        assert not ffn
        for s in range(NSEG - 1):
            finish(s, wo_part(s, 0, DX))
        for s in range(NSEG - 1):
            out_copy(s).start()
        pending = attention_fast(NSEG - 1, [], FU)
        att = wo_part(NSEG - 1, 0, KS)
        for f in pending:
            f()
        finish(NSEG - 1, att + wo_part(NSEG - 1, KS, DX))

    def main_safe():
        wait_ffn_weights(2, NSEG)

        def segment(s, carry):
            def body(g, c):
                g_rows = pl.ds(pl.multiple_of(GD * g, 8), GD)
                qk, pv = stage_fns(s, g, g_rows, mem_read(s, g))
                mem_update(s, g)
                for i in range(QT):
                    pv(i, qk(i))
                return c
            return lax.fori_loop(0, NG, body, carry)
        lax.fori_loop(0, NSEG, segment, 0)

        def ffn_body(u, c):
            ffn_down_part(u, 1, ffn_act(ffn_up_part(u, 1, 0, D)), 0, D)
            return c
        lax.fori_loop(0, FU, ffn_body, 0)
        ffn_finish()

        def project(s, c):
            finish(s, wo_part(s, 0, DX))
            return c
        lax.fori_loop(0, NSEG, project, 0)
        for s in range(NSEG - 1):
            out_copy(s).start()

    wait_ffn_weights(0, 2)
    lax.cond(no_shift_needed, main_fast, main_safe)
    out_copy(NSEG - 1).start()
    for s in range(NSEG):
        out_copy(s).wait()


@jax.jit
def pallas_parallel_sum__memory_aug_infini_attn__moe_arch_mod__prompt_kernel(
    A_x: jax.Array,
    A_wq: jax.Array,
    A_wk: jax.Array,
    A_wv: jax.Array,
    A_wo: jax.Array,
    A_beta: jax.Array,
    B_x: jax.Array,
    B_w_r: jax.Array,
    B_w_gate: jax.Array,
    B_w_up: jax.Array,
    B_w_down: jax.Array,
):
    del B_x
    xt = A_x.reshape(S, D).T
    wdt = B_w_down.T
    hbm = pl.BlockSpec(memory_space=pltpu.HBM)
    out = pl.pallas_call(
        _kernel,
        out_shape=jax.ShapeDtypeStruct((D, S), BF16),
        in_specs=[hbm] * 10,
        out_specs=hbm,
        scratch_shapes=[
            pltpu.VMEM((D, S), BF16),
            pltpu.VMEM((D, S), BF16),
            pltpu.VMEM((D, D), BF16),
            pltpu.VMEM((D, D), BF16),
            pltpu.VMEM((D, D), BF16),
            pltpu.VMEM((D, D), BF16),
            pltpu.VMEM((H,), BF16),
            pltpu.VMEM((D,), BF16),
            pltpu.VMEM((WROWS, D), BF16),
            pltpu.VMEM((D, DX), BF16),
            pltpu.VMEM((2, H, 128), F32),
            pltpu.VMEM((NSEG, D, L), F32),
            pltpu.VMEM((NSEG, NG, L, 128), BF16),
            pltpu.VMEM((NSEG, NG, KP, L), BF16),
            pltpu.VMEM((NSEG, NG, L, 128), BF16),
            pltpu.VMEM((NSEG, NG, 4 * HS, L), F32),
            pltpu.VMEM((NG, KP, 128), F32),
            pltpu.VMEM((NSEG, QT, D + 24, 128), F32),
            pltpu.VMEM((D, S), BF16),
            pltpu.VMEM((NSEG * QT, 128), F32),
            pltpu.VMEM((8, D), F32),
            pltpu.VMEM((8, D), F32),
            pltpu.VMEM((D, F), BF16),
            pltpu.VMEM((D, F), BF16),
            pltpu.VMEM((D, F), BF16),
            pltpu.SemaphoreType.DMA((N_SEMS,)),
        ],
        compiler_params=pltpu.CompilerParams(vmem_limit_bytes=110 * 1024 * 1024),
    )(xt, A_wq, A_wk, A_wv, A_wo, A_beta, B_w_r, B_w_gate, B_w_up, wdt)
    return out.T.reshape(1, S, D)
```

```python
import math

import jax
import jax.numpy as jnp
from jax import lax
import jax.experimental.pallas as pl
import jax.experimental.pallas.tpu as pltpu

S = 2048
D = 576
H = 32
DH = 18
NSEG = 4
L = S // NSEG
F = 4608
NG = 8
GD = 4 * DH
HS = 24
QT = L // 128
WROWS = 3 * D + 16
FU = F // 128
FC = F // NSEG
DX = D + 16
KP = 80

F32 = jnp.float32
BF16 = jnp.bfloat16
QSCALE = (DH ** -0.5) * math.log2(math.e)
SAFE_LOGIT_BOUND = 60.0
SAFE_VALUE_BOUND = 2.0 ** 40
XN_SQ_BOUND = 2.0 * D * 1.1

NT = (((1,), (1,)), ((), ()))

(SEM_X, SEM_WQ, SEM_WK, SEM_WV, SEM_WO, SEM_BETA, SEM_WR,
 SEM_OUT, SEM_LAST, SEM_FFN) = 0, 4, 5, 6, 7, 8, 9, 10, 13, 17
N_SEMS = SEM_FFN + 3 * NSEG


def _bf(x):
    return x.astype(BF16).astype(F32)


def _phi(t):
    return jnp.where(t > 0, t + 1.0, jnp.exp(t))


def _max_col_sq(w32):
    return jnp.max(jnp.sum(w32 * w32, axis=0, keepdims=True))


def _rows_padded(a, start, rows):
    stop = min(start + rows, a.shape[0])
    part = a[start:stop]
    if stop - start < rows:
        part = jnp.concatenate([part, jnp.zeros((rows - (stop - start), a.shape[1]), a.dtype)], axis=0)
    return part


def _kernel(x_hbm, wq_hbm, wk_hbm, wv_hbm, wo_hbm, beta_hbm, wr_hbm, wg_hbm, wu_hbm, wd_hbm,
            out_hbm,
            xs, xn, wq, wk, wv, wo, beta, wr, wt, wot, gtab, qts, kwin, pqt, pkwin, vts, mext, ot,
            outs, rbuf, yacc, xsel_ref, wg, wu, wd, sems):

    def seg_cols(s):
        if isinstance(s, int):
            return slice(s * L, (s + 1) * L)
        return pl.ds(pl.multiple_of(s * L, L), L)

    def x_copy(s):
        return pltpu.make_async_copy(x_hbm.at[:, seg_cols(s)], xs.at[:, seg_cols(s)], sems.at[SEM_X + s])

    def out_copy(s):
        return pltpu.make_async_copy(outs.at[:, seg_cols(s)], out_hbm.at[:, seg_cols(s)],
                                     sems.at[SEM_OUT + s])

    OC = D // 4

    def last_copy(c):
        rows, cols = slice(c * OC, (c + 1) * OC), seg_cols(NSEG - 1)
        return pltpu.make_async_copy(outs.at[rows, cols], out_hbm.at[rows, cols], sems.at[SEM_LAST + c])

    cp_wq = pltpu.make_async_copy(wq_hbm, wq, sems.at[SEM_WQ])
    cp_wk = pltpu.make_async_copy(wk_hbm, wk, sems.at[SEM_WK])
    cp_wv = pltpu.make_async_copy(wv_hbm, wv, sems.at[SEM_WV])
    cp_wo = pltpu.make_async_copy(wo_hbm, wo, sems.at[SEM_WO])

    def ffn_copies(s):
        if isinstance(s, int):
            cols = slice(s * FC, (s + 1) * FC)
        else:
            cols = pl.ds(pl.multiple_of(s * FC, 128), FC)
        return [pltpu.make_async_copy(src.at[:, cols], dst.at[:, cols], sems.at[SEM_FFN + 3 * s + k])
                for k, (src, dst) in enumerate(((wg_hbm, wg), (wu_hbm, wu), (wd_hbm, wd)))]

    cp_beta = pltpu.make_async_copy(beta_hbm, beta, sems.at[SEM_BETA])
    cp_wr = pltpu.make_async_copy(wr_hbm, wr, sems.at[SEM_WR])

    def transposed(w_ref):
        w32 = w_ref[...].astype(F32)
        return w32.T.astype(BF16), _max_col_sq(w32)

    def layernorm(s):
        x32 = xs[:, seg_cols(s)].astype(F32)
        mean = jnp.sum(x32, axis=0, keepdims=True) / D
        mean_b = _bf(mean)
        cen = x32 - mean_b
        shift = mean - mean_b
        var = jnp.sum(cen * cen, axis=0, keepdims=True) / D - shift * shift
        den = _bf(jnp.sqrt(_bf(_bf(var) + _bf(jnp.float32(1e-5)))))
        xn[:, seg_cols(s)] = (_bf(cen) * (1.0 / den)).astype(BF16)

    def proj_q(s, g0, g1):
        q = jnp.dot(wt[GD * g0:GD * g1, :], xn[:, seg_cols(s)], preferred_element_type=F32)
        qts[s, GD * g0:GD * g1, :] = q * QSCALE
        pq = _phi(q)
        pad = jnp.zeros((KP - GD, L), F32)
        for g in range(g0, g1):
            win = jnp.concatenate([pq[GD * (g - g0):GD * (g - g0 + 1)], pad], axis=0)
            pqt[s, g] = win.astype(BF16)

    def proj_k(s):
        k = jnp.dot(wt[D:2 * D, :], xn[:, seg_cols(s)], preferred_element_type=F32)
        for g in range(NG):
            kw = _rows_padded(k, GD * g, 128).T
            kwin[s, g] = kw.astype(BF16)
            pkwin[s, g] = _phi(kw).astype(BF16)

    def proj_v(s):
        v = jnp.dot(wt[2 * D:WROWS, :], xn[:, seg_cols(s)], preferred_element_type=F32)
        for j in range(QT):
            rbuf[s * QT + j:s * QT + j + 1, :] = _bf(v[D:D + 1, 128 * j:128 * (j + 1)])
        hrow = lax.broadcasted_iota(jnp.int32, (HS, L), 0)
        fill = jnp.where(hrow == DH, 1.0, 0.0)
        for h in range(H):
            g, hh = divmod(h, 4)
            vts[s, g, HS * hh:HS * (hh + 1), :] = jnp.where(
                hrow < DH, v[DH * h:DH * h + HS], fill)

    def tile_of(idx):
        return pl.ds(pl.multiple_of((idx // 128) * 128, 128), 128)

    def router():
        r = rbuf[...]
        tok = (lax.broadcasted_iota(jnp.int32, r.shape, 0) * 128
               + lax.broadcasted_iota(jnp.int32, r.shape, 1))
        r1 = jnp.max(r)
        i1 = jnp.min(jnp.where(r == r1, tok, S))
        rm = jnp.where(tok == i1, -jnp.inf, r)
        r2 = jnp.max(rm)
        i2 = jnp.min(jnp.where((rm == r2) & (tok != i1), tok, S))
        i1 = jnp.minimum(i1, S - 1)
        i2 = jnp.minimum(i2, S - 1)
        row8 = lax.broadcasted_iota(jnp.int32, (8, 128), 0)
        lane8 = lax.broadcasted_iota(jnp.int32, (8, 128), 1)
        hot1 = jnp.where((row8 == 0) & (lane8 == i1 % 128), 1.0, 0.0)
        hot2 = jnp.where((row8 == 1) & (lane8 == i2 % 128), 1.0, 0.0)
        return r1, r2, i1, i2, hot1, hot2

    x_copy(0).start()
    cp_wr.start()
    cp_beta.start()
    cp_wq.start()
    mext[...] = jnp.zeros(mext.shape, F32)
    yacc[...] = jnp.zeros(yacc.shape, F32)
    x_copy(0).wait()
    x_copy(1).start()
    cp_wv.start()
    cp_wk.start()
    cp_wr.wait()
    layernorm(0)
    cp_wq.wait()
    wt[0:D, :], nq = transposed(wq)
    proj_q(0, 0, NG // 2)
    x_copy(1).wait()
    proj_q(0, NG // 2, NG)
    layernorm(1)
    cp_wv.wait()
    wt[2 * D:3 * D, :], nv = transposed(wv)
    row16 = lax.broadcasted_iota(jnp.int32, (16, D), 0)
    wt[3 * D:WROWS, :] = jnp.where(
        row16 == 0, wr[...].astype(F32).reshape(1, D), 0.0).astype(BF16)
    cp_wk.wait()
    x_copy(2).start()
    x_copy(3).start()
    cp_wo.start()
    for s in range(NSEG):
        for cp in ffn_copies(s):
            cp.start()
    cp_beta.wait()
    proj_q(1, 0, NG)
    wt[D:2 * D, :], nk = transposed(wk)
    x_copy(2).wait()
    x_copy(3).wait()
    proj_v(0)
    proj_k(0)
    layernorm(2)
    layernorm(3)
    cp_wo.wait()
    for s in range(1, NSEG):
        proj_v(s)
    r1, r2, i1, i2, hot1, hot2 = router()
    wot[:, 0:D] = wo[...].astype(F32).T.astype(BF16)
    b = beta[...].astype(F32).reshape(1, H)
    bt = jnp.broadcast_to(
        jnp.concatenate([b, jnp.zeros((1, 128 - H), F32)], axis=1), (128, 128)).T
    gt_all = _bf(jax.nn.sigmoid(bt[0:H]))
    gtab[0] = gt_all
    gtab[1] = _bf(1.0 - gt_all)
    logit_bound = (DH * QSCALE * XN_SQ_BOUND) * jnp.sqrt(nq) * jnp.sqrt(nk)
    no_shift_needed = ((logit_bound <= SAFE_LOGIT_BOUND)
                       & (XN_SQ_BOUND * nv <= SAFE_VALUE_BOUND * SAFE_VALUE_BOUND))
    for s in range(1, NSEG):
        proj_k(s)
    for s in range(2, NSEG):
        proj_q(s, 0, NG)
    xsel_ref[...] = (
        lax.dot_general(hot1, xn[:, tile_of(i1)], NT, preferred_element_type=F32)
        + lax.dot_general(hot2, xn[:, tile_of(i2)], NT, preferred_element_type=F32))

    krow = lax.broadcasted_iota(jnp.int32, (128, 128), 0)
    kcol = lax.broadcasted_iota(jnp.int32, (128, 128), 1)
    causal = krow <= kcol

    def ffn_cols(u, n=1):
        if isinstance(u, int):
            return slice(u * 128, (u + n) * 128)
        return pl.ds(pl.multiple_of(u * 128, 128), n * 128)

    def ffn_up_part(u, n, lo, hi):
        w2 = jnp.concatenate([wg[lo:hi, ffn_cols(u, n)], wu[lo:hi, ffn_cols(u, n)]], axis=1)
        return jnp.dot(xsel_ref[:, lo:hi], w2, preferred_element_type=F32)

    def ffn_act(gu):
        n = gu.shape[1] // 2
        gate = _bf(gu[:, 0:n])
        return _bf(_bf(gate * jax.nn.sigmoid(gate)) * _bf(gu[:, n:]))

    def ffn_down_part(u, n, hid, lo, hi):
        yacc[:, lo:hi] += lax.dot_general(hid, wd[lo:hi, ffn_cols(u, n)], NT,
                                          preferred_element_type=F32)

    def ffn_items():
        st = {}

        def up(u, lo, hi):
            def run():
                part = ffn_up_part(u, 2, lo, hi)
                st[u] = part if lo == 0 else st[u] + part
                if hi == D:
                    st[u] = ffn_act(st[u])
            return run

        def down(u):
            return lambda: ffn_down_part(u, 1, st[u - u % 2][:, 128 * (u % 2):128 * (u % 2 + 1)], 0, 512)

        def down_tail(u):
            return lambda: ffn_down_part(
                u, 4, jnp.concatenate([st[u], st[u + 2]], axis=1), 512, D)

        bounds = [0, 128, 256, 384, 512, D]
        ups = lambda u: [up(u, bounds[k], bounds[k + 1]) for k in range(5)]
        downs = lambda u: [down(u + k) for k in range(4)] + [down_tail(u)]
        items = []
        for u in range(0, FU + 4, 4):
            if u < FU:
                items += [(f, u + 2) for f in ups(u)] + [(f, u + 4) for f in ups(u + 2)]
            if u > 0:
                items += [(f, u) for f in downs(u - 4)]
        return items + [(ffn_finish, FU)]

    def ffn_finish():
        rowd = lax.broadcasted_iota(jnp.int32, (8, D), 0)
        y = _bf(_bf(yacc[...]) * _bf(jax.nn.sigmoid(jnp.where(rowd == 0, r1, r2))))
        y = jnp.where(rowd < 2, y, 0.0)
        yt = jnp.concatenate([y, jnp.zeros((120, D), F32)], axis=0).T
        wot[:, D:DX] = yt[:, 0:DX - D].astype(BF16)

    def scatter_rows(s):
        row = lax.broadcasted_iota(jnp.int32, (DX - D, L), 0)
        tok = s * L + lax.broadcasted_iota(jnp.int32, (DX - D, L), 1)
        hit = ((row == 0) & (tok == i1)) | ((row == 1) & (tok == i2))
        return jnp.where(hit, 1.0, 0.0)

    def weight_tile(parts):
        blocks = []
        for b in range(KP // 8):
            row = 8 * b + lax.broadcasted_iota(jnp.int32, (8, 128), 0)
            lane = lax.broadcasted_iota(jnp.int32, (8, 128), 1)
            blk = jnp.zeros((8, 128), F32)
            for hh, vals, lo, hi in parts:
                r0, r1 = DH * hh, DH * hh + DH
                if r1 <= 8 * b or r0 >= 8 * b + 8:
                    continue
                keep = None
                for cond in ([row >= r0] if r0 > 8 * b else []) + ([row < r1] if r1 < 8 * b + 8 else []) \
                        + ([lane >= lo] if lo > 0 else []) + ([lane < hi] if hi < 128 else []):
                    keep = cond if keep is None else keep & cond
                v = vals[8 * b:8 * b + 8]
                blk = v if keep is None else jnp.where(keep, v, blk)
            blocks.append(blk)
        return jnp.concatenate(blocks, axis=0).astype(BF16)

    def stage_fns(s, g, g_rows, ret):
        def qk_safe(i):
            q = qts[s, g_rows, 128 * i:128 * (i + 1)]
            qm = jnp.concatenate([weight_tile([(hh, q, 0, 128)]) for hh in range(4)], axis=1)
            nk = 128 * (i + 1)
            st = jnp.dot(kwin[s, g, 0:nk, 0:KP], qm, preferred_element_type=F32)
            ps = []
            for hh in range(4):
                sc = st[:, 128 * hh:128 * (hh + 1)]
                diag = jnp.where(causal, sc[nk - 128:], -1e30)
                sc = jnp.concatenate([sc[:nk - 128], diag], axis=0) if i > 0 else diag
                sc = sc - jnp.max(sc, axis=0, keepdims=True)
                ps.append(jnp.exp2(sc).astype(BF16))
            return ps

        qk = qk_safe

        def pv(i, ps):
            nk = 128 * (i + 1)
            for hh in range(4):
                v = vts[s, g, HS * hh:HS * (hh + 1), 0:nk]
                combine(s, g, ret, i, hh, jnp.dot(v, ps[hh], preferred_element_type=F32))
        return qk, pv

    def combine(s, g, ret, i, hh, o):
        h = 4 * g + hh
        res = o * (gtab[1, pl.ds(h, 1), :] / o[DH:DH + 1])
        if ret is not None:
            mem = ret[DH * hh:DH * hh + HS, 128 * i:128 * (i + 1)]
            den = ret[GD + hh:GD + hh + 1, 128 * i:128 * (i + 1)]
            res = res + mem * (gtab[0, pl.ds(h, 1), :] / (den + 1e-6))
        ot[s, i, pl.ds(DH * h, HS), :] = res

    def qk_items(s, g, i):
        q = qts[s, GD * g:GD * (g + 1), 128 * i:128 * (i + 1)]
        base = 128 * i
        blocks = {}
        st = {}

        def scores(lo, hi, w):
            return jnp.exp2(jnp.dot(kwin[s, g, lo:hi, 0:KP], w, preferred_element_type=F32))

        tile = lambda e, t: e[:, 128 * t:128 * (t + 1)]
        roll = lambda e, t: pltpu.roll(e, t, 1)
        qm = jnp.concatenate([weight_tile([(hh, q, 0, 128)]) for hh in range(4)], axis=1)

        def full(j):
            def run():
                last = j == i - 1
                e = scores(128 * j, 128 * (j + 1) + (32 if last else 0), qm)
                blocks[j] = [tile(e, hh)[0:128].astype(BF16) for hh in range(4)]
                if last:
                    st[0] = e[128:160]
            return run

        def d0():
            st[0] = scores(0, 32, qm)

        def d1():
            st['q'] = [roll(q, t) for t in (32, 64, 96)]
            q32, q64, q96 = st['q']
            st[1] = scores(base + 32, base + 64, jnp.concatenate([
                weight_tile([(0, q, 32, 128), (3, q96, 0, 32)]),
                weight_tile([(1, q, 32, 128), (3, q64, 0, 32)]),
                weight_tile([(2, q, 32, 128), (3, q32, 0, 32)])], axis=1))

        def d2():
            q32, q64, q96 = st['q']
            st[2] = scores(base + 64, base + 96, jnp.concatenate([
                weight_tile([(0, q, 64, 128), (2, q64, 0, 64)]),
                weight_tile([(1, q, 64, 128), (3, q64, 0, 64)])], axis=1))

        def d3():
            q32, q64, q96 = st['q']
            e3 = scores(base + 96, base + 128,
                        weight_tile([(0, q, 96, 128), (1, q96, 64, 96), (2, q64, 32, 64), (3, q32, 0, 32)]))
            e0, e1, e2 = st[0], st[1], st[2]
            lane = lax.broadcasted_iota(jnp.int32, (32, 128), 1)
            blk1 = [tile(e1, 0), tile(e1, 1), tile(e1, 2),
                    jnp.where(lane < 64, roll(tile(e1, 0), 32),
                              jnp.where(lane < 96, roll(tile(e1, 1), 64), roll(tile(e1, 2), 96)))]
            blk2 = [tile(e2, 0), tile(e2, 1), roll(tile(e2, 0), 64), roll(tile(e2, 1), 64)]
            blk3 = [e3, roll(e3, 32), roll(e3, 64), roll(e3, 96)]
            blocks[i] = [
                jnp.where(causal, jnp.concatenate([tile(e0, hh), blk1[hh], blk2[hh], blk3[hh]], axis=0),
                          0.0).astype(BF16) for hh in range(4)]

        items = [full(j) for j in range(i)] + ([d0] if i == 0 else []) + [d1, d2, d3]
        return items, blocks

    def pv_items(s, g, i, rets, blocks):
        acc = {}

        def block(j):
            def run():
                for hh in range(4):
                    v = vts[s, g, HS * hh:HS * (hh + 1), 128 * j:128 * (j + 1)]
                    o = jnp.dot(v, blocks[j][hh], preferred_element_type=F32)
                    acc[hh] = o if j == 0 else acc[hh] + o
                    if j == i:
                        combine(s, g, rets[g], i, hh, acc[hh])
            return run
        return [block(j) for j in range(i + 1)]

    def mem_read(s, g):
        return jnp.dot(mext[g][:, 0:KP], pqt[s, g], preferred_element_type=F32)

    def mem_update(s, g):
        tail = lax.broadcasted_iota(jnp.int32, (KP - GD, L), 0)
        lhs = jnp.concatenate([vts[s, g, HS * hh:HS * hh + DH, :] for hh in range(4)]
                              + [jnp.where(tail == 0, 1.0, 0.0)], axis=0)
        upd = jnp.dot(lhs, pkwin[s, g], preferred_element_type=F32)
        upd = jnp.concatenate(
            [upd[0:GD], jnp.broadcast_to(upd[GD:GD + 1], (KP - GD, 128))], axis=0)
        row = lax.broadcasted_iota(jnp.int32, (KP, 128), 0)
        lane = lax.broadcasted_iota(jnp.int32, (KP, 128), 1)
        head = jnp.where(row < GD, row // DH, row - GD)
        mext[g] = mext[g] + jnp.where((lane >= head * DH) & (lane < head * DH + DH) & (head < 4),
                                      upd, 0.0)

    def wo_part(s, lo, hi, out_rows=slice(0, D)):
        rows = min(hi, D)
        otb = jnp.concatenate([ot[s, i, lo:rows, :] for i in range(QT)], axis=1)
        if hi > D:
            otb = jnp.concatenate([otb, scatter_rows(s)], axis=0)
        return jnp.dot(wot[out_rows, lo:hi], otb.astype(BF16), preferred_element_type=F32)

    def finish(s, att, out_rows=slice(0, D)):
        cols = seg_cols(s)
        res = xs[out_rows, cols].astype(F32) + att + xn[out_rows, cols].astype(F32)
        outs[out_rows, cols] = res.astype(BF16)

    def attention_fast(s, ffn, ffn_tiles_ready):
        pending = []
        rets = {}

        def extra():
            if ffn:
                f, needs = ffn.pop(0)
                assert needs <= ffn_tiles_ready
                f()

        for g in range(NG):
            rets[g] = None
            for i in range(QT):
                items, blocks = qk_items(s, g, i)
                for n in range(len(items)):
                    items[n]()
                    if n < len(pending) - 1:
                        pending[n]()
                    if n < i:
                        extra()
                    if (i, n) == (3, 1) and s == 1:
                        extra()
                    if (i, n) == (0, 1 if s < NSEG - 1 else 3) and s > 0:
                        rets[g] = mem_read(s, g)
                    if (i, n) == (0, 3) and s < NSEG - 1:
                        mem_update(s, g)
                if pending:
                    pending[-1]()
                pending = pv_items(s, g, i, rets, blocks)
        return pending

    def wait_ffn_weights(lo, hi):
        for c in range(lo, hi):
            for cp in ffn_copies(c):
                cp.wait()

    KS = 384

    def main_fast():
        ffn = ffn_items()
        for s in range(NSEG - 1):
            for f in attention_fast(s, ffn, FU // 2 if s == 0 else FU):
                f()
            if s == 0:
                wait_ffn_weights(2, NSEG)
        assert not ffn
        for s in range(NSEG - 1):
            finish(s, wo_part(s, 0, DX))
        for s in range(NSEG - 1):
            out_copy(s).start()
        pending = attention_fast(NSEG - 1, [], FU)
        att = wo_part(NSEG - 1, 0, KS)
        for f in pending:
            f()
        for c in range(4):
            rows = slice(c * OC, (c + 1) * OC)
            finish(NSEG - 1, att[rows] + wo_part(NSEG - 1, KS, DX, rows), rows)
            last_copy(c).start()

    def main_safe():
        wait_ffn_weights(2, NSEG)

        def segment(s, carry):
            def body(g, c):
                g_rows = pl.ds(pl.multiple_of(GD * g, 8), GD)
                qk, pv = stage_fns(s, g, g_rows, mem_read(s, g))
                mem_update(s, g)
                for i in range(QT):
                    pv(i, qk(i))
                return c
            return lax.fori_loop(0, NG, body, carry)
        lax.fori_loop(0, NSEG, segment, 0)

        def ffn_body(u, c):
            ffn_down_part(u, 1, ffn_act(ffn_up_part(u, 1, 0, D)), 0, D)
            return c
        lax.fori_loop(0, FU, ffn_body, 0)
        ffn_finish()

        def project(s, c):
            finish(s, wo_part(s, 0, DX))
            return c
        lax.fori_loop(0, NSEG, project, 0)
        for s in range(NSEG - 1):
            out_copy(s).start()
        for c in range(4):
            last_copy(c).start()

    wait_ffn_weights(0, 2)
    lax.cond(no_shift_needed, main_fast, main_safe)
    for s in range(NSEG - 1):
        out_copy(s).wait()
    for c in range(4):
        last_copy(c).wait()


@jax.jit
def pallas_parallel_sum__memory_aug_infini_attn__moe_arch_mod__prompt_kernel(
    A_x: jax.Array,
    A_wq: jax.Array,
    A_wk: jax.Array,
    A_wv: jax.Array,
    A_wo: jax.Array,
    A_beta: jax.Array,
    B_x: jax.Array,
    B_w_r: jax.Array,
    B_w_gate: jax.Array,
    B_w_up: jax.Array,
    B_w_down: jax.Array,
):
    del B_x
    xt = A_x.reshape(S, D).T
    wdt = B_w_down.T
    hbm = pl.BlockSpec(memory_space=pltpu.HBM)
    out = pl.pallas_call(
        _kernel,
        out_shape=jax.ShapeDtypeStruct((D, S), BF16),
        in_specs=[hbm] * 10,
        out_specs=hbm,
        scratch_shapes=[
            pltpu.VMEM((D, S), BF16),
            pltpu.VMEM((D, S), BF16),
            pltpu.VMEM((D, D), BF16),
            pltpu.VMEM((D, D), BF16),
            pltpu.VMEM((D, D), BF16),
            pltpu.VMEM((D, D), BF16),
            pltpu.VMEM((H,), BF16),
            pltpu.VMEM((D,), BF16),
            pltpu.VMEM((WROWS, D), BF16),
            pltpu.VMEM((D, DX), BF16),
            pltpu.VMEM((2, H, 128), F32),
            pltpu.VMEM((NSEG, D, L), F32),
            pltpu.VMEM((NSEG, NG, L, 128), BF16),
            pltpu.VMEM((NSEG, NG, KP, L), BF16),
            pltpu.VMEM((NSEG, NG, L, 128), BF16),
            pltpu.VMEM((NSEG, NG, 4 * HS, L), F32),
            pltpu.VMEM((NG, KP, 128), F32),
            pltpu.VMEM((NSEG, QT, D + 24, 128), F32),
            pltpu.VMEM((D, S), BF16),
            pltpu.VMEM((NSEG * QT, 128), F32),
            pltpu.VMEM((8, D), F32),
            pltpu.VMEM((8, D), F32),
            pltpu.VMEM((D, F), BF16),
            pltpu.VMEM((D, F), BF16),
            pltpu.VMEM((D, F), BF16),
            pltpu.SemaphoreType.DMA((N_SEMS,)),
        ],
        compiler_params=pltpu.CompilerParams(vmem_limit_bytes=110 * 1024 * 1024),
    )(xt, A_wq, A_wk, A_wv, A_wo, A_beta, B_w_r, B_w_gate, B_w_up, wdt)
    return out.T.reshape(1, S, D)
```

```python
import math

import jax
import jax.numpy as jnp
from jax import lax
import jax.experimental.pallas as pl
import jax.experimental.pallas.tpu as pltpu

S = 2048
D = 576
H = 32
DH = 18
NSEG = 4
L = S // NSEG
F = 4608
NG = 8
GD = 4 * DH
HS = 24
QT = L // 128
WROWS = 3 * D + 16
FU = F // 128
FC = F // NSEG
DX = D + 16
KP = 80

F32 = jnp.float32
BF16 = jnp.bfloat16
QSCALE = (DH ** -0.5) * math.log2(math.e)
SAFE_LOGIT_BOUND = 60.0
SAFE_VALUE_BOUND = 2.0 ** 40
XN_SQ_BOUND = 2.0 * D * 1.1

NT = (((1,), (1,)), ((), ()))

(SEM_X, SEM_WQ, SEM_WK, SEM_WV, SEM_WO, SEM_BETA, SEM_WR,
 SEM_OUT, SEM_LAST, SEM_FFN) = 0, 4, 5, 6, 7, 8, 9, 10, 13, 17
N_SEMS = SEM_FFN + 3 * NSEG


def _bf(x):
    return x.astype(BF16).astype(F32)


def _phi(t):
    return jnp.where(t > 0, t + 1.0, jnp.exp(t))


def _max_col_sq(w32):
    return jnp.max(jnp.sum(w32 * w32, axis=0, keepdims=True))


def _rows_padded(a, start, rows):
    stop = min(start + rows, a.shape[0])
    part = a[start:stop]
    if stop - start < rows:
        part = jnp.concatenate([part, jnp.zeros((rows - (stop - start), a.shape[1]), a.dtype)], axis=0)
    return part


def _kernel(x_hbm, wq_hbm, wk_hbm, wv_hbm, wo_hbm, beta_hbm, wr_hbm, wg_hbm, wu_hbm, wd_hbm,
            out_hbm,
            xs, xn, wq, wk, wv, wo, beta, wr, wt, wot, gtab, qts, kwin, pqt, pkwin, vts, mext, ot,
            outs, rbuf, yacc, xsel_ref, wg, wu, wd, sems):

    def seg_cols(s):
        if isinstance(s, int):
            return slice(s * L, (s + 1) * L)
        return pl.ds(pl.multiple_of(s * L, L), L)

    def x_copy(s):
        return pltpu.make_async_copy(x_hbm.at[:, seg_cols(s)], xs.at[:, seg_cols(s)], sems.at[SEM_X + s])

    def out_copy(s):
        return pltpu.make_async_copy(outs.at[:, seg_cols(s)], out_hbm.at[:, seg_cols(s)],
                                     sems.at[SEM_OUT + s])

    OC = D // 4

    def last_copy(c):
        rows, cols = slice(c * OC, (c + 1) * OC), seg_cols(NSEG - 1)
        return pltpu.make_async_copy(outs.at[rows, cols], out_hbm.at[rows, cols], sems.at[SEM_LAST + c])

    cp_wq = pltpu.make_async_copy(wq_hbm, wq, sems.at[SEM_WQ])
    cp_wk = pltpu.make_async_copy(wk_hbm, wk, sems.at[SEM_WK])
    cp_wv = pltpu.make_async_copy(wv_hbm, wv, sems.at[SEM_WV])
    cp_wo = pltpu.make_async_copy(wo_hbm, wo, sems.at[SEM_WO])

    def ffn_copies(s):
        if isinstance(s, int):
            cols = slice(s * FC, (s + 1) * FC)
        else:
            cols = pl.ds(pl.multiple_of(s * FC, 128), FC)
        return [pltpu.make_async_copy(src.at[:, cols], dst.at[:, cols], sems.at[SEM_FFN + 3 * s + k])
                for k, (src, dst) in enumerate(((wg_hbm, wg), (wu_hbm, wu), (wd_hbm, wd)))]

    cp_beta = pltpu.make_async_copy(beta_hbm, beta, sems.at[SEM_BETA])
    cp_wr = pltpu.make_async_copy(wr_hbm, wr, sems.at[SEM_WR])

    def transposed(w_ref):
        w32 = w_ref[...].astype(F32)
        return w32.T.astype(BF16), _max_col_sq(w32)

    def layernorm(s):
        x32 = xs[:, seg_cols(s)].astype(F32)
        mean = jnp.sum(x32, axis=0, keepdims=True) / D
        mean_b = _bf(mean)
        cen = x32 - mean_b
        shift = mean - mean_b
        var = jnp.sum(cen * cen, axis=0, keepdims=True) / D - shift * shift
        den = _bf(jnp.sqrt(_bf(_bf(var) + _bf(jnp.float32(1e-5)))))
        xn[:, seg_cols(s)] = (_bf(cen) * (1.0 / den)).astype(BF16)

    def proj_q(s, g0, g1):
        q = jnp.dot(wt[GD * g0:GD * g1, :], xn[:, seg_cols(s)], preferred_element_type=F32)
        qts[s, GD * g0:GD * g1, :] = q * QSCALE
        pq = _phi(q)
        pad = jnp.zeros((KP - GD, L), F32)
        for g in range(g0, g1):
            win = jnp.concatenate([pq[GD * (g - g0):GD * (g - g0 + 1)], pad], axis=0)
            pqt[s, g] = win.astype(BF16)

    def proj_k(s):
        k = jnp.dot(wt[D:2 * D, :], xn[:, seg_cols(s)], preferred_element_type=F32)
        for g in range(NG):
            kw = _rows_padded(k, GD * g, 128).T
            kwin[s, g] = kw.astype(BF16)
            pkwin[s, g] = _phi(kw).astype(BF16)

    def proj_v(s):
        v = jnp.dot(wt[2 * D:WROWS, :], xn[:, seg_cols(s)], preferred_element_type=F32)
        for j in range(QT):
            rbuf[s * QT + j:s * QT + j + 1, :] = _bf(v[D:D + 1, 128 * j:128 * (j + 1)])
        hrow = lax.broadcasted_iota(jnp.int32, (HS, L), 0)
        fill = jnp.where(hrow == DH, 1.0, 0.0)
        for h in range(H):
            g, hh = divmod(h, 4)
            vts[s, g, HS * hh:HS * (hh + 1), :] = jnp.where(
                hrow < DH, v[DH * h:DH * h + HS], fill)

    def tile_of(idx):
        return pl.ds(pl.multiple_of((idx // 128) * 128, 128), 128)

    def router():
        r = rbuf[...]
        tok = (lax.broadcasted_iota(jnp.int32, r.shape, 0) * 128
               + lax.broadcasted_iota(jnp.int32, r.shape, 1))
        r1 = jnp.max(r)
        i1 = jnp.min(jnp.where(r == r1, tok, S))
        rm = jnp.where(tok == i1, -jnp.inf, r)
        r2 = jnp.max(rm)
        i2 = jnp.min(jnp.where((rm == r2) & (tok != i1), tok, S))
        i1 = jnp.minimum(i1, S - 1)
        i2 = jnp.minimum(i2, S - 1)
        row8 = lax.broadcasted_iota(jnp.int32, (8, 128), 0)
        lane8 = lax.broadcasted_iota(jnp.int32, (8, 128), 1)
        hot1 = jnp.where((row8 == 0) & (lane8 == i1 % 128), 1.0, 0.0)
        hot2 = jnp.where((row8 == 1) & (lane8 == i2 % 128), 1.0, 0.0)
        return r1, r2, i1, i2, hot1, hot2

    x_copy(0).start()
    cp_wr.start()
    cp_beta.start()
    cp_wq.start()
    mext[...] = jnp.zeros(mext.shape, F32)
    yacc[...] = jnp.zeros(yacc.shape, F32)
    x_copy(0).wait()
    x_copy(1).start()
    cp_wv.start()
    cp_wk.start()
    cp_wr.wait()
    layernorm(0)
    cp_wq.wait()
    wt[0:D, :], nq = transposed(wq)
    proj_q(0, 0, NG // 2)
    x_copy(1).wait()
    proj_q(0, NG // 2, NG)
    layernorm(1)
    cp_wv.wait()
    wt[2 * D:3 * D, :], nv = transposed(wv)
    row16 = lax.broadcasted_iota(jnp.int32, (16, D), 0)
    wt[3 * D:WROWS, :] = jnp.where(
        row16 == 0, wr[...].astype(F32).reshape(1, D), 0.0).astype(BF16)
    cp_wk.wait()
    x_copy(2).start()
    x_copy(3).start()
    cp_wo.start()
    for s in range(NSEG):
        for cp in ffn_copies(s):
            cp.start()
    cp_beta.wait()
    proj_q(1, 0, NG)
    wt[D:2 * D, :], nk = transposed(wk)
    x_copy(2).wait()
    x_copy(3).wait()
    proj_v(0)
    proj_k(0)
    layernorm(2)
    layernorm(3)
    cp_wo.wait()
    for s in range(1, NSEG):
        proj_v(s)
    r1, r2, i1, i2, hot1, hot2 = router()
    wot[:, 0:D] = wo[...].astype(F32).T.astype(BF16)
    b = beta[...].astype(F32).reshape(1, H)
    bt = jnp.broadcast_to(
        jnp.concatenate([b, jnp.zeros((1, 128 - H), F32)], axis=1), (128, 128)).T
    gt_all = _bf(jax.nn.sigmoid(bt[0:H]))
    gtab[0] = gt_all
    gtab[1] = _bf(1.0 - gt_all)
    logit_bound = (DH * QSCALE * XN_SQ_BOUND) * jnp.sqrt(nq) * jnp.sqrt(nk)
    no_shift_needed = ((logit_bound <= SAFE_LOGIT_BOUND)
                       & (XN_SQ_BOUND * nv <= SAFE_VALUE_BOUND * SAFE_VALUE_BOUND))
    for s in range(1, NSEG):
        proj_k(s)
    for s in range(2, NSEG):
        proj_q(s, 0, NG)
    xsel_ref[...] = (
        lax.dot_general(hot1, xn[:, tile_of(i1)], NT, preferred_element_type=F32)
        + lax.dot_general(hot2, xn[:, tile_of(i2)], NT, preferred_element_type=F32))

    krow = lax.broadcasted_iota(jnp.int32, (128, 128), 0)
    kcol = lax.broadcasted_iota(jnp.int32, (128, 128), 1)
    causal = krow <= kcol

    def ffn_cols(u, n=1):
        if isinstance(u, int):
            return slice(u * 128, (u + n) * 128)
        return pl.ds(pl.multiple_of(u * 128, 128), n * 128)

    def ffn_up_part(u, n, lo, hi):
        w2 = jnp.concatenate([wg[lo:hi, ffn_cols(u, n)], wu[lo:hi, ffn_cols(u, n)]], axis=1)
        return jnp.dot(xsel_ref[:, lo:hi], w2, preferred_element_type=F32)

    def ffn_act(gu):
        n = gu.shape[1] // 2
        gate = _bf(gu[:, 0:n])
        return _bf(_bf(gate * jax.nn.sigmoid(gate)) * _bf(gu[:, n:]))

    def ffn_down_part(u, n, hid, lo, hi):
        yacc[:, lo:hi] += lax.dot_general(hid, wd[lo:hi, ffn_cols(u, n)], NT,
                                          preferred_element_type=F32)

    def ffn_items():
        st = {}

        def up(u, lo, hi):
            def run():
                part = ffn_up_part(u, 2, lo, hi)
                st[u] = part if lo == 0 else st[u] + part
                if hi == D:
                    st[u] = ffn_act(st[u])
            return run

        def down(u):
            return lambda: ffn_down_part(u, 1, st[u - u % 2][:, 128 * (u % 2):128 * (u % 2 + 1)], 0, 512)

        def down_tail(u):
            return lambda: ffn_down_part(
                u, 4, jnp.concatenate([st[u], st[u + 2]], axis=1), 512, D)

        bounds = [0, 128, 256, 384, 512, D]
        ups = lambda u: [up(u, bounds[k], bounds[k + 1]) for k in range(5)]
        downs = lambda u: [down(u + k) for k in range(4)] + [down_tail(u)]
        items = []
        for u in range(0, FU + 4, 4):
            if u < FU:
                items += [(f, u + 2) for f in ups(u)] + [(f, u + 4) for f in ups(u + 2)]
            if u > 0:
                items += [(f, u) for f in downs(u - 4)]
        return items + [(ffn_finish, FU)]

    def ffn_finish():
        rowd = lax.broadcasted_iota(jnp.int32, (8, D), 0)
        y = _bf(_bf(yacc[...]) * _bf(jax.nn.sigmoid(jnp.where(rowd == 0, r1, r2))))
        y = jnp.where(rowd < 2, y, 0.0)
        yt = jnp.concatenate([y, jnp.zeros((120, D), F32)], axis=0).T
        wot[:, D:DX] = yt[:, 0:DX - D].astype(BF16)

    def scatter_rows(s):
        row = lax.broadcasted_iota(jnp.int32, (DX - D, L), 0)
        tok = s * L + lax.broadcasted_iota(jnp.int32, (DX - D, L), 1)
        hit = ((row == 0) & (tok == i1)) | ((row == 1) & (tok == i2))
        return jnp.where(hit, 1.0, 0.0)

    def weight_tile(parts):
        blocks = []
        for b in range(KP // 8):
            row = 8 * b + lax.broadcasted_iota(jnp.int32, (8, 128), 0)
            lane = lax.broadcasted_iota(jnp.int32, (8, 128), 1)
            blk = jnp.zeros((8, 128), F32)
            for hh, vals, lo, hi in parts:
                r0, r1 = DH * hh, DH * hh + DH
                if r1 <= 8 * b or r0 >= 8 * b + 8:
                    continue
                keep = None
                for cond in ([row >= r0] if r0 > 8 * b else []) + ([row < r1] if r1 < 8 * b + 8 else []) \
                        + ([lane >= lo] if lo > 0 else []) + ([lane < hi] if hi < 128 else []):
                    keep = cond if keep is None else keep & cond
                v = vals[8 * b:8 * b + 8]
                blk = v if keep is None else jnp.where(keep, v, blk)
            blocks.append(blk)
        return jnp.concatenate(blocks, axis=0).astype(BF16)

    def stage_fns(s, g, g_rows, ret):
        def qk_safe(i):
            q = qts[s, g_rows, 128 * i:128 * (i + 1)]
            qm = jnp.concatenate([weight_tile([(hh, q, 0, 128)]) for hh in range(4)], axis=1)
            nk = 128 * (i + 1)
            st = jnp.dot(kwin[s, g, 0:nk, 0:KP], qm, preferred_element_type=F32)
            ps = []
            for hh in range(4):
                sc = st[:, 128 * hh:128 * (hh + 1)]
                diag = jnp.where(causal, sc[nk - 128:], -1e30)
                sc = jnp.concatenate([sc[:nk - 128], diag], axis=0) if i > 0 else diag
                sc = sc - jnp.max(sc, axis=0, keepdims=True)
                ps.append(jnp.exp2(sc).astype(BF16))
            return ps

        qk = qk_safe

        def pv(i, ps):
            nk = 128 * (i + 1)
            for hh in range(4):
                v = vts[s, g, HS * hh:HS * (hh + 1), 0:nk]
                combine(s, g, ret, i, hh, jnp.dot(v, ps[hh], preferred_element_type=F32))
        return qk, pv

    def combine(s, g, ret, i, hh, o):
        h = 4 * g + hh
        res = o * (gtab[1, pl.ds(h, 1), :] / o[DH:DH + 1])
        if ret is not None:
            mem = ret[DH * hh:DH * hh + HS, 128 * i:128 * (i + 1)]
            den = ret[GD + hh:GD + hh + 1, 128 * i:128 * (i + 1)]
            res = res + mem * (gtab[0, pl.ds(h, 1), :] / (den + 1e-6))
        ot[s, i, pl.ds(DH * h, HS), :] = res

    def qk_items(s, g, i):
        q = qts[s, GD * g:GD * (g + 1), 128 * i:128 * (i + 1)]
        base = 128 * i
        blocks = {}
        st = {}

        def scores(lo, hi, w):
            return jnp.exp2(jnp.dot(kwin[s, g, lo:hi, 0:KP], w, preferred_element_type=F32))

        tile = lambda e, t: e[:, 128 * t:128 * (t + 1)]
        roll = lambda e, t: pltpu.roll(e, t, 1)
        qm = jnp.concatenate([weight_tile([(hh, q, 0, 128)]) for hh in range(4)], axis=1)

        def full(j):
            def run():
                last = j == i - 1
                e = scores(128 * j, 128 * (j + 1) + (32 if last else 0), qm)
                blocks[j] = [tile(e, hh)[0:128].astype(BF16) for hh in range(4)]
                if last:
                    st[0] = e[128:160]
            return run

        def d0():
            st[0] = scores(0, 32, qm)

        def d1():
            st['q'] = [roll(q, t) for t in (32, 64, 96)]
            q32, q64, q96 = st['q']
            st[1] = scores(base + 32, base + 64, jnp.concatenate([
                weight_tile([(0, q, 32, 128), (3, q96, 0, 32)]),
                weight_tile([(1, q, 32, 128), (3, q64, 0, 32)]),
                weight_tile([(2, q, 32, 128), (3, q32, 0, 32)])], axis=1))

        def d2():
            q32, q64, q96 = st['q']
            st[2] = scores(base + 64, base + 96, jnp.concatenate([
                weight_tile([(0, q, 64, 128), (2, q64, 0, 64)]),
                weight_tile([(1, q, 64, 128), (3, q64, 0, 64)])], axis=1))

        def d3():
            q32, q64, q96 = st['q']
            e3 = scores(base + 96, base + 128,
                        weight_tile([(0, q, 96, 128), (1, q96, 64, 96), (2, q64, 32, 64), (3, q32, 0, 32)]))
            e0, e1, e2 = st[0], st[1], st[2]
            lane = lax.broadcasted_iota(jnp.int32, (32, 128), 1)
            blk1 = [tile(e1, 0), tile(e1, 1), tile(e1, 2),
                    jnp.where(lane < 64, roll(tile(e1, 0), 32),
                              jnp.where(lane < 96, roll(tile(e1, 1), 64), roll(tile(e1, 2), 96)))]
            blk2 = [tile(e2, 0), tile(e2, 1), roll(tile(e2, 0), 64), roll(tile(e2, 1), 64)]
            blk3 = [e3, roll(e3, 32), roll(e3, 64), roll(e3, 96)]
            blocks[i] = [
                jnp.where(causal, jnp.concatenate([tile(e0, hh), blk1[hh], blk2[hh], blk3[hh]], axis=0),
                          0.0).astype(BF16) for hh in range(4)]

        items = [full(j) for j in range(i)] + ([d0] if i == 0 else []) + [d1, d2, d3]
        return items, blocks

    def pv_items(s, g, i, rets, blocks):
        acc = {}

        def block(j):
            def run():
                for hh in range(4):
                    v = vts[s, g, HS * hh:HS * (hh + 1), 128 * j:128 * (j + 1)]
                    o = jnp.dot(v, blocks[j][hh], preferred_element_type=F32)
                    acc[hh] = o if j == 0 else acc[hh] + o
                    if j == i:
                        combine(s, g, rets[g], i, hh, acc[hh])
            return run
        return [block(j) for j in range(i + 1)]

    def mem_read(s, g):
        return jnp.dot(mext[g][:, 0:KP], pqt[s, g], preferred_element_type=F32)

    def mem_update(s, g):
        tail = lax.broadcasted_iota(jnp.int32, (KP - GD, L), 0)
        lhs = jnp.concatenate([vts[s, g, HS * hh:HS * hh + DH, :] for hh in range(4)]
                              + [jnp.where(tail == 0, 1.0, 0.0)], axis=0)
        upd = jnp.dot(lhs, pkwin[s, g], preferred_element_type=F32)
        upd = jnp.concatenate(
            [upd[0:GD], jnp.broadcast_to(upd[GD:GD + 1], (KP - GD, 128))], axis=0)
        row = lax.broadcasted_iota(jnp.int32, (KP, 128), 0)
        lane = lax.broadcasted_iota(jnp.int32, (KP, 128), 1)
        head = jnp.where(row < GD, row // DH, row - GD)
        mext[g] = mext[g] + jnp.where((lane >= head * DH) & (lane < head * DH + DH) & (head < 4),
                                      upd, 0.0)

    def wo_part(s, lo, hi, out_rows=slice(0, D)):
        rows = min(hi, D)
        otb = jnp.concatenate([ot[s, i, lo:rows, :] for i in range(QT)], axis=1)
        if hi > D:
            otb = jnp.concatenate([otb, scatter_rows(s)], axis=0)
        return jnp.dot(wot[out_rows, lo:hi], otb.astype(BF16), preferred_element_type=F32)

    def finish(s, att, out_rows=slice(0, D)):
        cols = seg_cols(s)
        res = xs[out_rows, cols].astype(F32) + att + xn[out_rows, cols].astype(F32)
        outs[out_rows, cols] = res.astype(BF16)

    def attention_fast(s, ffn, ffn_tiles_ready, pending):
        deferred = []
        rets = {}

        def extra():
            if ffn:
                f, needs = ffn.pop(0)
                assert needs <= ffn_tiles_ready
                f()

        for g in range(NG):
            rets[g] = None
            for i in range(QT):
                items, blocks = qk_items(s, g, i)
                for n in range(len(items)):
                    items[n]()
                    if n == 0 and deferred:
                        deferred.pop()()
                    if n < len(pending) - 1:
                        pending[n]()
                    if n < i:
                        extra()
                    if (i, n) == (3, 1) and s == 1:
                        extra()
                    if (i, n) == (0, 1 if s < NSEG - 1 else 3) and s > 0:
                        rets[g] = mem_read(s, g)
                    if (i, n) == (0, 3) and s < NSEG - 1:
                        mem_update(s, g)
                if pending and i == 0:
                    deferred.append(pending[-1])
                elif pending:
                    pending[-1]()
                pending = pv_items(s, g, i, rets, blocks)
        return pending

    def wait_ffn_weights(lo, hi):
        for c in range(lo, hi):
            for cp in ffn_copies(c):
                cp.wait()

    KS = 384

    def main_fast():
        ffn = ffn_items()
        pending = []
        for s in range(NSEG - 1):
            pending = attention_fast(s, ffn, FU // 2 if s == 0 else FU, pending)
            if s == 0:
                wait_ffn_weights(2, NSEG)
        assert not ffn
        for s in range(NSEG - 1):
            if s == NSEG - 2:
                for f in pending:
                    f()
            finish(s, wo_part(s, 0, DX))
            out_copy(s).start()
        pending = attention_fast(NSEG - 1, [], FU, [])
        att = wo_part(NSEG - 1, 0, KS)
        for f in pending:
            f()
        for c in range(4):
            rows = slice(c * OC, (c + 1) * OC)
            finish(NSEG - 1, att[rows] + wo_part(NSEG - 1, KS, DX, rows), rows)
            last_copy(c).start()

    def main_safe():
        wait_ffn_weights(2, NSEG)

        def segment(s, carry):
            def body(g, c):
                g_rows = pl.ds(pl.multiple_of(GD * g, 8), GD)
                qk, pv = stage_fns(s, g, g_rows, mem_read(s, g))
                mem_update(s, g)
                for i in range(QT):
                    pv(i, qk(i))
                return c
            return lax.fori_loop(0, NG, body, carry)
        lax.fori_loop(0, NSEG, segment, 0)

        def ffn_body(u, c):
            ffn_down_part(u, 1, ffn_act(ffn_up_part(u, 1, 0, D)), 0, D)
            return c
        lax.fori_loop(0, FU, ffn_body, 0)
        ffn_finish()

        def project(s, c):
            finish(s, wo_part(s, 0, DX))
            return c
        lax.fori_loop(0, NSEG, project, 0)
        for s in range(NSEG - 1):
            out_copy(s).start()
        for c in range(4):
            last_copy(c).start()

    wait_ffn_weights(0, 2)
    lax.cond(no_shift_needed, main_fast, main_safe)
    for s in range(NSEG - 1):
        out_copy(s).wait()
    for c in range(4):
        last_copy(c).wait()


@jax.jit
def pallas_parallel_sum__memory_aug_infini_attn__moe_arch_mod__prompt_kernel(
    A_x: jax.Array,
    A_wq: jax.Array,
    A_wk: jax.Array,
    A_wv: jax.Array,
    A_wo: jax.Array,
    A_beta: jax.Array,
    B_x: jax.Array,
    B_w_r: jax.Array,
    B_w_gate: jax.Array,
    B_w_up: jax.Array,
    B_w_down: jax.Array,
):
    del B_x
    xt = A_x.reshape(S, D).T
    wdt = B_w_down.T
    hbm = pl.BlockSpec(memory_space=pltpu.HBM)
    out = pl.pallas_call(
        _kernel,
        out_shape=jax.ShapeDtypeStruct((D, S), BF16),
        in_specs=[hbm] * 10,
        out_specs=hbm,
        scratch_shapes=[
            pltpu.VMEM((D, S), BF16),
            pltpu.VMEM((D, S), BF16),
            pltpu.VMEM((D, D), BF16),
            pltpu.VMEM((D, D), BF16),
            pltpu.VMEM((D, D), BF16),
            pltpu.VMEM((D, D), BF16),
            pltpu.VMEM((H,), BF16),
            pltpu.VMEM((D,), BF16),
            pltpu.VMEM((WROWS, D), BF16),
            pltpu.VMEM((D, DX), BF16),
            pltpu.VMEM((2, H, 128), F32),
            pltpu.VMEM((NSEG, D, L), F32),
            pltpu.VMEM((NSEG, NG, L, 128), BF16),
            pltpu.VMEM((NSEG, NG, KP, L), BF16),
            pltpu.VMEM((NSEG, NG, L, 128), BF16),
            pltpu.VMEM((NSEG, NG, 4 * HS, L), F32),
            pltpu.VMEM((NG, KP, 128), F32),
            pltpu.VMEM((NSEG, QT, D + 24, 128), F32),
            pltpu.VMEM((D, S), BF16),
            pltpu.VMEM((NSEG * QT, 128), F32),
            pltpu.VMEM((8, D), F32),
            pltpu.VMEM((8, D), F32),
            pltpu.VMEM((D, F), BF16),
            pltpu.VMEM((D, F), BF16),
            pltpu.VMEM((D, F), BF16),
            pltpu.SemaphoreType.DMA((N_SEMS,)),
        ],
        compiler_params=pltpu.CompilerParams(vmem_limit_bytes=110 * 1024 * 1024),
    )(xt, A_wq, A_wk, A_wv, A_wo, A_beta, B_w_r, B_w_gate, B_w_up, wdt)
    return out.T.reshape(1, S, D)
```

```python
import math

import jax
import jax.numpy as jnp
from jax import lax
import jax.experimental.pallas as pl
import jax.experimental.pallas.tpu as pltpu

S = 2048
D = 576
H = 32
DH = 18
NSEG = 4
L = S // NSEG
F = 4608
NG = 8
GD = 4 * DH
HS = 24
QT = L // 128
WROWS = 3 * D + 16
FU = F // 128
FC = F // NSEG
DX = D + 16
KP = 80

F32 = jnp.float32
BF16 = jnp.bfloat16
QSCALE = (DH ** -0.5) * math.log2(math.e)
SAFE_LOGIT_BOUND = 60.0
SAFE_VALUE_BOUND = 2.0 ** 40
XN_SQ_BOUND = 2.0 * D * 1.1

NT = (((1,), (1,)), ((), ()))

(SEM_X, SEM_WQ, SEM_WK, SEM_WV, SEM_WO, SEM_BETA, SEM_WR,
 SEM_OUT, SEM_LAST, SEM_FFN) = 0, 4, 5, 6, 7, 8, 9, 10, 13, 17
N_SEMS = SEM_FFN + 3 * NSEG


def _bf(x):
    return x.astype(BF16).astype(F32)


def _phi(t):
    return jnp.where(t > 0, t + 1.0, jnp.exp(t))


def _max_col_sq(w32):
    return jnp.max(jnp.sum(w32 * w32, axis=0, keepdims=True))


def _rows_padded(a, start, rows):
    stop = min(start + rows, a.shape[0])
    part = a[start:stop]
    if stop - start < rows:
        part = jnp.concatenate([part, jnp.zeros((rows - (stop - start), a.shape[1]), a.dtype)], axis=0)
    return part


def _kernel(x_hbm, wq_hbm, wk_hbm, wv_hbm, wo_hbm, beta_hbm, wr_hbm, wg_hbm, wu_hbm, wd_hbm,
            out_hbm,
            xs, xn, wq, wk, wv, wo, beta, wr, wt, wot, gtab, qts, kwin, pqt, pkwin, vts, mext, ot,
            outs, rbuf, yacc, xsel_ref, wg, wu, wd, sems):

    def seg_cols(s):
        if isinstance(s, int):
            return slice(s * L, (s + 1) * L)
        return pl.ds(pl.multiple_of(s * L, L), L)

    def x_copy(s):
        return pltpu.make_async_copy(x_hbm.at[:, seg_cols(s)], xs.at[:, seg_cols(s)], sems.at[SEM_X + s])

    def out_copy(s):
        return pltpu.make_async_copy(outs.at[:, seg_cols(s)], out_hbm.at[:, seg_cols(s)],
                                     sems.at[SEM_OUT + s])

    OC = D // 4

    def last_copy(c):
        rows, cols = slice(c * OC, (c + 1) * OC), seg_cols(NSEG - 1)
        return pltpu.make_async_copy(outs.at[rows, cols], out_hbm.at[rows, cols], sems.at[SEM_LAST + c])

    cp_wq = pltpu.make_async_copy(wq_hbm, wq, sems.at[SEM_WQ])
    cp_wk = pltpu.make_async_copy(wk_hbm, wk, sems.at[SEM_WK])
    cp_wv = pltpu.make_async_copy(wv_hbm, wv, sems.at[SEM_WV])
    cp_wo = pltpu.make_async_copy(wo_hbm, wo, sems.at[SEM_WO])

    def ffn_copies(s):
        if isinstance(s, int):
            cols = slice(s * FC, (s + 1) * FC)
        else:
            cols = pl.ds(pl.multiple_of(s * FC, 128), FC)
        return [pltpu.make_async_copy(src.at[:, cols], dst.at[:, cols], sems.at[SEM_FFN + 3 * s + k])
                for k, (src, dst) in enumerate(((wg_hbm, wg), (wu_hbm, wu), (wd_hbm, wd)))]

    cp_beta = pltpu.make_async_copy(beta_hbm, beta, sems.at[SEM_BETA])
    cp_wr = pltpu.make_async_copy(wr_hbm, wr, sems.at[SEM_WR])

    def transposed(w_ref):
        w32 = w_ref[...].astype(F32)
        return w32.T.astype(BF16), _max_col_sq(w32)

    def layernorm(s):
        x32 = xs[:, seg_cols(s)].astype(F32)
        mean = jnp.sum(x32, axis=0, keepdims=True) / D
        mean_b = _bf(mean)
        cen = x32 - mean_b
        shift = mean - mean_b
        var = jnp.sum(cen * cen, axis=0, keepdims=True) / D - shift * shift
        den = _bf(jnp.sqrt(_bf(_bf(var) + _bf(jnp.float32(1e-5)))))
        xn[:, seg_cols(s)] = (_bf(cen) * (1.0 / den)).astype(BF16)

    def proj_q(s, g0, g1):
        q = jnp.dot(wt[GD * g0:GD * g1, :], xn[:, seg_cols(s)], preferred_element_type=F32)
        qts[s, GD * g0:GD * g1, :] = q * QSCALE
        pq = _phi(q)
        pad = jnp.zeros((KP - GD, L), F32)
        for g in range(g0, g1):
            win = jnp.concatenate([pq[GD * (g - g0):GD * (g - g0 + 1)], pad], axis=0)
            pqt[s, g] = win.astype(BF16)

    def proj_k(s):
        k = jnp.dot(wt[D:2 * D, :], xn[:, seg_cols(s)], preferred_element_type=F32)
        for g in range(NG):
            kw = _rows_padded(k, GD * g, 128).T
            kwin[s, g] = kw.astype(BF16)
            pkwin[s, g] = _phi(kw).astype(BF16)

    def proj_v(s):
        v = jnp.dot(wt[2 * D:WROWS, :], xn[:, seg_cols(s)], preferred_element_type=F32)
        for j in range(QT):
            rbuf[s * QT + j:s * QT + j + 1, :] = _bf(v[D:D + 1, 128 * j:128 * (j + 1)])
        hrow = lax.broadcasted_iota(jnp.int32, (HS, L), 0)
        fill = jnp.where(hrow == DH, 1.0, 0.0)
        for h in range(H):
            g, hh = divmod(h, 4)
            vts[s, g, HS * hh:HS * (hh + 1), :] = jnp.where(
                hrow < DH, v[DH * h:DH * h + HS], fill)

    def tile_of(idx):
        return pl.ds(pl.multiple_of((idx // 128) * 128, 128), 128)

    def router():
        r = rbuf[...]
        tok = (lax.broadcasted_iota(jnp.int32, r.shape, 0) * 128
               + lax.broadcasted_iota(jnp.int32, r.shape, 1))
        r1 = jnp.max(r)
        i1 = jnp.min(jnp.where(r == r1, tok, S))
        rm = jnp.where(tok == i1, -jnp.inf, r)
        r2 = jnp.max(rm)
        i2 = jnp.min(jnp.where((rm == r2) & (tok != i1), tok, S))
        i1 = jnp.minimum(i1, S - 1)
        i2 = jnp.minimum(i2, S - 1)
        row8 = lax.broadcasted_iota(jnp.int32, (8, 128), 0)
        lane8 = lax.broadcasted_iota(jnp.int32, (8, 128), 1)
        hot1 = jnp.where((row8 == 0) & (lane8 == i1 % 128), 1.0, 0.0)
        hot2 = jnp.where((row8 == 1) & (lane8 == i2 % 128), 1.0, 0.0)
        return r1, r2, i1, i2, hot1, hot2

    x_copy(0).start()
    cp_wr.start()
    cp_beta.start()
    cp_wq.start()
    mext[...] = jnp.zeros(mext.shape, F32)
    yacc[...] = jnp.zeros(yacc.shape, F32)
    x_copy(0).wait()
    x_copy(1).start()
    cp_wv.start()
    cp_wk.start()
    cp_wr.wait()
    layernorm(0)
    cp_wq.wait()
    wt[0:D, :], nq = transposed(wq)
    proj_q(0, 0, NG // 2)
    x_copy(1).wait()
    proj_q(0, NG // 2, NG)
    layernorm(1)
    cp_wv.wait()
    wt[2 * D:3 * D, :], nv = transposed(wv)
    row16 = lax.broadcasted_iota(jnp.int32, (16, D), 0)
    wt[3 * D:WROWS, :] = jnp.where(
        row16 == 0, wr[...].astype(F32).reshape(1, D), 0.0).astype(BF16)
    cp_wk.wait()
    x_copy(2).start()
    x_copy(3).start()
    cp_wo.start()
    for s in range(NSEG):
        for cp in ffn_copies(s):
            cp.start()
    cp_beta.wait()
    proj_q(1, 0, NG)
    wt[D:2 * D, :], nk = transposed(wk)
    x_copy(2).wait()
    x_copy(3).wait()
    proj_v(0)
    proj_k(0)
    layernorm(2)
    layernorm(3)
    cp_wo.wait()
    for s in range(1, NSEG):
        proj_v(s)
    r1, r2, i1, i2, hot1, hot2 = router()
    wot[:, 0:D] = wo[...].astype(F32).T.astype(BF16)
    b = beta[...].astype(F32).reshape(1, H)
    bt = jnp.broadcast_to(
        jnp.concatenate([b, jnp.zeros((1, 128 - H), F32)], axis=1), (128, 128)).T
    gt_all = _bf(jax.nn.sigmoid(bt[0:H]))
    gtab[0] = gt_all
    gtab[1] = _bf(1.0 - gt_all)
    logit_bound = (DH * QSCALE * XN_SQ_BOUND) * jnp.sqrt(nq) * jnp.sqrt(nk)
    no_shift_needed = ((logit_bound <= SAFE_LOGIT_BOUND)
                       & (XN_SQ_BOUND * nv <= SAFE_VALUE_BOUND * SAFE_VALUE_BOUND))
    for s in range(1, NSEG):
        proj_k(s)
    for s in range(2, NSEG):
        proj_q(s, 0, NG)
    xsel_ref[...] = (
        lax.dot_general(hot1, xn[:, tile_of(i1)], NT, preferred_element_type=F32)
        + lax.dot_general(hot2, xn[:, tile_of(i2)], NT, preferred_element_type=F32))

    krow = lax.broadcasted_iota(jnp.int32, (128, 128), 0)
    kcol = lax.broadcasted_iota(jnp.int32, (128, 128), 1)
    causal = krow <= kcol

    def ffn_cols(u, n=1):
        if isinstance(u, int):
            return slice(u * 128, (u + n) * 128)
        return pl.ds(pl.multiple_of(u * 128, 128), n * 128)

    def ffn_up_part(u, n, lo, hi):
        w2 = jnp.concatenate([wg[lo:hi, ffn_cols(u, n)], wu[lo:hi, ffn_cols(u, n)]], axis=1)
        return jnp.dot(xsel_ref[:, lo:hi], w2, preferred_element_type=F32)

    def ffn_act(gu):
        n = gu.shape[1] // 2
        gate = _bf(gu[:, 0:n])
        return _bf(_bf(gate * jax.nn.sigmoid(gate)) * _bf(gu[:, n:]))

    def ffn_down_part(u, n, hid, lo, hi):
        yacc[:, lo:hi] += lax.dot_general(hid, wd[lo:hi, ffn_cols(u, n)], NT,
                                          preferred_element_type=F32)

    def ffn_items():
        st = {}

        def up(u, lo, hi):
            def run():
                part = ffn_up_part(u, 2, lo, hi)
                st[u] = part if lo == 0 else st[u] + part
                if hi == D:
                    st[u] = ffn_act(st[u])
            return run

        def down(u):
            return lambda: ffn_down_part(u, 1, st[u - u % 2][:, 128 * (u % 2):128 * (u % 2 + 1)], 0, 512)

        def down_tail(u):
            return lambda: ffn_down_part(
                u, 4, jnp.concatenate([st[u], st[u + 2]], axis=1), 512, D)

        bounds = [0, 128, 256, 384, 512, D]
        ups = lambda u: [up(u, bounds[k], bounds[k + 1]) for k in range(5)]
        downs = lambda u: [down(u + k) for k in range(4)] + [down_tail(u)]
        items = []
        for u in range(0, FU + 4, 4):
            if u < FU:
                items += [(f, u + 2) for f in ups(u)] + [(f, u + 4) for f in ups(u + 2)]
            if u > 0:
                items += [(f, u) for f in downs(u - 4)]
        return items + [(ffn_finish, FU)]

    def ffn_finish():
        rowd = lax.broadcasted_iota(jnp.int32, (8, D), 0)
        y = _bf(_bf(yacc[...]) * _bf(jax.nn.sigmoid(jnp.where(rowd == 0, r1, r2))))
        y = jnp.where(rowd < 2, y, 0.0)
        yt = jnp.concatenate([y, jnp.zeros((120, D), F32)], axis=0).T
        wot[:, D:DX] = yt[:, 0:DX - D].astype(BF16)

    def scatter_rows(s):
        row = lax.broadcasted_iota(jnp.int32, (DX - D, L), 0)
        tok = s * L + lax.broadcasted_iota(jnp.int32, (DX - D, L), 1)
        hit = ((row == 0) & (tok == i1)) | ((row == 1) & (tok == i2))
        return jnp.where(hit, 1.0, 0.0)

    def weight_tile(parts):
        blocks = []
        for b in range(KP // 8):
            row = 8 * b + lax.broadcasted_iota(jnp.int32, (8, 128), 0)
            lane = lax.broadcasted_iota(jnp.int32, (8, 128), 1)
            blk = jnp.zeros((8, 128), F32)
            for hh, vals, lo, hi in parts:
                r0, r1 = DH * hh, DH * hh + DH
                if r1 <= 8 * b or r0 >= 8 * b + 8:
                    continue
                keep = None
                for cond in ([row >= r0] if r0 > 8 * b else []) + ([row < r1] if r1 < 8 * b + 8 else []) \
                        + ([lane >= lo] if lo > 0 else []) + ([lane < hi] if hi < 128 else []):
                    keep = cond if keep is None else keep & cond
                v = vals[8 * b:8 * b + 8]
                blk = v if keep is None else jnp.where(keep, v, blk)
            blocks.append(blk)
        return jnp.concatenate(blocks, axis=0).astype(BF16)

    def stage_fns(s, g, g_rows, ret):
        def qk_safe(i):
            q = qts[s, g_rows, 128 * i:128 * (i + 1)]
            qm = jnp.concatenate([weight_tile([(hh, q, 0, 128)]) for hh in range(4)], axis=1)
            nk = 128 * (i + 1)
            st = jnp.dot(kwin[s, g, 0:nk, 0:KP], qm, preferred_element_type=F32)
            ps = []
            for hh in range(4):
                sc = st[:, 128 * hh:128 * (hh + 1)]
                diag = jnp.where(causal, sc[nk - 128:], -1e30)
                sc = jnp.concatenate([sc[:nk - 128], diag], axis=0) if i > 0 else diag
                sc = sc - jnp.max(sc, axis=0, keepdims=True)
                ps.append(jnp.exp2(sc).astype(BF16))
            return ps

        qk = qk_safe

        def pv(i, ps):
            nk = 128 * (i + 1)
            for hh in range(4):
                v = vts[s, g, HS * hh:HS * (hh + 1), 0:nk]
                combine(s, g, ret, i, hh, jnp.dot(v, ps[hh], preferred_element_type=F32))
        return qk, pv

    def combine(s, g, ret, i, hh, o):
        h = 4 * g + hh
        res = o * (gtab[1, pl.ds(h, 1), :] / o[DH:DH + 1])
        if ret is not None:
            mem = ret[DH * hh:DH * hh + HS, 128 * i:128 * (i + 1)]
            den = ret[GD + hh:GD + hh + 1, 128 * i:128 * (i + 1)]
            res = res + mem * (gtab[0, pl.ds(h, 1), :] / (den + 1e-6))
        ot[s, i, pl.ds(DH * h, HS), :] = res

    def qk_items(s, g, i):
        q = qts[s, GD * g:GD * (g + 1), 128 * i:128 * (i + 1)]
        base = 128 * i
        blocks = {}
        st = {}

        def scores(lo, hi, w):
            return jnp.exp2(jnp.dot(kwin[s, g, lo:hi, 0:KP], w, preferred_element_type=F32))

        tile = lambda e, t: e[:, 128 * t:128 * (t + 1)]
        roll = lambda e, t: pltpu.roll(e, t, 1)
        qm = jnp.concatenate([weight_tile([(hh, q, 0, 128)]) for hh in range(4)], axis=1)

        def full(j):
            def run():
                last = j == i - 1
                e = scores(128 * j, 128 * (j + 1) + (32 if last else 0), qm)
                blocks[j] = [tile(e, hh)[0:128].astype(BF16) for hh in range(4)]
                if last:
                    st[0] = e[128:160]
            return run

        def d0():
            st[0] = scores(0, 32, qm)

        def d1():
            st['q'] = [roll(q, t) for t in (32, 64, 96)]
            q32, q64, q96 = st['q']
            st[1] = scores(base + 32, base + 64, jnp.concatenate([
                weight_tile([(0, q, 32, 128), (3, q96, 0, 32)]),
                weight_tile([(1, q, 32, 128), (3, q64, 0, 32)]),
                weight_tile([(2, q, 32, 128), (3, q32, 0, 32)])], axis=1))

        def d2():
            q32, q64, q96 = st['q']
            st[2] = scores(base + 64, base + 96, jnp.concatenate([
                weight_tile([(0, q, 64, 128), (2, q64, 0, 64)]),
                weight_tile([(1, q, 64, 128), (3, q64, 0, 64)])], axis=1))

        def d3():
            q32, q64, q96 = st['q']
            e3 = scores(base + 96, base + 128,
                        weight_tile([(0, q, 96, 128), (1, q96, 64, 96), (2, q64, 32, 64), (3, q32, 0, 32)]))
            e0, e1, e2 = st[0], st[1], st[2]
            lane = lax.broadcasted_iota(jnp.int32, (32, 128), 1)
            blk1 = [tile(e1, 0), tile(e1, 1), tile(e1, 2),
                    jnp.where(lane < 64, roll(tile(e1, 0), 32),
                              jnp.where(lane < 96, roll(tile(e1, 1), 64), roll(tile(e1, 2), 96)))]
            blk2 = [tile(e2, 0), tile(e2, 1), roll(tile(e2, 0), 64), roll(tile(e2, 1), 64)]
            blk3 = [e3, roll(e3, 32), roll(e3, 64), roll(e3, 96)]
            blocks[i] = [
                jnp.where(causal, jnp.concatenate([tile(e0, hh), blk1[hh], blk2[hh], blk3[hh]], axis=0),
                          0.0).astype(BF16) for hh in range(4)]

        items = [full(j) for j in range(i)] + ([d0] if i == 0 else []) + [d1, d2, d3]
        return items, blocks

    def pv_items(s, g, i, rets, blocks):
        acc = {}

        def block(j):
            def run():
                for hh in range(4):
                    v = vts[s, g, HS * hh:HS * (hh + 1), 128 * j:128 * (j + 1)]
                    o = jnp.dot(v, blocks[j][hh], preferred_element_type=F32)
                    acc[hh] = o if j == 0 else acc[hh] + o
                    if j == i:
                        combine(s, g, rets[g], i, hh, acc[hh])
            return run
        return [block(j) for j in range(i + 1)]

    def mem_read(s, g):
        return jnp.dot(mext[g][:, 0:KP], pqt[s, g], preferred_element_type=F32)

    def mem_update(s, g):
        tail = lax.broadcasted_iota(jnp.int32, (KP - GD, L), 0)
        lhs = jnp.concatenate([vts[s, g, HS * hh:HS * hh + DH, :] for hh in range(4)]
                              + [jnp.where(tail == 0, 1.0, 0.0)], axis=0)
        upd = jnp.dot(lhs, pkwin[s, g], preferred_element_type=F32)
        upd = jnp.concatenate(
            [upd[0:GD], jnp.broadcast_to(upd[GD:GD + 1], (KP - GD, 128))], axis=0)
        row = lax.broadcasted_iota(jnp.int32, (KP, 128), 0)
        lane = lax.broadcasted_iota(jnp.int32, (KP, 128), 1)
        head = jnp.where(row < GD, row // DH, row - GD)
        mext[g] = mext[g] + jnp.where((lane >= head * DH) & (lane < head * DH + DH) & (head < 4),
                                      upd, 0.0)

    def wo_part(s, lo, hi, out_rows=slice(0, D)):
        rows = min(hi, D)
        otb = jnp.concatenate([ot[s, i, lo:rows, :] for i in range(QT)], axis=1)
        if hi > D:
            otb = jnp.concatenate([otb, scatter_rows(s)], axis=0)
        return jnp.dot(wot[out_rows, lo:hi], otb.astype(BF16), preferred_element_type=F32)

    def finish(s, att, out_rows=slice(0, D)):
        cols = seg_cols(s)
        res = xs[out_rows, cols].astype(F32) + att + xn[out_rows, cols].astype(F32)
        outs[out_rows, cols] = res.astype(BF16)

    def attention_fast(s, ffn, ffn_tiles_ready, pending, filler=None):
        deferred = []
        rets = {}

        def extra():
            if ffn:
                f, needs = ffn.pop(0)
                assert needs <= ffn_tiles_ready
                f()

        for g in range(NG):
            rets[g] = None
            for i in range(QT):
                items, blocks = qk_items(s, g, i)
                for n in range(len(items)):
                    items[n]()
                    if n == 0 and deferred:
                        deferred.pop()()
                    if n < len(pending) - 1:
                        pending[n]()
                    if n < i:
                        extra()
                    if (i, n) == (3, 1) and s == 1:
                        extra()
                    if (i, n) == (0, 1 if s < NSEG - 1 else 3) and s > 0:
                        rets[g] = mem_read(s, g)
                    if (i, n) == (0, 3) and s < NSEG - 1:
                        mem_update(s, g)
                if filler is not None and (g, i) == (0, 0):
                    filler()
                if pending and i == 0:
                    deferred.append(pending[-1])
                elif pending:
                    pending[-1]()
                pending = pv_items(s, g, i, rets, blocks)
        return pending

    def wait_ffn_weights(lo, hi):
        for c in range(lo, hi):
            for cp in ffn_copies(c):
                cp.wait()

    KS = 384

    def main_fast():
        ffn = ffn_items()
        pending = []
        for s in range(NSEG - 1):
            pending = attention_fast(s, ffn, FU // 2 if s == 0 else FU, pending)
            if s == 0:
                wait_ffn_weights(2, NSEG)
        assert not ffn
        def project(s):
            finish(s, wo_part(s, 0, DX))
            out_copy(s).start()

        project(0)
        for f in pending:
            f()
        project(1)
        pending = attention_fast(NSEG - 1, [], FU, [], filler=lambda: project(NSEG - 2))
        att = wo_part(NSEG - 1, 0, KS)
        for f in pending:
            f()
        for c in range(4):
            rows = slice(c * OC, (c + 1) * OC)
            finish(NSEG - 1, att[rows] + wo_part(NSEG - 1, KS, DX, rows), rows)
            last_copy(c).start()

    def main_safe():
        wait_ffn_weights(2, NSEG)

        def segment(s, carry):
            def body(g, c):
                g_rows = pl.ds(pl.multiple_of(GD * g, 8), GD)
                qk, pv = stage_fns(s, g, g_rows, mem_read(s, g))
                mem_update(s, g)
                for i in range(QT):
                    pv(i, qk(i))
                return c
            return lax.fori_loop(0, NG, body, carry)
        lax.fori_loop(0, NSEG, segment, 0)

        def ffn_body(u, c):
            ffn_down_part(u, 1, ffn_act(ffn_up_part(u, 1, 0, D)), 0, D)
            return c
        lax.fori_loop(0, FU, ffn_body, 0)
        ffn_finish()

        def project(s, c):
            finish(s, wo_part(s, 0, DX))
            return c
        lax.fori_loop(0, NSEG, project, 0)
        for s in range(NSEG - 1):
            out_copy(s).start()
        for c in range(4):
            last_copy(c).start()

    wait_ffn_weights(0, 2)
    lax.cond(no_shift_needed, main_fast, main_safe)
    for s in range(NSEG - 1):
        out_copy(s).wait()
    for c in range(4):
        last_copy(c).wait()


@jax.jit
def pallas_parallel_sum__memory_aug_infini_attn__moe_arch_mod__prompt_kernel(
    A_x: jax.Array,
    A_wq: jax.Array,
    A_wk: jax.Array,
    A_wv: jax.Array,
    A_wo: jax.Array,
    A_beta: jax.Array,
    B_x: jax.Array,
    B_w_r: jax.Array,
    B_w_gate: jax.Array,
    B_w_up: jax.Array,
    B_w_down: jax.Array,
):
    del B_x
    xt = A_x.reshape(S, D).T
    wdt = B_w_down.T
    hbm = pl.BlockSpec(memory_space=pltpu.HBM)
    out = pl.pallas_call(
        _kernel,
        out_shape=jax.ShapeDtypeStruct((D, S), BF16),
        in_specs=[hbm] * 10,
        out_specs=hbm,
        scratch_shapes=[
            pltpu.VMEM((D, S), BF16),
            pltpu.VMEM((D, S), BF16),
            pltpu.VMEM((D, D), BF16),
            pltpu.VMEM((D, D), BF16),
            pltpu.VMEM((D, D), BF16),
            pltpu.VMEM((D, D), BF16),
            pltpu.VMEM((H,), BF16),
            pltpu.VMEM((D,), BF16),
            pltpu.VMEM((WROWS, D), BF16),
            pltpu.VMEM((D, DX), BF16),
            pltpu.VMEM((2, H, 128), F32),
            pltpu.VMEM((NSEG, D, L), F32),
            pltpu.VMEM((NSEG, NG, L, 128), BF16),
            pltpu.VMEM((NSEG, NG, KP, L), BF16),
            pltpu.VMEM((NSEG, NG, L, 128), BF16),
            pltpu.VMEM((NSEG, NG, 4 * HS, L), F32),
            pltpu.VMEM((NG, KP, 128), F32),
            pltpu.VMEM((NSEG, QT, D + 24, 128), F32),
            pltpu.VMEM((D, S), BF16),
            pltpu.VMEM((NSEG * QT, 128), F32),
            pltpu.VMEM((8, D), F32),
            pltpu.VMEM((8, D), F32),
            pltpu.VMEM((D, F), BF16),
            pltpu.VMEM((D, F), BF16),
            pltpu.VMEM((D, F), BF16),
            pltpu.SemaphoreType.DMA((N_SEMS,)),
        ],
        compiler_params=pltpu.CompilerParams(vmem_limit_bytes=110 * 1024 * 1024),
    )(xt, A_wq, A_wk, A_wv, A_wo, A_beta, B_w_r, B_w_gate, B_w_up, wdt)
    return out.T.reshape(1, S, D)
```
